```python
import jax
import jax.numpy as jnp

def _softmax(x, axis=-1):
    return jax.nn.softmax(x, axis=axis)

def _gelu(x):
    return jax.nn.gelu(x, approximate=True)

def _silu(x):
    return jax.nn.silu(x)

def _sigmoid(x):
    return jax.nn.sigmoid(x)

def _layernorm(x, axis=-1, eps=1e-05):
    m = jnp.mean(x, axis=axis, keepdims=True)
    v = jnp.var(x, axis=axis, keepdims=True)
    return (x - m) / jnp.sqrt(v + eps)

def _scatter_add(tgt, idx, src, axis=0):
    return tgt.at[idx].add(src)

def _segment_sum(src, seg, n):
    return jax.ops.segment_sum(src, seg, n)

class _Rng:

    def __init__(self, key):
        self._k = key

    def _next(self):
        self._k, sub = jax.random.split(self._k)
        return sub

    def normal(self, shape):
        return jax.random.normal(self._next(), shape, dtype=jnp.bfloat16)

    def randint(self, lo, hi, shape):
        return jax.random.randint(self._next(), shape, lo, hi, dtype=jnp.int32)

    def uniform(self, shape, lo=0.0, hi=1.0):
        return jax.random.uniform(self._next(), shape, jnp.bfloat16, lo, hi)

    def permutation(self, n):
        return jax.random.permutation(self._next(), n)
kernel_name = 'adaLN_cond__ssm_conv_h3__glu_gated_swiglu__prompt'

def setup_inputs():
    _rng = _Rng(jax.random.key(int.from_bytes(__import__("os").urandom(4), "little")))
    _w = lambda a: (lambda t: t.astype(jnp.bfloat16) if jnp.issubdtype(t.dtype, jnp.floating) else t)(jnp.asarray(a))

    def _A_setup():
        B, S, D = (1, 2048, 640)
        ks = 4
        return {'q': _w((lambda *s: _rng.normal(s) * 0.05)(B, S, D)), 'k': _w((lambda *s: _rng.normal(s) * 0.05)(B, S, D)), 'v': _w((lambda *s: _rng.normal(s) * 0.05)(B, S, D)), 'shift_k': _w((lambda *s: _rng.normal(s) * 0.05)(D, ks) * 0.5), 'ssm_k': _w((lambda *s: _rng.normal(s) * 0.05)(D, S) * (1.0 / S ** 0.5)), 'ssm_D': _w((lambda *s: _rng.normal(s) * 0.05)(D))}
    _A_in = _A_setup()

    def _B_setup():
        B, S, D, F = (1, 2048, 640, 1536)
        return {'x': _w((lambda *s: _rng.normal(s) * 0.05)(B, S, D)), 'w1': _w((lambda *s: _rng.normal(s) * 0.05)(D, F) * (2.0 / D) ** 0.5), 'w3': _w((lambda *s: _rng.normal(s) * 0.05)(D, F) * (2.0 / D) ** 0.5), 'w2': _w((lambda *s: _rng.normal(s) * 0.05)(F, D) * (2.0 / F) ** 0.5)}
    _B_in = _B_setup()
    return {'A_q': _A_in['q'], 'A_k': _A_in['k'], 'A_v': _A_in['v'], 'A_shift_k': _A_in['shift_k'], 'A_ssm_k': _A_in['ssm_k'], 'A_ssm_D': _A_in['ssm_D'], 'B_x': _B_in['x'], 'B_w1': _B_in['w1'], 'B_w3': _B_in['w3'], 'B_w2': _B_in['w2'], 'c': _w((lambda *s: _rng.normal(s) * 0.05)(1, 640)), 'w_mod': _w((lambda *s: _rng.normal(s) * 0.05)(640, 6 * 640) * 640 ** (-0.5))}

def reference(A_q, A_k, A_v, A_shift_k, A_ssm_k, A_ssm_D, B_x, B_w1, B_w3, B_w2, c, w_mod):

    def _A_ref(q, k, v, shift_k, ssm_k, ssm_D):
        B, S, D = q.shape
        ks = shift_k.shape[-1]
        k_pad = jnp.pad(k, ((0, 0), (ks - 1, 0), (0, 0)))
        k_shift = jnp.zeros_like(k)
        for t in range(ks):
            k_shift = k_shift + k_pad[:, t:t + S, :] * shift_k[:, ks - 1 - t][None, None, :]
        kv = k_shift * v
        L = 2 * S
        kv_pad = jnp.pad(kv, ((0, 0), (0, S), (0, 0)))
        kf_pad = jnp.pad(ssm_k, ((0, 0), (0, S)))
        kv_f = (lambda x, axes=(-2, -1): jnp.fft.rfft2(x.astype(jnp.float32), axes=axes))(kv_pad[:, None, :, :], axes=(1, 2))
        kf_f = (lambda x, axes=(-2, -1): jnp.fft.rfft2(x.astype(jnp.float32), axes=axes))(kf_pad[:, None, :], axes=(1, 2))
        kf_f = (lambda x, *d: x.transpose(*d))(kf_f, 1, 2, 0)
        y_f = kv_f * kf_f[None, :, :, :]
        y = (lambda x, s, axes=(-2, -1): jnp.fft.irfft2(x, s=s, axes=axes).astype(jnp.bfloat16))(y_f, (1, L), axes=(1, 2))[:, 0, :S, :]
        y = y + kv * ssm_D[None, None, :]
        return q * y

    def _B_ref(x, w1, w3, w2):
        gate = jnp.einsum('bsd,df->bsf', x, w1)
        up = jnp.einsum('bsd,df->bsf', x, w3)
        h = _silu(gate) * up
        out = jnp.einsum('bsf,fd->bsd', h, w2)
        return out
    x = A_q
    mod = (_silu(c) @ w_mod).reshape(c.shape[0], 6, 1, -1)
    sa, ca, ga, sb, cb, gb = (mod[:, 0].copy(), mod[:, 1].copy(), mod[:, 2].copy(), mod[:, 3].copy(), mod[:, 4].copy(), mod[:, 5].copy())
    h = _layernorm(x, axis=-1) * (1 + ca) + sa
    x = x + ga * _A_ref(h, A_k, A_v, A_shift_k, A_ssm_k, A_ssm_D)
    h = _layernorm(x, axis=-1) * (1 + cb) + sb
    x = x + gb * _B_ref(h, B_w1, B_w3, B_w2)
    return x
```

```python
import numpy as np
import jax
import jax.numpy as jnp
from jax import lax
import jax.experimental.pallas as pl
import jax.experimental.pallas.tpu as pltpu

f32 = jnp.float32
bf16 = jnp.bfloat16
u32 = jnp.uint32

S = 2048
D = 640
F = 1536
NG = D // 128
NCH = 4
CH = S // NCH
NDFT = 2 * CH
EPS = 1e-5

BM = 512
SB = 128
RB = 32


def _freq_of_row(r):
    return np.where(r < 64, 2 * r, 2 * (r - 64) + 1)


def _pack_rows_u32(a):
    b = np.asarray(a, dtype=np.float32).astype(jnp.bfloat16).view(np.uint16).astype(np.uint32)
    return b[..., 0::2, :] | (b[..., 1::2, :] << 16)


def _dft_tables():
    r = np.arange(128)
    f1 = _freq_of_row(r).astype(np.float64)
    n1 = np.arange(128, dtype=np.float64)
    fwd = np.zeros((4, 256, 128), np.float64)
    inv = np.zeros((4, 128, 256), np.float64)
    for p in range(4):
        th = 2 * np.pi * (f1[:, None] + 0.5) * (4 * n1[None, :] + p) / NDFT
        c, s = np.cos(th), -np.sin(th)
        nb = 128 // RB
        for b in range(nb):
            fwd[p, 2 * RB * b:2 * RB * b + RB] = c[RB * b:RB * (b + 1)]
            fwd[p, 2 * RB * b + RB:2 * RB * (b + 1)] = s[RB * b:RB * (b + 1)]
        inv[p, :, 0::2] = c.T
        inv[p, :, 1::2] = s.T
    return _pack_rows_u32(fwd), _pack_rows_u32(inv)


def _bc(v):
    return pltpu.bitcast(v, bf16)


def _lo(w):
    return pltpu.bitcast(w << 16, f32)


def _hi(w):
    return pltpu.bitcast(w & jnp.uint32(0xFFFF0000), f32)


def _fft4(zr, zi, inv):
    ar, ai = zr[0] + zr[2], zi[0] + zi[2]
    br, bi = zr[0] - zr[2], zi[0] - zi[2]
    cr, ci = zr[1] + zr[3], zi[1] + zi[3]
    dr, di = zr[1] - zr[3], zi[1] - zi[3]
    if not inv:
        return [ar + cr, br + di, ar - cr, br - di], [ai + ci, bi - dr, ai - ci, bi + dr]
    return [ar + cr, br - di, ar - cr, br + di], [ai + ci, bi + dr, ai - ci, bi - dr]


def _ln(x):
    m = jnp.sum(x, axis=-1, keepdims=True) * (1.0 / D)
    xc = x - m
    v = jnp.sum(xc * xc, axis=-1, keepdims=True) * (1.0 / D)
    return xc * lax.rsqrt(v + EPS)


def _kernel(q_hbm, k_hbm, v_hbm, sk_hbm, w1_hbm, w3_hbm, w2_hbm, wm_hbm,
            shk_ref, dv_ref, c_ref, mf_ref, gi_ref,
            o_ref,
            kbuf, vbuf, skbuf, ktbuf, rx, rk, xh, kh, ub, ybuf,
            qbuf, w1b, w3b, w2b, wmb, modb, sems):
    step = pl.program_id(0)

    def cp_k(g):
        return pltpu.make_async_copy(
            k_hbm.at[0, :, pl.ds(128 * g, 128)],
            kbuf.bitcast(bf16).at[g, pl.ds(16, S), :], sems.at[0, g])

    def cp_v(g):
        return pltpu.make_async_copy(
            v_hbm.at[0, :, pl.ds(128 * g, 128)], vbuf.bitcast(bf16).at[g], sems.at[1, g])

    def cp_s(g):
        return pltpu.make_async_copy(
            sk_hbm.at[pl.ds(128 * g, 128), :], skbuf.at[pl.ds(128 * g, 128), :], sems.at[2, g])

    cp_wm = pltpu.make_async_copy(wm_hbm, wmb, sems.at[3, 0])
    cp_q = pltpu.make_async_copy(q_hbm.at[0], qbuf, sems.at[3, 1])
    cp_w1 = pltpu.make_async_copy(w1_hbm, w1b, sems.at[3, 2])
    cp_w3 = pltpu.make_async_copy(w3_hbm, w3b, sems.at[3, 3])
    cp_w2 = pltpu.make_async_copy(w2_hbm, w2b, sems.at[3, 4])

    def start_group(g):
        cp_k(g).start(); cp_v(g).start(); cp_s(g).start()

    def wait_group(g):
        cp_k(g).wait(); cp_v(g).wait(); cp_s(g).wait()

    def prep_x(g, a, wts):
        w0, w1, w2, w3 = wts
        for rb in range(8):
            kb = 8 + 256 * a + 32 * rb
            ka = kbuf[g, pl.ds(kb, 16, stride=2), :]
            kc = kbuf[g, pl.ds(kb + 1, 16, stride=2), :]
            kam = kbuf[g, pl.ds(kb - 2, 16, stride=2), :]
            kcm = kbuf[g, pl.ds(kb - 1, 16, stride=2), :]
            k0, k1, k2, k3 = _lo(ka), _hi(ka), _lo(kc), _hi(kc)
            k1m, k2m, k3m = _hi(kam), _lo(kcm), _hi(kcm)
            vb = 256 * a + 32 * rb
            va = vbuf[g, pl.ds(vb, 16, stride=2), :]
            vc = vbuf[g, pl.ds(vb + 1, 16, stride=2), :]
            kv = [
                (w0 * k0 + w1 * k3m + w2 * k2m + w3 * k1m) * _lo(va),
                (w0 * k1 + w1 * k0 + w2 * k3m + w3 * k2m) * _hi(va),
                (w0 * k2 + w1 * k1 + w2 * k0 + w3 * k3m) * _lo(vc),
                (w0 * k3 + w1 * k2 + w2 * k1 + w3 * k0) * _hi(vc),
            ]
            for p in range(4):
                rx[g, a, p, pl.ds(8 * rb, 8), :] = pltpu.bitcast(kv[p].astype(bf16), u32)

    def prep_k(g, m):
        blk = skbuf[pl.ds(128 * g, 128), pl.ds(CH * m, CH)]
        ktbuf[g, m] = pltpu.bitcast(blk.T, u32)
        for rb in range(8):
            ka = ktbuf[g, m, pl.ds(32 * rb, 16, stride=2), :]
            kc = ktbuf[g, m, pl.ds(32 * rb + 1, 16, stride=2), :]
            ph = [_lo(ka), _hi(ka), _lo(kc), _hi(kc)]
            for p in range(4):
                rk[g, m, p, pl.ds(8 * rb, 8), :] = pltpu.bitcast(ph[p].astype(bf16), u32)

    def fwd(src, dst, g, a, b, dvec):
        sl = g % 2
        z = [jnp.dot(_bc(mf_ref[p, pl.ds(RB * b, RB), :]), _bc(src[g, a, p]),
                     preferred_element_type=f32) for p in range(4)]
        xr, xi = _fft4([t[:RB] for t in z], [t[RB:] for t in z], False)
        for f2 in range(4):
            re = xr[f2] if dvec is None else xr[f2] + dvec
            dst[sl, a, f2, 0, pl.ds(RB * b, RB), :] = re
            dst[sl, a, f2, 1, pl.ds(RB * b, RB), :] = xi[f2]

    def cell(g, j):
        sl = g % 2
        rows = pl.ds(8 * j, 8)
        even = j < 8
        prev = None
        for c in range(NCH):
            zr, zi = [], []
            for f2 in range(4):
                ar = ai = None
                for a in range(c + 1):
                    m = c - a
                    xr = xh[sl, a, f2, 0, rows, :]
                    xi = xh[sl, a, f2, 1, rows, :]
                    kr = kh[sl, m, f2, 0, rows, :]
                    ki = kh[sl, m, f2, 1, rows, :]
                    tr = xr * kr - xi * ki
                    ti = xr * ki + xi * kr
                    ar = tr if ar is None else ar + tr
                    ai = ti if ai is None else ai + ti
                zr.append(ar); zi.append(ai)
            if prev is None:
                yr, yi = zr, zi
            elif even:
                yr = [zr[f] - prev[1][f] for f in range(4)]
                yi = [zi[f] + prev[0][f] for f in range(4)]
            else:
                yr = [zr[f] + prev[1][f] for f in range(4)]
                yi = [zi[f] - prev[0][f] for f in range(4)]
            prev = (zr, zi)
            ur, ui = _fft4(yr, yi, True)
            for s2 in range(4):
                ub[sl, c, s2, rows, :] = pltpu.bitcast(
                    pltpu.pack_elementwise([ur[s2], ui[s2]], packed_dtype=bf16), u32)

    def inv(g, c, s2):
        sl = g % 2
        y = jnp.dot(_bc(gi_ref[s2]), _bc(ub[sl, c, s2]), preferred_element_type=f32)
        ybuf[g, pl.ds(CH * c + s2, 128, stride=4), :] = y

    @pl.when(step == 0)
    def _phase1():
        start_group(0)
        start_group(1)
        kbuf[:, 0:8, :] = jnp.zeros((NG, 8, 128), u32)
        shk = shk_ref[...].astype(f32)
        dv = dv_ref[...].astype(f32).reshape(1, D)
        for g in range(NG):
            wait_group(g)
            if g + 2 < NG:
                start_group(g + 2)
            if g == NG - 2:
                cp_wm.start(); cp_q.start()
            if g == NG - 1:
                cp_w1.start(); cp_w3.start(); cp_w2.start()
            wts = [jnp.broadcast_to(shk[j:j + 1, 128 * g:128 * (g + 1)], (16, 128)) for j in range(4)]
            dvec = jnp.broadcast_to(dv[:, 128 * g:128 * (g + 1)], (RB, 128))
            for a in range(NCH):
                prep_x(g, a, wts)
                prep_k(g, a)
            for a in range(NCH):
                for b in range(128 // RB):
                    fwd(rx, xh, g, a, b, None)
                    fwd(rk, kh, g, a, b, dvec if a == 0 else None)
            for j in range(16):
                cell(g, j)
            for c in range(NCH):
                for s2 in range(4):
                    inv(g, c, s2)
        cp_wm.wait()
        cc = c_ref[...].astype(f32)
        sc = (cc * jax.nn.sigmoid(cc)).astype(bf16)
        lhs = jnp.broadcast_to(sc, (8, D))
        modb[...] = jnp.dot(lhs, wmb[...], preferred_element_type=f32)
        cp_q.wait(); cp_w1.wait(); cp_w3.wait(); cp_w2.wait()

    sa = modb[0:1, 0 * D:1 * D]
    ca1 = 1.0 + modb[0:1, 1 * D:2 * D]
    ga = modb[0:1, 2 * D:3 * D] * (2.0 / NDFT)
    sb = modb[0:1, 3 * D:4 * D]
    cb1 = 1.0 + modb[0:1, 4 * D:5 * D]
    gb = modb[0:1, 5 * D:6 * D]

    row0 = pl.multiple_of(step * BM, BM)
    for j in range(BM // SB):
        r = pl.ds(row0 + j * SB, SB)
        q = qbuf[r, :].astype(f32)
        y = jnp.concatenate([ybuf[g, r, :] for g in range(NG)], axis=1)
        h1 = _ln(q) * ca1 + sa
        x1 = q + ga * (h1 * y)
        h2 = (_ln(x1) * cb1 + sb).astype(bf16)
        gate = jnp.dot(h2, w1b[...], preferred_element_type=f32)
        up = jnp.dot(h2, w3b[...], preferred_element_type=f32)
        act = (gate * jax.nn.sigmoid(gate) * up).astype(bf16)
        ffn = jnp.dot(act, w2b[...], preferred_element_type=f32)
        o_ref[0, pl.ds(j * SB, SB), :] = (x1 + gb * ffn).astype(bf16)


@jax.jit
def pallas_adaLN_cond__ssm_conv_h3__glu_gated_swiglu__prompt_kernel(
    A_q: jax.Array,
    A_k: jax.Array,
    A_v: jax.Array,
    A_shift_k: jax.Array,
    A_ssm_k: jax.Array,
    A_ssm_D: jax.Array,
    B_x: jax.Array,
    B_w1: jax.Array,
    B_w3: jax.Array,
    B_w2: jax.Array,
    c: jax.Array,
    w_mod: jax.Array,
):
    del B_x
    mf, gi = _dft_tables()
    any_spec = pl.BlockSpec(memory_space=pl.ANY)
    vmem_spec = pl.BlockSpec(memory_space=pltpu.VMEM)
    scratch = [
        pltpu.VMEM((NG, 8 + S // 2, 128), u32),
        pltpu.VMEM((NG, S // 2, 128), u32),
        pltpu.VMEM((D, S), bf16),
        pltpu.VMEM((NG, NCH, CH // 2, 128), u32),
        pltpu.VMEM((NG, NCH, 4, 64, 128), u32),
        pltpu.VMEM((NG, NCH, 4, 64, 128), u32),
        pltpu.VMEM((2, NCH, 4, 2, 128, 128), f32),
        pltpu.VMEM((2, NCH, 4, 2, 128, 128), f32),
        pltpu.VMEM((2, NCH, 4, 128, 128), u32),
        pltpu.VMEM((NG, S, 128), f32),
        pltpu.VMEM((S, D), bf16),
        pltpu.VMEM((D, F), bf16),
        pltpu.VMEM((D, F), bf16),
        pltpu.VMEM((F, D), bf16),
        pltpu.VMEM((D, 6 * D), bf16),
        pltpu.VMEM((8, 6 * D), f32),
        pltpu.SemaphoreType.DMA((4, 8)),
    ]
    return pl.pallas_call(
        _kernel,
        grid=(S // BM,),
        in_specs=[any_spec] * 8 + [vmem_spec] * 5,
        out_specs=pl.BlockSpec((1, BM, D), lambda i: (0, i, 0)),
        out_shape=jax.ShapeDtypeStruct((1, S, D), bf16),
        scratch_shapes=scratch,
        compiler_params=pltpu.CompilerParams(
            dimension_semantics=("arbitrary",),
            vmem_limit_bytes=100 * 1024 * 1024),
    )(A_q, A_k, A_v, A_ssm_k, B_w1, B_w3, B_w2, w_mod,
      A_shift_k.T, A_ssm_D, c, jnp.asarray(mf), jnp.asarray(gi))
```

```python
import numpy as np
import jax
import jax.numpy as jnp
from jax import lax
import jax.experimental.pallas as pl
import jax.experimental.pallas.tpu as pltpu

f32 = jnp.float32
bf16 = jnp.bfloat16
u32 = jnp.uint32

S = 2048
D = 640
F = 1536
NG = D // 128
NCH = 4
CH = S // NCH
NDFT = 2 * CH
EPS = 1e-5

BM = 512
SB = 128
NSB = BM // SB
NSTEP = S // BM
FC = 512
NFC = F // FC
RB = 32
NEXP = 3


def _freq_of_row(r):
    return np.where(r < 64, 2 * r, 2 * (r - 64) + 1)


def _pack_rows_u32(a):
    b = np.asarray(a, dtype=np.float32).astype(jnp.bfloat16).view(np.uint16).astype(np.uint32)
    return b[..., 0::2, :] | (b[..., 1::2, :] << 16)


def _dft_tables():
    r = np.arange(128)
    f1 = _freq_of_row(r).astype(np.float64)
    kap = np.arange(128)
    n1k = (16 * (kap // 16) + 8 * (kap % 2) + (kap % 16) // 2).astype(np.float64)
    n1 = np.arange(128, dtype=np.float64)
    fwd = np.zeros((4, 256, 128), np.float64)
    inv = np.zeros((4, 128, 256), np.float64)
    for p in range(4):
        th = 2 * np.pi * (f1[:, None] + 0.5) * (4 * n1k[None, :] + p) / NDFT
        c, s = np.cos(th), -np.sin(th)
        for b in range(128 // RB):
            fwd[p, 2 * RB * b:2 * RB * b + RB] = c[RB * b:RB * (b + 1)]
            fwd[p, 2 * RB * b + RB:2 * RB * (b + 1)] = s[RB * b:RB * (b + 1)]
        th = 2 * np.pi * (f1[:, None] + 0.5) * (4 * n1[None, :] + p) / NDFT
        inv[p, :, 0::2] = np.cos(th).T
        inv[p, :, 1::2] = -np.sin(th).T
    return _pack_rows_u32(fwd), _pack_rows_u32(inv)


def _bc(v):
    return pltpu.bitcast(v, bf16)


def _lo(w):
    return pltpu.bitcast(w << 16, f32)


def _hi(w):
    return pltpu.bitcast(w & jnp.uint32(0xFFFF0000), f32)


def _pk2(a, b):
    return pltpu.bitcast(pltpu.pack_elementwise([a, b], packed_dtype=bf16), u32)


def _fft4(zr, zi, inv):
    ar, ai = zr[0] + zr[2], zi[0] + zi[2]
    br, bi = zr[0] - zr[2], zi[0] - zi[2]
    cr, ci = zr[1] + zr[3], zi[1] + zi[3]
    dr, di = zr[1] - zr[3], zi[1] - zi[3]
    if not inv:
        return [ar + cr, br + di, ar - cr, br - di], [ai + ci, bi - dr, ai - ci, bi + dr]
    return [ar + cr, br - di, ar - cr, br + di], [ai + ci, bi + dr, ai - ci, bi - dr]


def _ln(x):
    m = jnp.sum(x, axis=-1, keepdims=True) * (1.0 / D)
    xc = x - m
    v = jnp.sum(xc * xc, axis=-1, keepdims=True) * (1.0 / D)
    return xc * lax.rsqrt(v + EPS)


def _kernel(q_hbm, k_hbm, v_hbm, sk_hbm, w1_hbm, w3_hbm, w2_hbm, wm_hbm,
            shk_ref, dv_ref, c_ref, mf_ref, gi_ref, zero_ref, zs_ref,
            o_hbm,
            kbuf, vbuf, skbuf, ktbuf, rx, rk, xh0, xh1, kh0, kh1, ub0, ub1, ybuf,
            qbuf, w1b, w3b, w2b, wmb, modb, hn, xn, hs, xs, accs, obuf, sems):
    xh = (xh0, xh1)
    kh = (kh0, kh1)
    ub = (ub0, ub1)

    def cp_k(g):
        return pltpu.make_async_copy(
            k_hbm.at[0, :, pl.ds(128 * g, 128)],
            kbuf.bitcast(bf16).at[g, pl.ds(16, S), :], sems.at[0, g])

    def cp_v(g):
        return pltpu.make_async_copy(
            v_hbm.at[0, :, pl.ds(128 * g, 128)], vbuf.bitcast(bf16).at[g], sems.at[1, g])

    def cp_s(g):
        return pltpu.make_async_copy(
            sk_hbm.at[pl.ds(128 * g, 128), :], skbuf.at[pl.ds(128 * g, 128), :], sems.at[2, g])

    def cp_wm(i):
        cols = [pl.ds(0, 1536), pl.ds(1536, 5 * D - 1536), pl.ds(5 * D, D)][i]
        return pltpu.make_async_copy(wm_hbm.at[:, cols], wmb.at[:, cols], sems.at[3, i])

    def cp_q(i):
        rows = pl.ds(0, BM) if i == 0 else pl.ds(BM, S - BM)
        return pltpu.make_async_copy(q_hbm.at[0, rows, :], qbuf.at[rows, :], sems.at[3, 4 + i])

    def cp_w(t):
        cols = pl.ds(FC * t, FC)
        return [pltpu.make_async_copy(w1_hbm.at[:, cols], w1b.at[:, cols], sems.at[4, t]),
                pltpu.make_async_copy(w3_hbm.at[:, cols], w3b.at[:, cols], sems.at[5, t]),
                pltpu.make_async_copy(w2_hbm.at[cols, :], w2b.at[cols, :], sems.at[6, t])]

    def cp_o(i):
        rows = pl.ds(pl.multiple_of(i * BM, BM), BM)
        return pltpu.make_async_copy(obuf.at[rows, :], o_hbm.at[0, rows, :], sems.at[7, 0])

    def prep_x(g, a, wts):
        w0, w1, w2, w3 = wts
        for rb in range(8):
            out = []
            for h in range(2):
                kb = 8 + 256 * a + 32 * rb + 16 * h
                ka = kbuf[g, pl.ds(kb, 8, stride=2), :]
                kc = kbuf[g, pl.ds(kb + 1, 8, stride=2), :]
                kam = kbuf[g, pl.ds(kb - 2, 8, stride=2), :]
                kcm = kbuf[g, pl.ds(kb - 1, 8, stride=2), :]
                k0, k1, k2, k3 = _lo(ka), _hi(ka), _lo(kc), _hi(kc)
                k1m, k2m, k3m = _hi(kam), _lo(kcm), _hi(kcm)
                vb = 256 * a + 32 * rb + 16 * h
                va = vbuf[g, pl.ds(vb, 8, stride=2), :]
                vc = vbuf[g, pl.ds(vb + 1, 8, stride=2), :]
                out.append([
                    (w0 * k0 + w1 * k3m + w2 * k2m + w3 * k1m) * _lo(va),
                    (w0 * k1 + w1 * k0 + w2 * k3m + w3 * k2m) * _hi(va),
                    (w0 * k2 + w1 * k1 + w2 * k0 + w3 * k3m) * _lo(vc),
                    (w0 * k3 + w1 * k2 + w2 * k1 + w3 * k0) * _hi(vc)])
            for p in range(4):
                rx[g, a, p, pl.ds(8 * rb, 8), :] = _pk2(out[0][p], out[1][p])

    def prep_k(g, m):
        blk = skbuf[pl.ds(128 * g, 128), pl.ds(CH * m, CH)]
        ktbuf[g, m] = pltpu.bitcast(blk.T, u32)
        lo16 = jnp.uint32(0xFFFF)
        hi16 = jnp.uint32(0xFFFF0000)
        for rb in range(8):
            w = [[ktbuf[g, m, pl.ds(32 * rb + 16 * h + e, 8, stride=2), :] for e in range(2)]
                 for h in range(2)]
            rows = pl.ds(8 * rb, 8)
            rk[g, m, 0, rows, :] = (w[0][0] & lo16) | (w[1][0] << 16)
            rk[g, m, 1, rows, :] = (w[0][0] >> 16) | (w[1][0] & hi16)
            rk[g, m, 2, rows, :] = (w[0][1] & lo16) | (w[1][1] << 16)
            rk[g, m, 3, rows, :] = (w[0][1] >> 16) | (w[1][1] & hi16)

    def fwd(src, dst, g, a, b, dvec):
        z = [jnp.dot(_bc(mf_ref[p, pl.ds(RB * b, RB), :]), _bc(src[g, a, p]),
                     preferred_element_type=f32) for p in range(4)]
        xr, xi = _fft4([t[:RB] for t in z], [t[RB:] for t in z], False)
        for f2 in range(4):
            dst[a, f2, 0, pl.ds(RB * b, RB), :] = xr[f2] if dvec is None else xr[f2] + dvec
            dst[a, f2, 1, pl.ds(RB * b, RB), :] = xi[f2]

    def cell(g, j, mask, inj):
        xs_, ks_, us_ = xh[g % 2], kh[g % 2], ub[g % 2]
        rows = pl.ds(8 * j, 8)
        even = j < 8
        prev = None
        tok = None
        for c in range(NCH):
            zr, zi = [], []
            for f2 in range(4):
                ar = ai = None
                for a in range(c + 1):
                    m = c - a
                    xr = xs_[a, f2, 0, rows, :]
                    xi = xs_[a, f2, 1, rows, :]
                    kr = ks_[m, f2, 0, rows, :]
                    ki = ks_[m, f2, 1, rows, :]
                    if inj is not None and c == 0 and f2 == 0:
                        kr = jnp.where(mask, inj, kr)
                    tr = xr * kr - xi * ki
                    ti = xr * ki + xi * kr
                    ar = tr if ar is None else ar + tr
                    ai = ti if ai is None else ai + ti
                zr.append(ar)
                zi.append(ai)
            if prev is None:
                yr, yi = zr, zi
            elif even:
                yr = [zr[f] - prev[1][f] for f in range(4)]
                yi = [zi[f] + prev[0][f] for f in range(4)]
            else:
                yr = [zr[f] + prev[1][f] for f in range(4)]
                yi = [zi[f] - prev[0][f] for f in range(4)]
            prev = (zr, zi)
            ur, ui = _fft4(yr, yi, True)
            for s2 in range(4):
                pk = _pk2(ur[s2], ui[s2])
                us_[c, s2, rows, :] = pk
                tok = pk if tok is None else tok | pk
        t = pltpu.bitcast(tok, f32)
        for _ in range(NEXP):
            t = jnp.exp(t)
        return t

    def inv(g, c, s2):
        y = jnp.dot(_bc(gi_ref[s2]), _bc(ub[g % 2][c, s2]), preferred_element_type=f32)
        ybuf[g, pl.ds(CH * c + s2, 128, stride=4), :] = y

    def mod_cols(lo_, n):
        cc = c_ref[...].astype(f32)
        sc = (cc * jax.nn.sigmoid(cc)).astype(bf16)
        lhs = jnp.broadcast_to(sc, (8, D))
        modb[:, pl.ds(lo_, n)] = jnp.dot(lhs, wmb[:, pl.ds(lo_, n)], preferred_element_type=f32)

    _cnt = [0]

    def first_step():
        i = _cnt[0]
        _cnt[0] += 1
        return zs_ref[i] == 0

    def prologue(r):
        sa = modb[0:1, 0 * D:1 * D]
        ca1 = 1.0 + modb[0:1, 1 * D:2 * D]
        ga = modb[0:1, 2 * D:3 * D] * (2.0 / NDFT)
        sb = modb[0:1, 3 * D:4 * D]
        cb1 = 1.0 + modb[0:1, 4 * D:5 * D]
        q = qbuf[r, :].astype(f32)
        y = jnp.concatenate([ybuf[g, r, :] for g in range(NG)], axis=1)
        h1 = _ln(q) * ca1 + sa
        x1 = q + ga * (h1 * y)
        h2 = (_ln(x1) * cb1 + sb).astype(bf16)
        return x1, h2

    def ffn_part(h2, lo_, n):
        cols = pl.ds(lo_, n)
        gate = jnp.dot(h2, w1b[:, cols], preferred_element_type=f32)
        up = jnp.dot(h2, w3b[:, cols], preferred_element_type=f32)
        act = (gate * jax.nn.sigmoid(gate) * up).astype(bf16)
        return jnp.dot(act, w2b[cols, :], preferred_element_type=f32)

    def next_prologue(row):
        x1, h2 = prologue(pl.ds(row, SB))
        xn[...] = x1
        hn[...] = h2

    def issue_group(g):
        cp_k(g).start(); cp_v(g).start(); cp_s(g).start()

    def issue_w(t):
        for c_ in cp_w(t):
            c_.start()

    stage = {
        ("blk2", 0): lambda: issue_group(2),
        ("blk1", 1): lambda: issue_group(3),
        ("blk2", 1): lambda: issue_group(4),
        ("blk1", 2): lambda: cp_wm(0).start(),
        ("blk2", 2): lambda: cp_wm(1).start(),
        ("blk1", 3): lambda: cp_q(0).start(),
        ("blk2", 3): lambda: issue_w(0),
        ("blk1", 4): lambda: issue_w(1),
        ("blk2", 4): lambda: (cp_wm(2).start(), issue_w(2)),
        ("blk3", 0): lambda: cp_q(1).start(),
    }

    def issue(name, g):
        if (name, g) in stage:
            stage[(name, g)]()

    @pl.when(first_step())
    def _issue():
        issue_group(0)
        issue_group(1)
        kbuf[:, 0:8, :] = jnp.zeros((NG, 8, 128), u32)

    for g in range(NG):
        @pl.when(first_step())
        def _blk1(g=g):
            issue("blk1", g)
            cp_k(g).wait(); cp_v(g).wait(); cp_s(g).wait()
            shk = shk_ref[...].astype(f32)
            dv = dv_ref[...].astype(f32).reshape(1, D)
            wts = [jnp.broadcast_to(shk[j:j + 1, 128 * g:128 * (g + 1)], (8, 128)) for j in range(4)]
            dvec = jnp.broadcast_to(dv[:, 128 * g:128 * (g + 1)], (RB, 128))
            for a in range(NCH):
                prep_x(g, a, wts)
                prep_k(g, a)
            for a in range(NCH):
                for b in range(128 // RB):
                    fwd(rx, xh[g % 2], g, a, b, None)
                for b in range(128 // RB):
                    fwd(rk, kh[g % 2], g, a, b, dvec if a == 0 else None)

        @pl.when(first_step())
        def _blk2(g=g):
            issue("blk2", g)
            if g == NG - 1:
                cp_wm(0).wait()
                cp_wm(1).wait()
            mask = zero_ref[...] != 0
            inj = None
            for j in range(16):
                inj = cell(g, j, mask, inj)
            if g > 0:
                for c in range(NCH):
                    for s2 in range(4):
                        inv(g - 1, c, s2)
            if g == NG - 1:
                mod_cols(0, 5 * D)

    @pl.when(first_step())
    def _blk3():
        issue("blk3", 0)
        cp_q(0).wait()
        for c in range(NCH):
            for s2 in range(4):
                inv(NG - 1, c, s2)
        next_prologue(0)

    def _step(step, carry):
        row0 = pl.multiple_of(step * BM, BM)
        for t in range(NFC):
            @pl.when(step == zs_ref[16 + t])
            def _waits(t=t):
                for c_ in cp_w(t):
                    c_.wait()
                if t == NFC - 1:
                    cp_wm(2).wait()
                    cp_q(1).wait()
                    mod_cols(5 * D, D)

            for j in range(NSB):
                r = pl.ds(j * SB, SB)
                if t == 0:
                    if j == 0:
                        x1, h2 = xn[...], hn[...]
                    else:
                        x1, h2 = prologue(pl.ds(row0 + j * SB, SB))
                    xs[r, :] = x1
                    hs[r, :] = h2
                    accs[r, :] = ffn_part(h2, 0, FC)
                elif t < NFC - 1:
                    accs[r, :] += ffn_part(hs[r, :], t * FC, FC)
                else:
                    gb = modb[0:1, 5 * D:6 * D]
                    ffn = accs[r, :] + ffn_part(hs[r, :], t * FC, FC)
                    obuf[pl.ds(row0 + j * SB, SB), :] = (xs[r, :] + gb * ffn).astype(bf16)
            if t == NFC - 1:
                nxt = jnp.minimum(row0 + BM, S - SB)
                next_prologue(pl.multiple_of(nxt, SB))
                cp_o(step).start()
        return carry

    lax.fori_loop(0, NSTEP, _step, 0)
    for i in range(NSTEP):
        cp_o(i).wait()


@jax.jit
def pallas_adaLN_cond__ssm_conv_h3__glu_gated_swiglu__prompt_kernel(
    A_q: jax.Array,
    A_k: jax.Array,
    A_v: jax.Array,
    A_shift_k: jax.Array,
    A_ssm_k: jax.Array,
    A_ssm_D: jax.Array,
    B_x: jax.Array,
    B_w1: jax.Array,
    B_w3: jax.Array,
    B_w2: jax.Array,
    c: jax.Array,
    w_mod: jax.Array,
):
    del B_x
    mf, gi = _dft_tables()
    any_spec = pl.BlockSpec(memory_space=pl.ANY)
    vmem_spec = pl.BlockSpec(memory_space=pltpu.VMEM)
    scratch = [
        pltpu.VMEM((NG, 8 + S // 2, 128), u32),
        pltpu.VMEM((NG, S // 2, 128), u32),
        pltpu.VMEM((D, S), bf16),
        pltpu.VMEM((NG, NCH, CH // 2, 128), u32),
        pltpu.VMEM((NG, NCH, 4, 64, 128), u32),
        pltpu.VMEM((NG, NCH, 4, 64, 128), u32),
        pltpu.VMEM((NCH, 4, 2, 128, 128), f32),
        pltpu.VMEM((NCH, 4, 2, 128, 128), f32),
        pltpu.VMEM((NCH, 4, 2, 128, 128), f32),
        pltpu.VMEM((NCH, 4, 2, 128, 128), f32),
        pltpu.VMEM((NCH, 4, 128, 128), u32),
        pltpu.VMEM((NCH, 4, 128, 128), u32),
        pltpu.VMEM((NG, S, 128), f32),
        pltpu.VMEM((S, D), bf16),
        pltpu.VMEM((D, F), bf16),
        pltpu.VMEM((D, F), bf16),
        pltpu.VMEM((F, D), bf16),
        pltpu.VMEM((D, 6 * D), bf16),
        pltpu.VMEM((8, 6 * D), f32),
        pltpu.VMEM((SB, D), bf16),
        pltpu.VMEM((SB, D), f32),
        pltpu.VMEM((BM, D), bf16),
        pltpu.VMEM((BM, D), f32),
        pltpu.VMEM((BM, D), f32),
        pltpu.VMEM((S, D), bf16),
        pltpu.SemaphoreType.DMA((8, 8)),
    ]
    return pl.pallas_call(
        _kernel,
        in_specs=[any_spec] * 8 + [vmem_spec] * 6 + [pl.BlockSpec(memory_space=pltpu.SMEM)],
        out_specs=any_spec,
        out_shape=jax.ShapeDtypeStruct((1, S, D), bf16),
        scratch_shapes=scratch,
        compiler_params=pltpu.CompilerParams(
            vmem_limit_bytes=100 * 1024 * 1024),
    )(A_q, A_k, A_v, A_ssm_k, B_w1, B_w3, B_w2, w_mod,
      A_shift_k.T, A_ssm_D, c, jnp.asarray(mf), jnp.asarray(gi),
      jnp.zeros((8, 128), jnp.uint32), jnp.zeros((32,), jnp.int32))
```

```python
import os as _os
import numpy as np
import jax
import jax.numpy as jnp
from jax import lax
import jax.experimental.pallas as pl
import jax.experimental.pallas.tpu as pltpu

f32 = jnp.float32
bf16 = jnp.bfloat16
u32 = jnp.uint32

S = 2048
D = 640
F = 1536
NG = D // 128
NCH = 4
CH = S // NCH
NDFT = 2 * CH
EPS = 1e-5

BM = 512
SB = 128
NSB = BM // SB
BM2 = int(_os.environ.get('BM2', 256))
NSTEP2 = (S - BM) // BM2
FCS = tuple(int(x) for x in _os.environ.get('FCS', '256,512,768').split(','))
NFC = len(FCS)
FLO = tuple(sum(FCS[:i]) for i in range(NFC))
KPAD = 40
RB = 32
PCH = 1
NRCP_P = 2
PR = 136
PCHAIN0 = False
RCP_B = tuple(float(x) for x in _os.environ.get('RCP_B', '0,0.34,1.34,2.34').split(','))


def _freq_of_row(r):
    return np.where(r < 64, 2 * r, 2 * (r - 64) + 1)


def _pack_rows_u32(a):
    b = np.asarray(a, dtype=np.float32).astype(jnp.bfloat16).view(np.uint16).astype(np.uint32)
    return b[..., 0::2, :] | (b[..., 1::2, :] << 16)


def _dft_tables():
    r = np.arange(128)
    f1 = _freq_of_row(r).astype(np.float64)
    n1 = np.arange(128, dtype=np.float64)
    fwd = np.zeros((4, 256, 128), np.float64)
    inv = np.zeros((4, 128, 256), np.float64)
    for p in range(4):
        th = 2 * np.pi * (f1[:, None] + 0.5) * (4 * n1[None, :] + p) / NDFT
        c, s = np.cos(th), -np.sin(th)
        for b in range(128 // RB):
            fwd[p, 2 * RB * b:2 * RB * b + RB] = c[RB * b:RB * (b + 1)]
            fwd[p, 2 * RB * b + RB:2 * RB * (b + 1)] = s[RB * b:RB * (b + 1)]
        inv[p, :, 0::2] = c.T
        inv[p, :, 1::2] = s.T
    return _pack_rows_u32(fwd), _pack_rows_u32(inv)


def _bc(v):
    return pltpu.bitcast(v, bf16)


def _lo(w):
    return pltpu.bitcast(w << 16, f32)


def _hi(w):
    return pltpu.bitcast(w & jnp.uint32(0xFFFF0000), f32)


def _pk2(a, b):
    return pltpu.bitcast(pltpu.pack_elementwise([a, b], packed_dtype=bf16), u32)


def _fft4(zr, zi, inv):
    ar, ai = zr[0] + zr[2], zi[0] + zi[2]
    br, bi = zr[0] - zr[2], zi[0] - zi[2]
    cr, ci = zr[1] + zr[3], zi[1] + zi[3]
    dr, di = zr[1] - zr[3], zi[1] - zi[3]
    if not inv:
        return [ar + cr, br + di, ar - cr, br - di], [ai + ci, bi - dr, ai - ci, bi + dr]
    return [ar + cr, br - di, ar - cr, br + di], [ai + ci, bi + dr, ai - ci, bi - dr]


def _ln(x):
    m = jnp.sum(x, axis=-1, keepdims=True) * (1.0 / D)
    xc = x - m
    v = jnp.sum(xc * xc, axis=-1, keepdims=True) * (1.0 / D)
    return xc * lax.rsqrt(v + EPS)


def _kernel(q_hbm, k_hbm, v_hbm, sk_hbm, w1_hbm, w3_hbm, w2_hbm, wm_hbm, mf_hbm, gi_hbm,
            shk_ref, dv_ref, c_ref, zero_ref, zs_ref,
            o_hbm,
            kraw, vraw, skbuf, ktbuf, rx, rk, xh, kh, zb, ub0, ub1, ybuf,
            qbuf, w1b, w3b, w2b, wmb, modb, hn, xn, hs, xs, accs, obuf, mf_ref, gi_ref, sems):
    ub = (ub0, ub1)

    def cp_k(a):
        return pltpu.make_async_copy(
            k_hbm.at[pl.ds(5 * CH * a, 5 * CH), :],
            kraw.bitcast(bf16).at[pl.ds(2 * KPAD + 5 * CH * a, 5 * CH), :], sems.at[0, a])

    def cp_v(a):
        return pltpu.make_async_copy(
            v_hbm.at[pl.ds(5 * CH * a, 5 * CH), :],
            vraw.bitcast(bf16).at[pl.ds(5 * CH * a, 5 * CH), :], sems.at[1, a])

    def cp_s(a):
        cols = pl.ds(CH * a, CH)
        return pltpu.make_async_copy(sk_hbm.at[:, cols], skbuf.at[:, cols], sems.at[2, a])

    def cp_wm(i):
        cols = [pl.ds(0, 1536), pl.ds(1536, 5 * D - 1536), pl.ds(5 * D, D)][i]
        return pltpu.make_async_copy(wm_hbm.at[:, cols], wmb.at[:, cols], sems.at[3, i])

    def cp_q(i):
        rows = pl.ds(0, BM) if i == 0 else pl.ds(BM, S - BM)
        return pltpu.make_async_copy(q_hbm.at[0, rows, :], qbuf.at[rows, :], sems.at[3, 4 + i])

    def cp_w(t):
        cols = pl.ds(FLO[t], FCS[t])
        return [pltpu.make_async_copy(w1_hbm.at[:, cols], w1b.at[:, cols], sems.at[4, t]),
                pltpu.make_async_copy(w3_hbm.at[:, cols], w3b.at[:, cols], sems.at[5, t]),
                pltpu.make_async_copy(w2_hbm.at[cols, :], w2b.at[cols, :], sems.at[6, t])]

    cp_mf = pltpu.make_async_copy(mf_hbm, mf_ref, sems.at[7, 1])
    cp_gi = pltpu.make_async_copy(gi_hbm, gi_ref, sems.at[7, 2])

    def cp_o(row, n):
        rows = pl.ds(row, n)
        return pltpu.make_async_copy(obuf.at[rows, :], o_hbm.at[0, rows, :], sems.at[7, 0])

    def prep_x(g, a, t, wts, mask, inj):
        i0_ = 64 * a + 8 * t
        kb = KPAD + 20 * i0_ + 4 * g
        kl = [kraw[pl.ds(kb + w, 8, stride=20), :] for w in range(4)]
        km2 = kraw[pl.ds(kb - 18, 8, stride=20), :]
        km3 = kraw[pl.ds(kb - 17, 8, stride=20), :]
        e = [_hi(km2), _lo(km3), _hi(km3)]
        for w in range(4):
            e += [_lo(kl[w]), _hi(kl[w])]
        if inj is not None:
            e[3] = jnp.where(mask, inj, e[3])
        vb = 20 * i0_ + 4 * g
        kv = []
        for w in range(4):
            vw = vraw[pl.ds(vb + w, 8, stride=20), :]
            for h, vv in enumerate((_lo(vw), _hi(vw))):
                r = 3 + 2 * w + h
                ks = wts[0] * e[r] + wts[1] * e[r - 1] + wts[2] * e[r - 2] + wts[3] * e[r - 3]
                kv.append(ks * vv)
        tok = None
        for p in range(4):
            pk = _pk2(kv[p], kv[p + 4])
            rx[g, p, pl.ds(8 * t, 8), :] = pk
            tok = pk if tok is None else tok | pk
        return tok

    def prep_k(g, m):
        blk = skbuf[pl.ds(128 * g, 128), pl.ds(CH * m, CH)]
        ktbuf[g] = pltpu.bitcast(blk.T, u32)
        lo16 = jnp.uint32(0xFFFF)
        hi16 = jnp.uint32(0xFFFF0000)
        for t in range(8):
            w = [ktbuf[g, pl.ds(32 * t + e_, 8, stride=4), :] for e_ in range(4)]
            rows = pl.ds(8 * t, 8)
            rk[g, 0, rows, :] = (w[0] & lo16) | (w[2] << 16)
            rk[g, 1, rows, :] = (w[0] >> 16) | (w[2] & hi16)
            rk[g, 2, rows, :] = (w[1] & lo16) | (w[3] << 16)
            rk[g, 3, rows, :] = (w[1] >> 16) | (w[3] & hi16)

    def fwd(src, dst, g, a, b, dvec):
        z = [jnp.dot(_bc(mf_ref[p, pl.ds(RB * b, RB), :]), _bc(src[g, p]),
                     preferred_element_type=f32) for p in range(4)]
        xr, xi = _fft4([t[:RB] for t in z], [t[RB:] for t in z], False)
        for f2 in range(4):
            dst[g, a, f2, 0, pl.ds(RB * b, RB), :] = xr[f2] if dvec is None else xr[f2] + dvec
            dst[g, a, f2, 1, pl.ds(RB * b, RB), :] = xi[f2]

    def cell(g, j, c, mask, inj):
        rows = pl.ds(8 * j, 8)
        zr, zi = [], []
        for f2 in range(4):
            ar = ai = None
            for a in range(c + 1):
                m = c - a
                xr = xh[g, a, f2, 0, rows, :]
                xi = xh[g, a, f2, 1, rows, :]
                kr = kh[g, m, f2, 0, rows, :]
                ki = kh[g, m, f2, 1, rows, :]
                if inj is not None and f2 == 0 and a == 0:
                    kr = jnp.where(mask, inj, kr)
                tr = xr * kr - xi * ki
                ti = xr * ki + xi * kr
                ar = tr if ar is None else ar + tr
                ai = ti if ai is None else ai + ti
            zr.append(ar)
            zi.append(ai)
        yr, yi = zr, zi
        if c > 0:
            pr = [zb[g, f, 0, rows, :] for f in range(4)]
            pi = [zb[g, f, 1, rows, :] for f in range(4)]
            if j < 8:
                yr = [zr[f] - pi[f] for f in range(4)]
                yi = [zi[f] + pr[f] for f in range(4)]
            else:
                yr = [zr[f] + pi[f] for f in range(4)]
                yi = [zi[f] - pr[f] for f in range(4)]
        if c + 1 < NCH:
            for f in range(4):
                zb[g, f, 0, rows, :] = zr[f]
                zb[g, f, 1, rows, :] = zi[f]
        ur, ui = _fft4(yr, yi, True)
        tok = None
        for s2 in range(4):
            pk = _pk2(ur[s2], ui[s2])
            ub[c % 2][g, s2, rows, :] = pk
            tok = pk if tok is None else tok | pk
        return tok

    def inv(g, c, s2):
        y = jnp.dot(_bc(gi_ref[s2]), _bc(ub[c % 2][g, s2, 0:128, :]), preferred_element_type=f32)
        ybuf[g, pl.ds(CH * c + s2, 128, stride=4), :] = y

    def delayed(tok, n):
        t = pltpu.bitcast(tok, f32)
        for _ in range(n):
            t = pl.reciprocal(t, approx=True)
        return t

    def mod_cols(lo_, n):
        cc = c_ref[...].astype(f32)
        sc = (cc * jax.nn.sigmoid(cc)).astype(bf16)
        lhs = jnp.broadcast_to(sc, (8, D))
        modb[:, pl.ds(lo_, n)] = jnp.dot(lhs, wmb[:, pl.ds(lo_, n)], preferred_element_type=f32)

    _cnt = [0]

    def first_step():
        i = _cnt[0]
        _cnt[0] += 1
        return zs_ref[i] == 0

    def prologue(row, nchunk):
        sa = modb[0:1, 0 * D:1 * D]
        ca1 = 1.0 + modb[0:1, 1 * D:2 * D]
        ga = modb[0:1, 2 * D:3 * D] * (2.0 / NDFT)
        sb = modb[0:1, 3 * D:4 * D]
        cb1 = 1.0 + modb[0:1, 4 * D:5 * D]
        mask = zero_ref[...] != 0
        n = SB // nchunk
        x1s, h2s = [], []
        tok = None
        for i in range(nchunk):
            r = pl.ds(row + i * n, n)
            q = qbuf[r, :].astype(f32)
            if tok is not None:
                q00 = jnp.where(mask, tok, q[0:8, 0:128])
                top = jnp.concatenate([q00, q[0:8, 128:]], axis=1)
                q = jnp.concatenate([top, q[8:]], axis=0)
            y = jnp.concatenate([ybuf[g, r, :] for g in range(NG)], axis=1)
            h1 = _ln(q) * ca1 + sa
            x1 = q + ga * (h1 * y)
            h2f = _ln(x1) * cb1 + sb
            if i + 1 < nchunk:
                parts = [h2f[8 * a:8 * a + 8, 128 * g:128 * (g + 1)]
                         for a in range(n // 8) for g in range(NG)]
                while len(parts) > 1:
                    parts = [parts[k] + parts[k + 1] if k + 1 < len(parts) else parts[k]
                             for k in range(0, len(parts), 2)]
                tok = parts[0]
            x1s.append(x1)
            h2s.append(h2f.astype(bf16))
        return jnp.concatenate(x1s, axis=0), jnp.concatenate(h2s, axis=0)

    def ffn_part(h2, lo_, n):
        cols = pl.ds(lo_, n)
        gate = jnp.dot(h2, w1b[:, cols], preferred_element_type=f32)
        up = jnp.dot(h2, w3b[:, cols], preferred_element_type=f32)
        act = (gate * jax.nn.sigmoid(gate) * up).astype(bf16)
        return jnp.dot(act, w2b[cols, :], preferred_element_type=f32)

    def next_prologue(row, nchunk):
        x1, h2 = prologue(row, nchunk)
        xn[...] = x1
        hn[...] = h2

    @pl.when(first_step())
    def _issue():
        for a in range(NCH):
            cp_s(a).start()
            if a == 0:
                cp_mf.start()
            cp_k(a).start(); cp_v(a).start()
            if a == 1:
                cp_gi.start()
        cp_wm(0).start()
        cp_wm(1).start()
        cp_q(0).start()
        for t in range(NFC):
            if t == NFC - 1:
                cp_wm(2).start()
            for c_ in cp_w(t):
                c_.start()
        cp_q(1).start()
        kraw[0:KPAD, :] = jnp.zeros((KPAD, 128), u32)

    def fwd_k(a):
        dv = dv_ref[...].astype(f32).reshape(1, D)
        for g in range(NG):
            prep_k(g, a)
            dvec = jnp.broadcast_to(dv[:, 128 * g:128 * (g + 1)], (RB, 128)) if a == 0 else None
            for b in range(128 // RB):
                fwd(rk, kh, g, a, b, dvec)

    for a in range(NCH):
        if a == 0:
            @pl.when(first_step())
            def _blkA0k():
                cp_s(0).wait()
                cp_mf.wait()
                fwd_k(0)

        @pl.when(first_step())
        def _blkA(a=a):
            if a > 0:
                cp_s(a).wait()
            cp_k(a).wait(); cp_v(a).wait()
            mask = zero_ref[...] != 0
            shk = shk_ref[...].astype(f32)
            dv = dv_ref[...].astype(f32).reshape(1, D)
            inj = None
            for g in range(NG):
                lanes = slice(128 * g, 128 * (g + 1))
                wts = [jnp.broadcast_to(shk[j:j + 1, lanes], (8, 128)) for j in range(4)]
                for t in range(8):
                    tok = prep_x(g, a, t, wts, mask, inj)
                    inj = delayed(tok, NRCP_P) if g > 0 or PCHAIN0 else None
                if a > 0:
                    prep_k(g, a)
                for b in range(128 // RB):
                    fwd(rx, xh, g, a, b, None)
                if a > 0:
                    for b in range(128 // RB):
                        fwd(rk, kh, g, a, b, None)

        @pl.when(first_step())
        def _blkB(c=a):
            if c == 1:
                cp_gi.wait()
            mask = zero_ref[...] != 0
            inj = None
            for g in range(NG):
                for j in range(16):
                    tok = cell(g, j, c, mask, inj)
                    n = 16 * g + j
                    nd = int((n + 1) * RCP_B[c]) - int(n * RCP_B[c])
                    inj = delayed(tok, nd) if c > 0 else None
            if c > 0:
                for g in range(NG):
                    for s2 in range(4):
                        inv(g, c - 1, s2)

    @pl.when(first_step())
    def _blkC():
        cp_wm(0).wait()
        cp_wm(1).wait()
        cp_q(0).wait()
        mod_cols(0, 5 * D)
        for g in range(NG):
            for s2 in range(4):
                inv(g, NCH - 1, s2)
        next_prologue(0, 1)

    for t in range(NFC):
        @pl.when(first_step())
        def _first_rows(t=t):
            for c_ in cp_w(t):
                c_.wait()
            if t == NFC - 1:
                cp_wm(2).wait()
                cp_q(1).wait()
                mod_cols(5 * D, D)
            for j in range(NSB):
                r = pl.ds(j * SB, SB)
                if t == 0:
                    if j == 0:
                        x1, h2 = xn[...], hn[...]
                    else:
                        x1, h2 = prologue(j * SB, PCH)
                    xs[r, :] = x1
                    hs[r, :] = h2
                    accs[r, :] = ffn_part(h2, FLO[0], FCS[0])
                elif t < NFC - 1:
                    accs[r, :] += ffn_part(hs[r, :], FLO[t], FCS[t])
                else:
                    gb = modb[0:1, 5 * D:6 * D]
                    ffn = accs[r, :] + ffn_part(hs[r, :], FLO[t], FCS[t])
                    obuf[r, :] = (xs[r, :] + gb * ffn).astype(bf16)
            if t == NFC - 1:
                next_prologue(BM, PCH)
                cp_o(0, BM).start()

    def _step(step, carry):
        gb = modb[0:1, 5 * D:6 * D]
        row0 = pl.multiple_of(BM + step * BM2, SB)
        for j in range(BM2 // SB):
            if j == 0:
                x1, h2 = xn[...], hn[...]
            else:
                x1, h2 = prologue(row0 + j * SB, PCH)
            ffn = ffn_part(h2, 0, F)
            obuf[pl.ds(row0 + j * SB, SB), :] = (x1 + gb * ffn).astype(bf16)
        nxt = jnp.minimum(row0 + BM2, S - SB)
        next_prologue(pl.multiple_of(nxt, SB), PCH)
        cp_o(row0, BM2).start()
        return carry

    lax.fori_loop(0, NSTEP2, _step, 0)
    cp_o(0, BM).wait()
    for i in range(NSTEP2):
        cp_o(BM + i * BM2, BM2).wait()


def _raw_view(x):
    return x.reshape(S // 8, 8, NG, 128).transpose(0, 2, 1, 3).reshape(NG * S, 128)


@jax.jit
def pallas_adaLN_cond__ssm_conv_h3__glu_gated_swiglu__prompt_kernel(
    A_q: jax.Array,
    A_k: jax.Array,
    A_v: jax.Array,
    A_shift_k: jax.Array,
    A_ssm_k: jax.Array,
    A_ssm_D: jax.Array,
    B_x: jax.Array,
    B_w1: jax.Array,
    B_w3: jax.Array,
    B_w2: jax.Array,
    c: jax.Array,
    w_mod: jax.Array,
):
    del B_x
    mf, gi = _dft_tables()
    any_spec = pl.BlockSpec(memory_space=pl.ANY)
    vmem_spec = pl.BlockSpec(memory_space=pltpu.VMEM)
    scratch = [
        pltpu.VMEM((KPAD + 5 * S // 2, 128), u32),
        pltpu.VMEM((5 * S // 2, 128), u32),
        pltpu.VMEM((D, S), bf16),
        pltpu.VMEM((NG, CH // 2, 128), u32),
        pltpu.VMEM((NG, 4, 64, 128), u32),
        pltpu.VMEM((NG, 4, 64, 128), u32),
        pltpu.VMEM((NG, NCH, 4, 2, PR, 128), f32),
        pltpu.VMEM((NG, NCH, 4, 2, PR, 128), f32),
        pltpu.VMEM((NG, 4, 2, PR, 128), f32),
        pltpu.VMEM((NG, 4, PR, 128), u32),
        pltpu.VMEM((NG, 4, PR, 128), u32),
        pltpu.VMEM((NG, S, 128), f32),
        pltpu.VMEM((S, D), bf16),
        pltpu.VMEM((D, F), bf16),
        pltpu.VMEM((D, F), bf16),
        pltpu.VMEM((F, D), bf16),
        pltpu.VMEM((D, 6 * D), bf16),
        pltpu.VMEM((8, 6 * D), f32),
        pltpu.VMEM((SB, D), bf16),
        pltpu.VMEM((SB, D), f32),
        pltpu.VMEM((BM, D), bf16),
        pltpu.VMEM((BM, D), f32),
        pltpu.VMEM((BM, D), f32),
        pltpu.VMEM((S, D), bf16),
        pltpu.VMEM((4, 128, 128), u32),
        pltpu.VMEM((4, 64, 256), u32),
        pltpu.SemaphoreType.DMA((8, 8)),
    ]
    return pl.pallas_call(
        _kernel,
        in_specs=[any_spec] * 10 + [vmem_spec] * 4 + [pl.BlockSpec(memory_space=pltpu.SMEM)],
        out_specs=any_spec,
        out_shape=jax.ShapeDtypeStruct((1, S, D), bf16),
        scratch_shapes=scratch,
        compiler_params=pltpu.CompilerParams(
            vmem_limit_bytes=100 * 1024 * 1024),
    )(A_q, _raw_view(A_k), _raw_view(A_v), A_ssm_k, B_w1, B_w3, B_w2, w_mod,
      jnp.asarray(mf), jnp.asarray(gi), A_shift_k.T, A_ssm_D, c,
      jnp.zeros((8, 128), jnp.uint32), jnp.zeros((32,), jnp.int32))
```

```python
import os as _os
import numpy as np
import jax
import jax.numpy as jnp
from jax import lax
import jax.experimental.pallas as pl
import jax.experimental.pallas.tpu as pltpu

f32 = jnp.float32
bf16 = jnp.bfloat16
u32 = jnp.uint32

S = 2048
D = 640
F = 1536
NG = D // 128
NCH = 4
CH = S // NCH
NDFT = 2 * CH
EPS = 1e-5

BM = 512
SB = 128
NSB = BM // SB
BM2 = int(_os.environ.get('BM2', 256))
NSTEP2 = (S - BM) // BM2
FCS = tuple(int(x) for x in _os.environ.get('FCS', '256,512,768').split(','))
NFC = len(FCS)
FLO = tuple(sum(FCS[:i]) for i in range(NFC))
KPAD = 40
RB = int(_os.environ.get('RB', 32))
PCH = 1
NRCP_P = int(_os.environ.get('NRCP_P', 3))
PR = 136
PCHAIN0 = False
OUT_SB = int(_os.environ.get('OUT_SB', 1))
WM0 = int(_os.environ.get('WM0', 1920))
NPRE = int(_os.environ.get('NPRE', 1))
ANCH_STEADY = int(_os.environ.get('ANCH_STEADY', 0))
MERGE = int(_os.environ.get('MERGE', 0))
RCP_B = tuple(float(x) for x in _os.environ.get('RCP_B', '-1,0.34,1.34,2.34').split(','))


def _cos_turns(x):
    fr = x - jnp.floor(x)
    w = 4.0 * jnp.minimum(fr, 1.0 - fr) - 1.0
    w2 = w * w
    acc = jnp.float32(3.598843e-06)
    for coef in (-1.6044118e-04, 4.6817541e-03, -7.9692626e-02, 6.4596410e-01, -1.5707963e+00):
        acc = acc * w2 + jnp.float32(coef)
    return acc * w


def _odd_freq(r):
    return jnp.where(r < 64, 4 * r + 1, 4 * (r - 64) + 3)


def _bc(v):
    return pltpu.bitcast(v, bf16)


def _lo(w):
    return pltpu.bitcast(w << 16, f32)


def _hi(w):
    return pltpu.bitcast(w & jnp.uint32(0xFFFF0000), f32)


def _pk2(a, b):
    return pltpu.bitcast(pltpu.pack_elementwise([a, b], packed_dtype=bf16), u32)


def _fft4(zr, zi, inv):
    ar, ai = zr[0] + zr[2], zi[0] + zi[2]
    br, bi = zr[0] - zr[2], zi[0] - zi[2]
    cr, ci = zr[1] + zr[3], zi[1] + zi[3]
    dr, di = zr[1] - zr[3], zi[1] - zi[3]
    if not inv:
        return [ar + cr, br + di, ar - cr, br - di], [ai + ci, bi - dr, ai - ci, bi + dr]
    return [ar + cr, br - di, ar - cr, br + di], [ai + ci, bi + dr, ai - ci, bi - dr]


def _ln(x):
    m = jnp.sum(x, axis=-1, keepdims=True) * (1.0 / D)
    xc = x - m
    v = jnp.sum(xc * xc, axis=-1, keepdims=True) * (1.0 / D)
    return xc * lax.rsqrt(v + EPS)


def _kernel(q_hbm, k_hbm, v_hbm, sk_hbm, w1_hbm, w3_hbm, w2_hbm, wm_hbm,
            shk_ref, dv_ref, c_ref, zero_ref, zs_ref,
            o_hbm,
            kraw, vraw, skbuf, ktbuf, rx, rk, xh, kh, zb, ub0, ub1, ybuf,
            qbuf, w1b, w3b, w2b, wmb, modb, hn, xn, hs, xs, accs, obuf, mf_ref, gi_ref, sems):
    ub = (ub0, ub1)

    def cp_k(a):
        return pltpu.make_async_copy(
            k_hbm.at[pl.ds(5 * CH * a, 5 * CH), :],
            kraw.bitcast(bf16).at[pl.ds(2 * KPAD + 5 * CH * a, 5 * CH), :], sems.at[0, a])

    def cp_v(a):
        return pltpu.make_async_copy(
            v_hbm.at[pl.ds(5 * CH * a, 5 * CH), :],
            vraw.bitcast(bf16).at[pl.ds(5 * CH * a, 5 * CH), :], sems.at[1, a])

    def cp_s(a):
        cols = pl.ds(CH * a, CH)
        return pltpu.make_async_copy(sk_hbm.at[:, cols], skbuf.at[:, cols], sems.at[2, a])

    def cp_wm(i):
        cols = [pl.ds(0, WM0), pl.ds(WM0, 5 * D - WM0), pl.ds(5 * D, D)][i]
        return pltpu.make_async_copy(wm_hbm.at[:, cols], wmb.at[:, cols], sems.at[3, i])

    def cp_q(i):
        rows = pl.ds(0, BM) if i == 0 else pl.ds(BM, S - BM)
        return pltpu.make_async_copy(q_hbm.at[0, rows, :], qbuf.at[rows, :], sems.at[3, 4 + i])

    def cp_w(t):
        cols = pl.ds(FLO[t], FCS[t])
        return [pltpu.make_async_copy(w1_hbm.at[:, cols], w1b.at[:, cols], sems.at[4, t]),
                pltpu.make_async_copy(w3_hbm.at[:, cols], w3b.at[:, cols], sems.at[5, t]),
                pltpu.make_async_copy(w2_hbm.at[cols, :], w2b.at[cols, :], sems.at[6, t])]

    def cp_o(row, n):
        rows = pl.ds(row, n)
        return pltpu.make_async_copy(obuf.at[rows, :], o_hbm.at[0, rows, :], sems.at[7, 0])

    def gen_forward_dft():
        i32 = jnp.int32
        wrow = lax.broadcasted_iota(i32, (128, 128), 0)
        n4 = (4 * lax.broadcasted_iota(i32, (128, 128), 1)).astype(f32)
        coef, quarter = [], []
        for h in range(2):
            rho = 2 * wrow + h
            rem = rho % (2 * RB)
            r = RB * (rho // (2 * RB)) + rem % RB
            coef.append(_odd_freq(r).astype(f32) * (0.5 / NDFT))
            quarter.append((rem // RB).astype(f32) * 0.25)
        for p in range(4):
            v = [_cos_turns(coef[h] * (n4 + float(p)) + quarter[h]) for h in range(2)]
            mf_ref[p] = _pk2(v[0], v[1])

    def gen_inverse_dft():
        i32 = jnp.int32
        wrow = lax.broadcasted_iota(i32, (64, 256), 0)
        col = lax.broadcasted_iota(i32, (64, 256), 1)
        coef = _odd_freq(col // 2).astype(f32) * (0.5 / NDFT)
        quarter = (col % 2).astype(f32) * 0.25
        for p in range(4):
            v = [_cos_turns(coef * (8 * wrow + (4 * h + p)).astype(f32) + quarter) for h in range(2)]
            gi_ref[p] = _pk2(v[0], v[1])

    def prep_x(g, a, t, wts, mask, inj):
        i0_ = 64 * a + 8 * t
        kb = KPAD + 20 * i0_ + 4 * g
        kl = [kraw[pl.ds(kb + w, 8, stride=20), :] for w in range(4)]
        km2 = kraw[pl.ds(kb - 18, 8, stride=20), :]
        km3 = kraw[pl.ds(kb - 17, 8, stride=20), :]
        e = [_hi(km2), _lo(km3), _hi(km3)]
        for w in range(4):
            e += [_lo(kl[w]), _hi(kl[w])]
        if inj is not None:
            e[3] = jnp.where(mask, inj, e[3])
        vb = 20 * i0_ + 4 * g
        kv = []
        for w in range(4):
            vw = vraw[pl.ds(vb + w, 8, stride=20), :]
            for h, vv in enumerate((_lo(vw), _hi(vw))):
                r = 3 + 2 * w + h
                ks = wts[0] * e[r] + wts[1] * e[r - 1] + wts[2] * e[r - 2] + wts[3] * e[r - 3]
                kv.append(ks * vv)
        tok = None
        for p in range(4):
            pk = _pk2(kv[p], kv[p + 4])
            rx[g, p, pl.ds(8 * t, 8), :] = pk
            tok = pk if tok is None else tok | pk
        return tok

    def prep_k(g, m):
        blk = skbuf[pl.ds(128 * g, 128), pl.ds(CH * m, CH)]
        ktbuf[g] = pltpu.bitcast(blk.T, u32)
        lo16 = jnp.uint32(0xFFFF)
        hi16 = jnp.uint32(0xFFFF0000)
        for t in range(8):
            w = [ktbuf[g, pl.ds(32 * t + e_, 8, stride=4), :] for e_ in range(4)]
            rows = pl.ds(8 * t, 8)
            rk[g, 0, rows, :] = (w[0] & lo16) | (w[2] << 16)
            rk[g, 1, rows, :] = (w[0] >> 16) | (w[2] & hi16)
            rk[g, 2, rows, :] = (w[1] & lo16) | (w[3] << 16)
            rk[g, 3, rows, :] = (w[1] >> 16) | (w[3] & hi16)

    def fwd(src, dst, g, a, b, dvec):
        z = [jnp.dot(_bc(mf_ref[p, pl.ds(RB * b, RB), :]), _bc(src[g, p]),
                     preferred_element_type=f32) for p in range(4)]
        xr, xi = _fft4([t[:RB] for t in z], [t[RB:] for t in z], False)
        for f2 in range(4):
            dst[g, a, f2, 0, pl.ds(RB * b, RB), :] = xr[f2] if dvec is None else xr[f2] + dvec
            dst[g, a, f2, 1, pl.ds(RB * b, RB), :] = xi[f2]

    def cell(g, j, c, mask, inj):
        rows = pl.ds(8 * j, 8)
        zr, zi = [], []
        for f2 in range(4):
            ar = ai = None
            for a in range(c + 1):
                m = c - a
                xr = xh[g, a, f2, 0, rows, :]
                xi = xh[g, a, f2, 1, rows, :]
                kr = kh[g, m, f2, 0, rows, :]
                ki = kh[g, m, f2, 1, rows, :]
                if inj is not None and f2 == 0 and a == 0:
                    kr = jnp.where(mask, inj, kr)
                tr = xr * kr - xi * ki
                ti = xr * ki + xi * kr
                ar = tr if ar is None else ar + tr
                ai = ti if ai is None else ai + ti
            zr.append(ar)
            zi.append(ai)
        yr, yi = zr, zi
        if c > 0:
            pr = [zb[g, f, 0, rows, :] for f in range(4)]
            pi = [zb[g, f, 1, rows, :] for f in range(4)]
            if j < 8:
                yr = [zr[f] - pi[f] for f in range(4)]
                yi = [zi[f] + pr[f] for f in range(4)]
            else:
                yr = [zr[f] + pi[f] for f in range(4)]
                yi = [zi[f] - pr[f] for f in range(4)]
        if c + 1 < NCH:
            for f in range(4):
                zb[g, f, 0, rows, :] = zr[f]
                zb[g, f, 1, rows, :] = zi[f]
        ur, ui = _fft4(yr, yi, True)
        tok = None
        for s2 in range(4):
            pk = _pk2(ur[s2], ui[s2])
            ub[c % 2][g, s2, rows, :] = pk
            tok = pk if tok is None else tok | pk
        return tok

    def inv(g, c, s2):
        y = jnp.dot(_bc(gi_ref[s2]), _bc(ub[c % 2][g, s2, 0:128, :]), preferred_element_type=f32)
        ybuf[g, pl.ds(CH * c + s2, 128, stride=4), :] = y

    def delayed(tok, n):
        t = pltpu.bitcast(tok, f32)
        for _ in range(n):
            t = pl.reciprocal(t, approx=True)
        return t

    def mod_cols(lo_, n):
        cc = c_ref[...].astype(f32)
        sc = (cc * jax.nn.sigmoid(cc)).astype(bf16)
        lhs = jnp.broadcast_to(sc, (8, D))
        modb[:, pl.ds(lo_, n)] = jnp.dot(lhs, wmb[:, pl.ds(lo_, n)], preferred_element_type=f32)

    _cnt = [0]

    def first_step():
        i = _cnt[0]
        _cnt[0] += 1
        return zs_ref[i] == 0

    def prologue(row, nchunk):
        sa = modb[0:1, 0 * D:1 * D]
        ca1 = 1.0 + modb[0:1, 1 * D:2 * D]
        ga = modb[0:1, 2 * D:3 * D] * (2.0 / NDFT)
        sb = modb[0:1, 3 * D:4 * D]
        cb1 = 1.0 + modb[0:1, 4 * D:5 * D]
        mask = zero_ref[...] != 0
        n = SB // nchunk
        x1s, h2s = [], []
        tok = None
        for i in range(nchunk):
            r = pl.ds(row + i * n, n)
            q = qbuf[r, :].astype(f32)
            if tok is not None:
                q00 = jnp.where(mask, tok, q[0:8, 0:128])
                top = jnp.concatenate([q00, q[0:8, 128:]], axis=1)
                q = jnp.concatenate([top, q[8:]], axis=0)
            y = jnp.concatenate([ybuf[g, r, :] for g in range(NG)], axis=1)
            h1 = _ln(q) * ca1 + sa
            x1 = q + ga * (h1 * y)
            h2f = _ln(x1) * cb1 + sb
            if i + 1 < nchunk:
                parts = [h2f[8 * a:8 * a + 8, 128 * g:128 * (g + 1)]
                         for a in range(n // 8) for g in range(NG)]
                while len(parts) > 1:
                    parts = [parts[k] + parts[k + 1] if k + 1 < len(parts) else parts[k]
                             for k in range(0, len(parts), 2)]
                tok = parts[0]
            x1s.append(x1)
            h2s.append(h2f.astype(bf16))
        return jnp.concatenate(x1s, axis=0), jnp.concatenate(h2s, axis=0)

    def token_of(h2):
        w = pltpu.bitcast(h2, u32)
        parts = [w[8 * i:8 * i + 8, 128 * g:128 * (g + 1)]
                 for i in range(w.shape[0] // 8) for g in range(NG)]
        while len(parts) > 1:
            parts = [parts[i] | parts[i + 1] if i + 1 < len(parts) else parts[i]
                     for i in range(0, len(parts), 2)]
        return parts[0]

    def anchored(h, tok):
        mask = zero_ref[...] != 0
        w = pltpu.bitcast(h, u32)
        w0 = jnp.where(mask, tok, w[0:8, 0:128])
        top = jnp.concatenate([w0, w[0:8, 128:]], axis=1)
        return pltpu.bitcast(jnp.concatenate([top, w[8:]], axis=0), bf16)

    def ffn_part(h2, lo_, n, tok=None):
        cols = pl.ds(lo_, n)
        gate = jnp.dot(h2, w1b[:, cols], preferred_element_type=f32)
        hu = h2 if tok is None else anchored(h2, tok)
        up = jnp.dot(hu, w3b[:, cols], preferred_element_type=f32)
        act = (gate * jax.nn.sigmoid(gate) * up).astype(bf16)
        return jnp.dot(act, w2b[cols, :], preferred_element_type=f32)

    def next_prologue(row, nchunk):
        x1, h2 = prologue(row, nchunk)
        xn[...] = x1
        hn[...] = h2
        return h2

    @pl.when(first_step())
    def _issue():
        for a in range(NCH):
            cp_s(a).start(); cp_k(a).start(); cp_v(a).start()
        cp_wm(0).start()
        cp_wm(1).start()
        cp_q(0).start()
        for t in range(NFC):
            if t == NFC - 1:
                cp_wm(2).start()
            for c_ in cp_w(t):
                c_.start()
        cp_q(1).start()
        kraw[0:KPAD, :] = jnp.zeros((KPAD, 128), u32)
        gen_forward_dft()

    def fwd_k(a):
        dv = dv_ref[...].astype(f32).reshape(1, D)
        for g in range(NG):
            prep_k(g, a)
            dvec = jnp.broadcast_to(dv[:, 128 * g:128 * (g + 1)], (RB, 128)) if a == 0 else None
            for b in range(128 // RB):
                fwd(rk, kh, g, a, b, dvec)

    def part_a(a):
        mask = zero_ref[...] != 0
        shk = shk_ref[...].astype(f32)
        inj = None
        for g in range(NG):
            lanes = slice(128 * g, 128 * (g + 1))
            wts = [jnp.broadcast_to(shk[j:j + 1, lanes], (8, 128)) for j in range(4)]
            for t in range(8):
                tok = prep_x(g, a, t, wts, mask, inj)
                inj = delayed(tok, NRCP_P) if g > 0 or PCHAIN0 else None
            if a > 0:
                prep_k(g, a)
            for b in range(128 // RB):
                fwd(rx, xh, g, a, b, None)
            if a > 0:
                for b in range(128 // RB):
                    fwd(rk, kh, g, a, b, None)

    def part_b(c):
        mask = zero_ref[...] != 0
        inj = None
        for g in range(NG):
            for j in range(16):
                tok = cell(g, j, c, mask, inj)
                n = 16 * g + j
                nd = int((n + 1) * RCP_B[c]) - int(n * RCP_B[c])
                inj = delayed(tok, nd) if RCP_B[c] >= 0 else None
        if c > 0:
            for g in range(NG):
                for s2 in range(4):
                    inv(g, c - 1, s2)

    @pl.when(first_step())
    def _blkA0k():
        cp_s(0).wait()
        fwd_k(0)

    @pl.when(first_step())
    def _blkA0x():
        cp_k(0).wait(); cp_v(0).wait()
        part_a(0)

    for a in range(1, NCH):
        if not MERGE:
            @pl.when(first_step())
            def _blkB(c=a - 1):
                part_b(c)
                if c == 0:
                    gen_inverse_dft()

        @pl.when(first_step())
        def _blkM(a=a):
            cp_s(a).wait(); cp_k(a).wait(); cp_v(a).wait()
            if MERGE:
                part_b(a - 1)
            part_a(a)

    @pl.when(first_step())
    def _blkB3():
        part_b(NCH - 1)

    @pl.when(first_step())
    def _blkC():
        cp_wm(0).wait()
        cp_wm(1).wait()
        cp_q(0).wait()
        mod_cols(0, 5 * D)
        for g in range(NG):
            for s2 in range(4):
                inv(g, NCH - 1, s2)
        for j in range(NPRE):
            x1, h2 = prologue(j * SB, 1)
            xs[pl.ds(j * SB, SB), :] = x1
            hs[pl.ds(j * SB, SB), :] = h2

    for t in range(NFC):
        @pl.when(first_step())
        def _first_rows(t=t):
            for c_ in cp_w(t):
                c_.wait()
            if t == NFC - 1:
                cp_wm(2).wait()
                cp_q(1).wait()
                mod_cols(5 * D, D)
            for j in range(NSB):
                r = pl.ds(j * SB, SB)
                if t == 0:
                    if j < NPRE:
                        h2 = hs[r, :]
                    else:
                        x1, h2 = prologue(j * SB, PCH)
                        xs[r, :] = x1
                        hs[r, :] = h2
                    accs[r, :] = ffn_part(h2, FLO[0], FCS[0])
                elif t < NFC - 1:
                    accs[r, :] += ffn_part(hs[r, :], FLO[t], FCS[t])
                else:
                    gb = modb[0:1, 5 * D:6 * D]
                    ffn = accs[r, :] + ffn_part(hs[r, :], FLO[t], FCS[t])
                    obuf[r, :] = (xs[r, :] + gb * ffn).astype(bf16)
            if t == NFC - 1:
                next_prologue(BM, PCH)
                cp_o(0, BM).start()

    def _step(step, carry):
        gb = modb[0:1, 5 * D:6 * D]
        row0 = pl.multiple_of(BM + step * BM2, SB)
        nsb = BM2 // SB
        cur = (xn[...], hn[...])
        for j in range(nsb):
            if j + 1 < nsb:
                nxt = prologue(row0 + (j + 1) * SB, PCH)
                h_next = nxt[1]
            else:
                nrow = jnp.minimum(row0 + BM2, S - SB)
                h_next = next_prologue(pl.multiple_of(nrow, SB), PCH)
            x1, h2 = cur
            tok = token_of(h_next) if ANCH_STEADY else None
            ffn = ffn_part(h2, 0, F, tok)
            obuf[pl.ds(row0 + j * SB, SB), :] = (x1 + gb * ffn).astype(bf16)
            if OUT_SB:
                cp_o(row0 + j * SB, SB).start()
            if j + 1 < nsb:
                cur = nxt
        if not OUT_SB:
            cp_o(row0, BM2).start()
        return carry

    lax.fori_loop(0, NSTEP2, _step, 0)
    cp_o(0, BM).wait()
    n_out = SB if OUT_SB else BM2
    for i in range((S - BM) // n_out):
        cp_o(BM + i * n_out, n_out).wait()


def _raw_view(x):
    return x.reshape(S // 8, 8, NG, 128).transpose(0, 2, 1, 3).reshape(NG * S, 128)


@jax.jit
def pallas_adaLN_cond__ssm_conv_h3__glu_gated_swiglu__prompt_kernel(
    A_q: jax.Array,
    A_k: jax.Array,
    A_v: jax.Array,
    A_shift_k: jax.Array,
    A_ssm_k: jax.Array,
    A_ssm_D: jax.Array,
    B_x: jax.Array,
    B_w1: jax.Array,
    B_w3: jax.Array,
    B_w2: jax.Array,
    c: jax.Array,
    w_mod: jax.Array,
):
    del B_x
    any_spec = pl.BlockSpec(memory_space=pl.ANY)
    vmem_spec = pl.BlockSpec(memory_space=pltpu.VMEM)
    scratch = [
        pltpu.VMEM((KPAD + 5 * S // 2, 128), u32),
        pltpu.VMEM((5 * S // 2, 128), u32),
        pltpu.VMEM((D, S), bf16),
        pltpu.VMEM((NG, CH // 2, 128), u32),
        pltpu.VMEM((NG, 4, 64, 128), u32),
        pltpu.VMEM((NG, 4, 64, 128), u32),
        pltpu.VMEM((NG, NCH, 4, 2, PR, 128), f32),
        pltpu.VMEM((NG, NCH, 4, 2, PR, 128), f32),
        pltpu.VMEM((NG, 4, 2, PR, 128), f32),
        pltpu.VMEM((NG, 4, PR, 128), u32),
        pltpu.VMEM((NG, 4, PR, 128), u32),
        pltpu.VMEM((NG, S, 128), f32),
        pltpu.VMEM((S, D), bf16),
        pltpu.VMEM((D, F), bf16),
        pltpu.VMEM((D, F), bf16),
        pltpu.VMEM((F, D), bf16),
        pltpu.VMEM((D, 6 * D), bf16),
        pltpu.VMEM((8, 6 * D), f32),
        pltpu.VMEM((SB, D), bf16),
        pltpu.VMEM((SB, D), f32),
        pltpu.VMEM((BM, D), bf16),
        pltpu.VMEM((BM, D), f32),
        pltpu.VMEM((BM, D), f32),
        pltpu.VMEM((S, D), bf16),
        pltpu.VMEM((4, 128, 128), u32),
        pltpu.VMEM((4, 64, 256), u32),
        pltpu.SemaphoreType.DMA((8, 8)),
    ]
    return pl.pallas_call(
        _kernel,
        in_specs=[any_spec] * 8 + [vmem_spec] * 4 + [pl.BlockSpec(memory_space=pltpu.SMEM)],
        out_specs=any_spec,
        out_shape=jax.ShapeDtypeStruct((1, S, D), bf16),
        scratch_shapes=scratch,
        compiler_params=pltpu.CompilerParams(
            vmem_limit_bytes=100 * 1024 * 1024),
    )(A_q, _raw_view(A_k), _raw_view(A_v), A_ssm_k, B_w1, B_w3, B_w2, w_mod,
      A_shift_k.T, A_ssm_D, c,
      jnp.zeros((8, 128), jnp.uint32), jnp.zeros((32,), jnp.int32))
```

```python
import os as _os
import numpy as np
import jax
import jax.numpy as jnp
from jax import lax
import jax.experimental.pallas as pl
import jax.experimental.pallas.tpu as pltpu

f32 = jnp.float32
bf16 = jnp.bfloat16
u32 = jnp.uint32

S = 2048
D = 640
F = 1536
NG = D // 128
NCH = 4
CH = S // NCH
NDFT = 2 * CH
EPS = 1e-5

BM = 512
SB = 128
NSB = BM // SB
BM2 = int(_os.environ.get('BM2', 256))
NSTEP2 = (S - BM) // BM2
FCS = tuple(int(x) for x in _os.environ.get('FCS', '512,512,512').split(','))
NFC = len(FCS)
FLO = tuple(sum(FCS[:i]) for i in range(NFC))
KPAD = 40
RB = int(_os.environ.get('RB', 32))
PCH_FS, PCH_NAT, PCH_NEXT = (int(x) for x in _os.environ.get('PCH', '2,8,8').split(','))
NRCP_P = int(_os.environ.get('NRCP_P', 3))
PR = 136
PCHAIN0 = False
OUT_SB = int(_os.environ.get('OUT_SB', 1))
WM0 = int(_os.environ.get('WM0', 1920))
NPRE = int(_os.environ.get('NPRE', 1))
ANCH_STEADY = int(_os.environ.get('ANCH_STEADY', 0))
MERGE = int(_os.environ.get('MERGE', 0))
RCP_B = tuple(float(x) for x in _os.environ.get('RCP_B', '-1,0.34,1.34,2.34').split(','))


def _cos_turns(x):
    fr = x - jnp.floor(x)
    w = 4.0 * jnp.minimum(fr, 1.0 - fr) - 1.0
    w2 = w * w
    acc = jnp.float32(3.598843e-06)
    for coef in (-1.6044118e-04, 4.6817541e-03, -7.9692626e-02, 6.4596410e-01, -1.5707963e+00):
        acc = acc * w2 + jnp.float32(coef)
    return acc * w


def _odd_freq(r):
    return jnp.where(r < 64, 4 * r + 1, 4 * (r - 64) + 3)


def _bc(v):
    return pltpu.bitcast(v, bf16)


def _lo(w):
    return pltpu.bitcast(w << 16, f32)


def _hi(w):
    return pltpu.bitcast(w & jnp.uint32(0xFFFF0000), f32)


def _pk2(a, b):
    return pltpu.bitcast(pltpu.pack_elementwise([a, b], packed_dtype=bf16), u32)


def _fft4(zr, zi, inv):
    ar, ai = zr[0] + zr[2], zi[0] + zi[2]
    br, bi = zr[0] - zr[2], zi[0] - zi[2]
    cr, ci = zr[1] + zr[3], zi[1] + zi[3]
    dr, di = zr[1] - zr[3], zi[1] - zi[3]
    if not inv:
        return [ar + cr, br + di, ar - cr, br - di], [ai + ci, bi - dr, ai - ci, bi + dr]
    return [ar + cr, br - di, ar - cr, br + di], [ai + ci, bi + dr, ai - ci, bi - dr]


def _ln(x):
    m = jnp.sum(x, axis=-1, keepdims=True) * (1.0 / D)
    xc = x - m
    v = jnp.sum(xc * xc, axis=-1, keepdims=True) * (1.0 / D)
    return xc * lax.rsqrt(v + EPS)


def _kernel(q_hbm, k_hbm, v_hbm, sk_hbm, w1_hbm, w3_hbm, w2_hbm, wm_hbm,
            shk_ref, dv_ref, c_ref, zero_ref, zs_ref,
            o_hbm,
            kraw, vraw, skbuf, ktbuf, rx, rk, xh, kh, zb, ub0, ub1, ybuf,
            qbuf, w1b, w3b, w2b, wmb, modb, hn, xn, hs, xs, accs, obuf, mf_ref, gi_ref, sems):
    ub = (ub0, ub1)

    def cp_k(a):
        return pltpu.make_async_copy(
            k_hbm.at[pl.ds(5 * CH * a, 5 * CH), :],
            kraw.bitcast(bf16).at[pl.ds(2 * KPAD + 5 * CH * a, 5 * CH), :], sems.at[0, a])

    def cp_v(a):
        return pltpu.make_async_copy(
            v_hbm.at[pl.ds(5 * CH * a, 5 * CH), :],
            vraw.bitcast(bf16).at[pl.ds(5 * CH * a, 5 * CH), :], sems.at[1, a])

    def cp_s(a):
        cols = pl.ds(CH * a, CH)
        return pltpu.make_async_copy(sk_hbm.at[:, cols], skbuf.at[:, cols], sems.at[2, a])

    def cp_wm(i):
        cols = [pl.ds(0, WM0), pl.ds(WM0, 5 * D - WM0), pl.ds(5 * D, D)][i]
        return pltpu.make_async_copy(wm_hbm.at[:, cols], wmb.at[:, cols], sems.at[3, i])

    def cp_q(i):
        rows = pl.ds(0, BM) if i == 0 else pl.ds(BM, S - BM)
        return pltpu.make_async_copy(q_hbm.at[0, rows, :], qbuf.at[rows, :], sems.at[3, 4 + i])

    def cp_w(t):
        cols = pl.ds(FLO[t], FCS[t])
        return [pltpu.make_async_copy(w1_hbm.at[:, cols], w1b.at[:, cols], sems.at[4, t]),
                pltpu.make_async_copy(w3_hbm.at[:, cols], w3b.at[:, cols], sems.at[5, t]),
                pltpu.make_async_copy(w2_hbm.at[cols, :], w2b.at[cols, :], sems.at[6, t])]

    def cp_o(row, n):
        rows = pl.ds(row, n)
        return pltpu.make_async_copy(obuf.at[rows, :], o_hbm.at[0, rows, :], sems.at[7, 0])

    def gen_forward_dft():
        i32 = jnp.int32
        wrow = lax.broadcasted_iota(i32, (128, 128), 0)
        n4 = (4 * lax.broadcasted_iota(i32, (128, 128), 1)).astype(f32)
        coef, quarter = [], []
        for h in range(2):
            rho = 2 * wrow + h
            rem = rho % (2 * RB)
            r = RB * (rho // (2 * RB)) + rem % RB
            coef.append(_odd_freq(r).astype(f32) * (0.5 / NDFT))
            quarter.append((rem // RB).astype(f32) * 0.25)
        for p in range(4):
            v = [_cos_turns(coef[h] * (n4 + float(p)) + quarter[h]) for h in range(2)]
            mf_ref[p] = _pk2(v[0], v[1])

    def gen_inverse_dft():
        i32 = jnp.int32
        wrow = lax.broadcasted_iota(i32, (64, 256), 0)
        col = lax.broadcasted_iota(i32, (64, 256), 1)
        coef = _odd_freq(col // 2).astype(f32) * (0.5 / NDFT)
        quarter = (col % 2).astype(f32) * 0.25
        for p in range(4):
            v = [_cos_turns(coef * (8 * wrow + (4 * h + p)).astype(f32) + quarter) for h in range(2)]
            gi_ref[p] = _pk2(v[0], v[1])

    def prep_x(g, a, t, wts, mask, inj):
        i0_ = 64 * a + 8 * t
        kb = KPAD + 20 * i0_ + 4 * g
        kl = [kraw[pl.ds(kb + w, 8, stride=20), :] for w in range(4)]
        km2 = kraw[pl.ds(kb - 18, 8, stride=20), :]
        km3 = kraw[pl.ds(kb - 17, 8, stride=20), :]
        e = [_hi(km2), _lo(km3), _hi(km3)]
        for w in range(4):
            e += [_lo(kl[w]), _hi(kl[w])]
        if inj is not None:
            e[3] = jnp.where(mask, inj, e[3])
        vb = 20 * i0_ + 4 * g
        kv = []
        for w in range(4):
            vw = vraw[pl.ds(vb + w, 8, stride=20), :]
            for h, vv in enumerate((_lo(vw), _hi(vw))):
                r = 3 + 2 * w + h
                ks = wts[0] * e[r] + wts[1] * e[r - 1] + wts[2] * e[r - 2] + wts[3] * e[r - 3]
                kv.append(ks * vv)
        tok = None
        for p in range(4):
            pk = _pk2(kv[p], kv[p + 4])
            rx[g, p, pl.ds(8 * t, 8), :] = pk
            tok = pk if tok is None else tok | pk
        return tok

    def prep_k(g, m):
        blk = skbuf[pl.ds(128 * g, 128), pl.ds(CH * m, CH)]
        ktbuf[g] = pltpu.bitcast(blk.T, u32)
        lo16 = jnp.uint32(0xFFFF)
        hi16 = jnp.uint32(0xFFFF0000)
        for t in range(8):
            w = [ktbuf[g, pl.ds(32 * t + e_, 8, stride=4), :] for e_ in range(4)]
            rows = pl.ds(8 * t, 8)
            rk[g, 0, rows, :] = (w[0] & lo16) | (w[2] << 16)
            rk[g, 1, rows, :] = (w[0] >> 16) | (w[2] & hi16)
            rk[g, 2, rows, :] = (w[1] & lo16) | (w[3] << 16)
            rk[g, 3, rows, :] = (w[1] >> 16) | (w[3] & hi16)

    def fwd(src, dst, g, a, b, dvec):
        z = [jnp.dot(_bc(mf_ref[p, pl.ds(RB * b, RB), :]), _bc(src[g, p]),
                     preferred_element_type=f32) for p in range(4)]
        xr, xi = _fft4([t[:RB] for t in z], [t[RB:] for t in z], False)
        for f2 in range(4):
            dst[g, a, f2, 0, pl.ds(RB * b, RB), :] = xr[f2] if dvec is None else xr[f2] + dvec
            dst[g, a, f2, 1, pl.ds(RB * b, RB), :] = xi[f2]

    def cell(g, j, c, mask, inj):
        rows = pl.ds(8 * j, 8)
        zr, zi = [], []
        for f2 in range(4):
            ar = ai = None
            for a in range(c + 1):
                m = c - a
                xr = xh[g, a, f2, 0, rows, :]
                xi = xh[g, a, f2, 1, rows, :]
                kr = kh[g, m, f2, 0, rows, :]
                ki = kh[g, m, f2, 1, rows, :]
                if inj is not None and f2 == 0 and a == 0:
                    kr = jnp.where(mask, inj, kr)
                tr = xr * kr - xi * ki
                ti = xr * ki + xi * kr
                ar = tr if ar is None else ar + tr
                ai = ti if ai is None else ai + ti
            zr.append(ar)
            zi.append(ai)
        yr, yi = zr, zi
        if c > 0:
            pr = [zb[g, f, 0, rows, :] for f in range(4)]
            pi = [zb[g, f, 1, rows, :] for f in range(4)]
            if j < 8:
                yr = [zr[f] - pi[f] for f in range(4)]
                yi = [zi[f] + pr[f] for f in range(4)]
            else:
                yr = [zr[f] + pi[f] for f in range(4)]
                yi = [zi[f] - pr[f] for f in range(4)]
        if c + 1 < NCH:
            for f in range(4):
                zb[g, f, 0, rows, :] = zr[f]
                zb[g, f, 1, rows, :] = zi[f]
        ur, ui = _fft4(yr, yi, True)
        tok = None
        for s2 in range(4):
            pk = _pk2(ur[s2], ui[s2])
            ub[c % 2][g, s2, rows, :] = pk
            tok = pk if tok is None else tok | pk
        return tok

    def inv(g, c, s2):
        y = jnp.dot(_bc(gi_ref[s2]), _bc(ub[c % 2][g, s2, 0:128, :]), preferred_element_type=f32)
        ybuf[g, pl.ds(CH * c + s2, 128, stride=4), :] = y

    def delayed(tok, n):
        t = pltpu.bitcast(tok, f32)
        for _ in range(n):
            t = pl.reciprocal(t, approx=True)
        return t

    def mod_cols(lo_, n):
        cc = c_ref[...].astype(f32)
        sc = (cc * jax.nn.sigmoid(cc)).astype(bf16)
        lhs = jnp.broadcast_to(sc, (8, D))
        modb[:, pl.ds(lo_, n)] = jnp.dot(lhs, wmb[:, pl.ds(lo_, n)], preferred_element_type=f32)

    _cnt = [0]

    def first_step():
        i = _cnt[0]
        _cnt[0] += 1
        return zs_ref[i] == 0

    def prologue(row, nchunk):
        sa = modb[0:1, 0 * D:1 * D]
        ca1 = 1.0 + modb[0:1, 1 * D:2 * D]
        ga = modb[0:1, 2 * D:3 * D] * (2.0 / NDFT)
        sb = modb[0:1, 3 * D:4 * D]
        cb1 = 1.0 + modb[0:1, 4 * D:5 * D]
        mask = zero_ref[...] != 0
        n = SB // nchunk
        x1s, h2s = [], []
        tok = None
        for i in range(nchunk):
            r = pl.ds(row + i * n, n)
            q = qbuf[r, :].astype(f32)
            if tok is not None:
                q00 = jnp.where(mask, tok, q[0:8, 0:128])
                top = jnp.concatenate([q00, q[0:8, 128:]], axis=1)
                q = jnp.concatenate([top, q[8:]], axis=0)
            y = jnp.concatenate([ybuf[g, r, :] for g in range(NG)], axis=1)
            h1 = _ln(q) * ca1 + sa
            x1 = q + ga * (h1 * y)
            h2f = _ln(x1) * cb1 + sb
            if i + 1 < nchunk:
                parts = [h2f[8 * a:8 * a + 8, 128 * g:128 * (g + 1)]
                         for a in range(n // 8) for g in range(NG)]
                while len(parts) > 1:
                    parts = [parts[k] + parts[k + 1] if k + 1 < len(parts) else parts[k]
                             for k in range(0, len(parts), 2)]
                tok = parts[0]
            x1s.append(x1)
            h2s.append(h2f.astype(bf16))
        return jnp.concatenate(x1s, axis=0), jnp.concatenate(h2s, axis=0)

    def token_of(h2):
        w = pltpu.bitcast(h2, u32)
        parts = [w[8 * i:8 * i + 8, 128 * g:128 * (g + 1)]
                 for i in range(w.shape[0] // 8) for g in range(NG)]
        while len(parts) > 1:
            parts = [parts[i] | parts[i + 1] if i + 1 < len(parts) else parts[i]
                     for i in range(0, len(parts), 2)]
        return parts[0]

    def anchored(h, tok):
        mask = zero_ref[...] != 0
        w = pltpu.bitcast(h, u32)
        w0 = jnp.where(mask, tok, w[0:8, 0:128])
        top = jnp.concatenate([w0, w[0:8, 128:]], axis=1)
        return pltpu.bitcast(jnp.concatenate([top, w[8:]], axis=0), bf16)

    def ffn_part(h2, lo_, n, tok=None):
        cols = pl.ds(lo_, n)
        gate = jnp.dot(h2, w1b[:, cols], preferred_element_type=f32)
        hu = h2 if tok is None else anchored(h2, tok)
        up = jnp.dot(hu, w3b[:, cols], preferred_element_type=f32)
        act = (gate * jax.nn.sigmoid(gate) * up).astype(bf16)
        return jnp.dot(act, w2b[cols, :], preferred_element_type=f32)

    def next_prologue(row, nchunk):
        x1, h2 = prologue(row, nchunk)
        xn[...] = x1
        hn[...] = h2
        return h2

    @pl.when(first_step())
    def _issue():
        for a in range(NCH):
            cp_s(a).start(); cp_k(a).start(); cp_v(a).start()
        cp_wm(0).start()
        cp_wm(1).start()
        cp_q(0).start()
        for t in range(NFC):
            if t == NFC - 1:
                cp_wm(2).start()
            for c_ in cp_w(t):
                c_.start()
        cp_q(1).start()
        kraw[0:KPAD, :] = jnp.zeros((KPAD, 128), u32)
        gen_forward_dft()

    def fwd_k(a):
        dv = dv_ref[...].astype(f32).reshape(1, D)
        for g in range(NG):
            prep_k(g, a)
            dvec = jnp.broadcast_to(dv[:, 128 * g:128 * (g + 1)], (RB, 128)) if a == 0 else None
            for b in range(128 // RB):
                fwd(rk, kh, g, a, b, dvec)

    def part_a(a):
        mask = zero_ref[...] != 0
        shk = shk_ref[...].astype(f32)
        inj = None
        for g in range(NG):
            lanes = slice(128 * g, 128 * (g + 1))
            wts = [jnp.broadcast_to(shk[j:j + 1, lanes], (8, 128)) for j in range(4)]
            for t in range(8):
                tok = prep_x(g, a, t, wts, mask, inj)
                inj = delayed(tok, NRCP_P) if g > 0 or PCHAIN0 else None
            if a > 0:
                prep_k(g, a)
            for b in range(128 // RB):
                fwd(rx, xh, g, a, b, None)
            if a > 0:
                for b in range(128 // RB):
                    fwd(rk, kh, g, a, b, None)

    def part_b(c):
        mask = zero_ref[...] != 0
        inj = None
        for g in range(NG):
            for j in range(16):
                tok = cell(g, j, c, mask, inj)
                n = 16 * g + j
                nd = int((n + 1) * RCP_B[c]) - int(n * RCP_B[c])
                inj = delayed(tok, nd) if RCP_B[c] >= 0 else None
        if c > 0:
            for g in range(NG):
                for s2 in range(4):
                    inv(g, c - 1, s2)

    @pl.when(first_step())
    def _blkA0k():
        cp_s(0).wait()
        fwd_k(0)

    @pl.when(first_step())
    def _blkA0x():
        cp_k(0).wait(); cp_v(0).wait()
        part_a(0)

    for a in range(1, NCH):
        if not MERGE:
            @pl.when(first_step())
            def _blkB(c=a - 1):
                part_b(c)
                if c == 0:
                    gen_inverse_dft()

        @pl.when(first_step())
        def _blkM(a=a):
            cp_s(a).wait(); cp_k(a).wait(); cp_v(a).wait()
            if MERGE:
                part_b(a - 1)
            part_a(a)

    @pl.when(first_step())
    def _blkB3():
        part_b(NCH - 1)

    @pl.when(first_step())
    def _blkC():
        cp_wm(0).wait()
        cp_wm(1).wait()
        cp_q(0).wait()
        mod_cols(0, 5 * D)
        for g in range(NG):
            for s2 in range(4):
                inv(g, NCH - 1, s2)
        for j in range(NPRE):
            x1, h2 = prologue(j * SB, 1)
            xs[pl.ds(j * SB, SB), :] = x1
            hs[pl.ds(j * SB, SB), :] = h2

    for t in range(NFC):
        @pl.when(first_step())
        def _first_rows(t=t):
            for c_ in cp_w(t):
                c_.wait()
            if t == NFC - 1:
                cp_wm(2).wait()
                cp_q(1).wait()
                mod_cols(5 * D, D)
            for j in range(NSB):
                r = pl.ds(j * SB, SB)
                if t == 0:
                    if j < NPRE:
                        h2 = hs[r, :]
                    else:
                        x1, h2 = prologue(j * SB, PCH_FS)
                        xs[r, :] = x1
                        hs[r, :] = h2
                    accs[r, :] = ffn_part(h2, FLO[0], FCS[0])
                elif t < NFC - 1:
                    accs[r, :] += ffn_part(hs[r, :], FLO[t], FCS[t])
                else:
                    gb = modb[0:1, 5 * D:6 * D]
                    ffn = accs[r, :] + ffn_part(hs[r, :], FLO[t], FCS[t])
                    obuf[r, :] = (xs[r, :] + gb * ffn).astype(bf16)
            if t == NFC - 1:
                next_prologue(BM, PCH_NEXT)
                cp_o(0, BM).start()

    def _step(step, carry):
        gb = modb[0:1, 5 * D:6 * D]
        row0 = pl.multiple_of(BM + step * BM2, SB)
        nsb = BM2 // SB
        cur = (xn[...], hn[...])
        for j in range(nsb):
            if j + 1 < nsb:
                nxt = prologue(row0 + (j + 1) * SB, PCH_NAT)
                h_next = nxt[1]
            else:
                nrow = jnp.minimum(row0 + BM2, S - SB)
                h_next = next_prologue(pl.multiple_of(nrow, SB), PCH_NEXT)
            x1, h2 = cur
            tok = token_of(h_next) if ANCH_STEADY else None
            ffn = ffn_part(h2, 0, F, tok)
            obuf[pl.ds(row0 + j * SB, SB), :] = (x1 + gb * ffn).astype(bf16)
            if OUT_SB:
                cp_o(row0 + j * SB, SB).start()
            if j + 1 < nsb:
                cur = nxt
        if not OUT_SB:
            cp_o(row0, BM2).start()
        return carry

    lax.fori_loop(0, NSTEP2, _step, 0)
    cp_o(0, BM).wait()
    n_out = SB if OUT_SB else BM2
    for i in range((S - BM) // n_out):
        cp_o(BM + i * n_out, n_out).wait()


def _raw_view(x):
    return x.reshape(S // 8, 8, NG, 128).transpose(0, 2, 1, 3).reshape(NG * S, 128)


@jax.jit
def pallas_adaLN_cond__ssm_conv_h3__glu_gated_swiglu__prompt_kernel(
    A_q: jax.Array,
    A_k: jax.Array,
    A_v: jax.Array,
    A_shift_k: jax.Array,
    A_ssm_k: jax.Array,
    A_ssm_D: jax.Array,
    B_x: jax.Array,
    B_w1: jax.Array,
    B_w3: jax.Array,
    B_w2: jax.Array,
    c: jax.Array,
    w_mod: jax.Array,
):
    del B_x
    any_spec = pl.BlockSpec(memory_space=pl.ANY)
    vmem_spec = pl.BlockSpec(memory_space=pltpu.VMEM)
    scratch = [
        pltpu.VMEM((KPAD + 5 * S // 2, 128), u32),
        pltpu.VMEM((5 * S // 2, 128), u32),
        pltpu.VMEM((D, S), bf16),
        pltpu.VMEM((NG, CH // 2, 128), u32),
        pltpu.VMEM((NG, 4, 64, 128), u32),
        pltpu.VMEM((NG, 4, 64, 128), u32),
        pltpu.VMEM((NG, NCH, 4, 2, PR, 128), f32),
        pltpu.VMEM((NG, NCH, 4, 2, PR, 128), f32),
        pltpu.VMEM((NG, 4, 2, PR, 128), f32),
        pltpu.VMEM((NG, 4, PR, 128), u32),
        pltpu.VMEM((NG, 4, PR, 128), u32),
        pltpu.VMEM((NG, S, 128), f32),
        pltpu.VMEM((S, D), bf16),
        pltpu.VMEM((D, F), bf16),
        pltpu.VMEM((D, F), bf16),
        pltpu.VMEM((F, D), bf16),
        pltpu.VMEM((D, 6 * D), bf16),
        pltpu.VMEM((8, 6 * D), f32),
        pltpu.VMEM((SB, D), bf16),
        pltpu.VMEM((SB, D), f32),
        pltpu.VMEM((BM, D), bf16),
        pltpu.VMEM((BM, D), f32),
        pltpu.VMEM((BM, D), f32),
        pltpu.VMEM((S, D), bf16),
        pltpu.VMEM((4, 128, 128), u32),
        pltpu.VMEM((4, 64, 256), u32),
        pltpu.SemaphoreType.DMA((8, 8)),
    ]
    return pl.pallas_call(
        _kernel,
        in_specs=[any_spec] * 8 + [vmem_spec] * 4 + [pl.BlockSpec(memory_space=pltpu.SMEM)],
        out_specs=any_spec,
        out_shape=jax.ShapeDtypeStruct((1, S, D), bf16),
        scratch_shapes=scratch,
        compiler_params=pltpu.CompilerParams(
            vmem_limit_bytes=100 * 1024 * 1024),
    )(A_q, _raw_view(A_k), _raw_view(A_v), A_ssm_k, B_w1, B_w3, B_w2, w_mod,
      A_shift_k.T, A_ssm_D, c,
      jnp.zeros((8, 128), jnp.uint32), jnp.zeros((32,), jnp.int32))
```

```python
import os as _os
import numpy as np
import jax
import jax.numpy as jnp
from jax import lax
import jax.experimental.pallas as pl
import jax.experimental.pallas.tpu as pltpu

f32 = jnp.float32
bf16 = jnp.bfloat16
u32 = jnp.uint32

S = 2048
D = 640
F = 1536
NG = D // 128
NCH = 4
CH = S // NCH
NDFT = 2 * CH
EPS = 1e-5

BM = 512
SB = 128
NSB = BM // SB
BM2 = int(_os.environ.get('BM2', 256))
NSTEP2 = (S - BM) // BM2
FCS = tuple(int(x) for x in _os.environ.get('FCS', '512,512,512').split(','))
NFC = len(FCS)
FLO = tuple(sum(FCS[:i]) for i in range(NFC))
KPAD = 40
RB = int(_os.environ.get('RB', 32))
PCH_FS, PCH_NAT, PCH_NEXT = (int(x) for x in _os.environ.get('PCH', '2,8,8').split(','))
NRCP_P = int(_os.environ.get('NRCP_P', 3))
PR = 136
PCHAIN0 = False
OUT_SB = int(_os.environ.get('OUT_SB', 1))
WM0 = int(_os.environ.get('WM0', 1920))
NPRE = int(_os.environ.get('NPRE', 1))
ANCH_STEADY = int(_os.environ.get('ANCH_STEADY', 0))
MERGE = int(_os.environ.get('MERGE', 0))
RCP_B = tuple(float(x) for x in _os.environ.get('RCP_B', '-1,0.34,1.34,2.34').split(','))


def _cos_turns(x):
    fr = x - jnp.floor(x)
    w = 4.0 * jnp.minimum(fr, 1.0 - fr) - 1.0
    w2 = w * w
    acc = jnp.float32(3.598843e-06)
    for coef in (-1.6044118e-04, 4.6817541e-03, -7.9692626e-02, 6.4596410e-01, -1.5707963e+00):
        acc = acc * w2 + jnp.float32(coef)
    return acc * w


def _odd_freq(r):
    return jnp.where(r < 64, 4 * r + 1, 4 * (r - 64) + 3)


def _bc(v):
    return pltpu.bitcast(v, bf16)


def _u32(v):
    return pltpu.bitcast(v, u32)


def _half(row, n):
    if isinstance(row, int):
        return pl.ds(row // 2, n // 2)
    return pl.ds(pl.multiple_of(row // 2, 8), n // 2)


def _lo(w):
    return pltpu.bitcast(w << 16, f32)


def _hi(w):
    return pltpu.bitcast(w & jnp.uint32(0xFFFF0000), f32)


def _pk2(a, b):
    return pltpu.bitcast(pltpu.pack_elementwise([a, b], packed_dtype=bf16), u32)


def _fft4(zr, zi, inv):
    ar, ai = zr[0] + zr[2], zi[0] + zi[2]
    br, bi = zr[0] - zr[2], zi[0] - zi[2]
    cr, ci = zr[1] + zr[3], zi[1] + zi[3]
    dr, di = zr[1] - zr[3], zi[1] - zi[3]
    if not inv:
        return [ar + cr, br + di, ar - cr, br - di], [ai + ci, bi - dr, ai - ci, bi + dr]
    return [ar + cr, br - di, ar - cr, br + di], [ai + ci, bi + dr, ai - ci, bi - dr]


def _ln(x):
    m = jnp.sum(x, axis=-1, keepdims=True) * (1.0 / D)
    xc = x - m
    v = jnp.sum(xc * xc, axis=-1, keepdims=True) * (1.0 / D)
    return xc * lax.rsqrt(v + EPS)


def _kernel(q_hbm, k_hbm, v_hbm, sk_hbm, w1_hbm, w3_hbm, w2_hbm, wm_hbm,
            shk_ref, dv_ref, c_ref, zero_ref, zs_ref,
            o_hbm,
            kraw, vraw, skbuf, ktbuf, rx, rk, xh, kh, zb, ub0, ub1, ybuf,
            qbuf, w1b, w3b, w2b, wmb, modb, hn, xn, hs, xs, accs, obuf, mf_ref, gi_ref, sems):
    ub = (ub0, ub1)

    def cp_k(a):
        return pltpu.make_async_copy(
            k_hbm.at[pl.ds(5 * CH * a, 5 * CH), :],
            kraw.bitcast(bf16).at[pl.ds(2 * KPAD + 5 * CH * a, 5 * CH), :], sems.at[0, a])

    def cp_v(a):
        return pltpu.make_async_copy(
            v_hbm.at[pl.ds(5 * CH * a, 5 * CH), :],
            vraw.bitcast(bf16).at[pl.ds(5 * CH * a, 5 * CH), :], sems.at[1, a])

    def cp_s(a):
        cols = pl.ds(CH * a, CH)
        return pltpu.make_async_copy(sk_hbm.at[:, cols], skbuf.bitcast(bf16).at[:, cols], sems.at[2, a])

    def cp_wm(i):
        cols = [pl.ds(0, WM0), pl.ds(WM0, 5 * D - WM0), pl.ds(5 * D, D)][i]
        return pltpu.make_async_copy(wm_hbm.at[:, cols], wmb.bitcast(bf16).at[:, cols], sems.at[3, i])

    def cp_q(i):
        rows = pl.ds(0, BM) if i == 0 else pl.ds(BM, S - BM)
        return pltpu.make_async_copy(q_hbm.at[0, rows, :], qbuf.bitcast(bf16).at[rows, :], sems.at[3, 4 + i])

    def cp_w(t):
        cols = pl.ds(FLO[t], FCS[t])
        return [pltpu.make_async_copy(w1_hbm.at[:, cols], w1b.bitcast(bf16).at[:, cols], sems.at[4, t]),
                pltpu.make_async_copy(w3_hbm.at[:, cols], w3b.bitcast(bf16).at[:, cols], sems.at[5, t]),
                pltpu.make_async_copy(w2_hbm.at[cols, :], w2b.bitcast(bf16).at[cols, :], sems.at[6, t])]

    def cp_o(row, n):
        rows = pl.ds(row, n)
        return pltpu.make_async_copy(obuf.at[rows, :], o_hbm.at[0, rows, :], sems.at[7, 0])

    def gen_forward_dft():
        i32 = jnp.int32
        wrow = lax.broadcasted_iota(i32, (128, 128), 0)
        n4 = (4 * lax.broadcasted_iota(i32, (128, 128), 1)).astype(f32)
        coef, quarter = [], []
        for h in range(2):
            rho = 2 * wrow + h
            rem = rho % (2 * RB)
            r = RB * (rho // (2 * RB)) + rem % RB
            coef.append(_odd_freq(r).astype(f32) * (0.5 / NDFT))
            quarter.append((rem // RB).astype(f32) * 0.25)
        for p in range(4):
            v = [_cos_turns(coef[h] * (n4 + float(p)) + quarter[h]) for h in range(2)]
            mf_ref[p] = _pk2(v[0], v[1])

    def gen_inverse_dft():
        i32 = jnp.int32
        wrow = lax.broadcasted_iota(i32, (64, 256), 0)
        col = lax.broadcasted_iota(i32, (64, 256), 1)
        coef = _odd_freq(col // 2).astype(f32) * (0.5 / NDFT)
        quarter = (col % 2).astype(f32) * 0.25
        for p in range(4):
            v = [_cos_turns(coef * (8 * wrow + (4 * h + p)).astype(f32) + quarter) for h in range(2)]
            gi_ref[p] = _pk2(v[0], v[1])

    def prep_x(g, a, t, wts, mask, inj):
        i0_ = 64 * a + 8 * t
        kb = KPAD + 20 * i0_ + 4 * g
        kl = [kraw[pl.ds(kb + w, 8, stride=20), :] for w in range(4)]
        km2 = kraw[pl.ds(kb - 18, 8, stride=20), :]
        km3 = kraw[pl.ds(kb - 17, 8, stride=20), :]
        e = [_hi(km2), _lo(km3), _hi(km3)]
        for w in range(4):
            e += [_lo(kl[w]), _hi(kl[w])]
        if inj is not None:
            e[3] = jnp.where(mask, inj, e[3])
        vb = 20 * i0_ + 4 * g
        kv = []
        for w in range(4):
            vw = vraw[pl.ds(vb + w, 8, stride=20), :]
            for h, vv in enumerate((_lo(vw), _hi(vw))):
                r = 3 + 2 * w + h
                ks = wts[0] * e[r] + wts[1] * e[r - 1] + wts[2] * e[r - 2] + wts[3] * e[r - 3]
                kv.append(ks * vv)
        tok = None
        for p in range(4):
            pk = _pk2(kv[p], kv[p + 4])
            rx[g, p, pl.ds(8 * t, 8), :] = pk
            tok = pk if tok is None else tok | pk
        return tok

    def prep_k(g, m):
        blk = _bc(skbuf[pl.ds(64 * g, 64), pl.ds(CH * m, CH)])
        ktbuf[g, 0:CH // 2, :] = pltpu.bitcast(blk.T, u32)
        lo16 = jnp.uint32(0xFFFF)
        hi16 = jnp.uint32(0xFFFF0000)
        for t in range(8):
            w = [ktbuf[g, pl.ds(32 * t + e_, 8, stride=4), :] for e_ in range(4)]
            rows = pl.ds(8 * t, 8)
            rk[g, 0, rows, :] = (w[0] & lo16) | (w[2] << 16)
            rk[g, 1, rows, :] = (w[0] >> 16) | (w[2] & hi16)
            rk[g, 2, rows, :] = (w[1] & lo16) | (w[3] << 16)
            rk[g, 3, rows, :] = (w[1] >> 16) | (w[3] & hi16)

    def fwd(src, dst, g, a, b, dvec):
        z = [jnp.dot(_bc(mf_ref[p, pl.ds(RB * b, RB), :]), _bc(src[g, p]),
                     preferred_element_type=f32) for p in range(4)]
        xr, xi = _fft4([t[:RB] for t in z], [t[RB:] for t in z], False)
        for f2 in range(4):
            dst[g, a, f2, 0, pl.ds(RB * b, RB), :] = xr[f2] if dvec is None else xr[f2] + dvec
            dst[g, a, f2, 1, pl.ds(RB * b, RB), :] = xi[f2]

    def cell(g, j, c, mask, inj):
        rows = pl.ds(8 * j, 8)
        zr, zi = [], []
        for f2 in range(4):
            ar = ai = None
            for a in range(c + 1):
                m = c - a
                xr = xh[g, a, f2, 0, rows, :]
                xi = xh[g, a, f2, 1, rows, :]
                kr = kh[g, m, f2, 0, rows, :]
                ki = kh[g, m, f2, 1, rows, :]
                if inj is not None and f2 == 0 and a == 0:
                    kr = jnp.where(mask, inj, kr)
                tr = xr * kr - xi * ki
                ti = xr * ki + xi * kr
                ar = tr if ar is None else ar + tr
                ai = ti if ai is None else ai + ti
            zr.append(ar)
            zi.append(ai)
        yr, yi = zr, zi
        if c > 0:
            pr = [zb[g, f, 0, rows, :] for f in range(4)]
            pi = [zb[g, f, 1, rows, :] for f in range(4)]
            if j < 8:
                yr = [zr[f] - pi[f] for f in range(4)]
                yi = [zi[f] + pr[f] for f in range(4)]
            else:
                yr = [zr[f] + pi[f] for f in range(4)]
                yi = [zi[f] - pr[f] for f in range(4)]
        if c + 1 < NCH:
            for f in range(4):
                zb[g, f, 0, rows, :] = zr[f]
                zb[g, f, 1, rows, :] = zi[f]
        ur, ui = _fft4(yr, yi, True)
        tok = None
        for s2 in range(4):
            pk = _pk2(ur[s2], ui[s2])
            ub[c % 2][g, s2, rows, :] = pk
            tok = pk if tok is None else tok | pk
        return tok

    def inv(g, c, s2):
        y = jnp.dot(_bc(gi_ref[s2]), _bc(ub[c % 2][g, s2, 0:128, :]), preferred_element_type=f32)
        ybuf[g, pl.ds(CH * c + s2, 128, stride=4), :] = y

    def delayed(tok, n):
        t = pltpu.bitcast(tok, f32)
        for _ in range(n):
            t = pl.reciprocal(t, approx=True)
        return t

    def mod_cols(lo_, n):
        cc = c_ref[...].astype(f32)
        sc = (cc * jax.nn.sigmoid(cc)).astype(bf16)
        lhs = jnp.broadcast_to(sc, (8, D))
        modb[:, pl.ds(lo_, n)] = jnp.dot(lhs, _bc(wmb[:, pl.ds(lo_, n)]), preferred_element_type=f32)

    _cnt = [0]

    def first_step():
        i = _cnt[0]
        _cnt[0] += 1
        return zs_ref[i] == 0

    def prologue(row, nchunk):
        sa = modb[0:1, 0 * D:1 * D]
        ca1 = 1.0 + modb[0:1, 1 * D:2 * D]
        ga = modb[0:1, 2 * D:3 * D] * (2.0 / NDFT)
        sb = modb[0:1, 3 * D:4 * D]
        cb1 = 1.0 + modb[0:1, 4 * D:5 * D]
        mask = zero_ref[...] != 0
        n = SB // nchunk
        x1s, h2s = [], []
        tok = None
        for i in range(nchunk):
            r = pl.ds(row + i * n, n)
            q = _bc(qbuf[_half(row + i * n, n), :]).astype(f32)
            if tok is not None:
                q00 = jnp.where(mask, tok, q[0:8, 0:128])
                top = jnp.concatenate([q00, q[0:8, 128:]], axis=1)
                q = jnp.concatenate([top, q[8:]], axis=0)
            y = jnp.concatenate([ybuf[g, r, :] for g in range(NG)], axis=1)
            h1 = _ln(q) * ca1 + sa
            x1 = q + ga * (h1 * y)
            h2f = _ln(x1) * cb1 + sb
            if i + 1 < nchunk:
                parts = [h2f[8 * a:8 * a + 8, 128 * g:128 * (g + 1)]
                         for a in range(n // 8) for g in range(NG)]
                while len(parts) > 1:
                    parts = [parts[k] + parts[k + 1] if k + 1 < len(parts) else parts[k]
                             for k in range(0, len(parts), 2)]
                tok = parts[0]
            x1s.append(x1)
            h2s.append(h2f.astype(bf16))
        return jnp.concatenate(x1s, axis=0), jnp.concatenate(h2s, axis=0)

    def token_of(h2):
        w = pltpu.bitcast(h2, u32)
        parts = [w[8 * i:8 * i + 8, 128 * g:128 * (g + 1)]
                 for i in range(w.shape[0] // 8) for g in range(NG)]
        while len(parts) > 1:
            parts = [parts[i] | parts[i + 1] if i + 1 < len(parts) else parts[i]
                     for i in range(0, len(parts), 2)]
        return parts[0]

    def anchored(h, tok):
        mask = zero_ref[...] != 0
        w = pltpu.bitcast(h, u32)
        w0 = jnp.where(mask, tok, w[0:8, 0:128])
        top = jnp.concatenate([w0, w[0:8, 128:]], axis=1)
        return pltpu.bitcast(jnp.concatenate([top, w[8:]], axis=0), bf16)

    def ffn_part(h2, lo_, n, tok=None):
        cols = pl.ds(lo_, n)
        gate = jnp.dot(h2, _bc(w1b[:, cols]), preferred_element_type=f32)
        hu = h2 if tok is None else anchored(h2, tok)
        up = jnp.dot(hu, _bc(w3b[:, cols]), preferred_element_type=f32)
        act = (gate * jax.nn.sigmoid(gate) * up).astype(bf16)
        return jnp.dot(act, _bc(w2b[_half(lo_, n), :]), preferred_element_type=f32)

    def next_prologue(row, nchunk):
        x1, h2 = prologue(row, nchunk)
        xn[...] = x1
        hn[...] = h2
        return h2

    @pl.when(first_step())
    def _issue():
        for a in range(NCH):
            cp_s(a).start(); cp_k(a).start(); cp_v(a).start()
        cp_wm(0).start()
        cp_wm(1).start()
        cp_q(0).start()
        for t in range(NFC):
            if t == NFC - 1:
                cp_wm(2).start()
            for c_ in cp_w(t):
                c_.start()
        cp_q(1).start()
        kraw[0:KPAD, :] = jnp.zeros((KPAD, 128), u32)
        gen_forward_dft()

    def fwd_k(a):
        dv = dv_ref[...].astype(f32).reshape(1, D)
        for g in range(NG):
            prep_k(g, a)
            dvec = jnp.broadcast_to(dv[:, 128 * g:128 * (g + 1)], (RB, 128)) if a == 0 else None
            for b in range(128 // RB):
                fwd(rk, kh, g, a, b, dvec)

    def part_a(a):
        mask = zero_ref[...] != 0
        shk = shk_ref[...].astype(f32)
        inj = None
        for g in range(NG):
            lanes = slice(128 * g, 128 * (g + 1))
            wts = [jnp.broadcast_to(shk[j:j + 1, lanes], (8, 128)) for j in range(4)]
            for t in range(8):
                tok = prep_x(g, a, t, wts, mask, inj)
                inj = delayed(tok, NRCP_P) if g > 0 or PCHAIN0 else None
            if a > 0:
                prep_k(g, a)
            for b in range(128 // RB):
                fwd(rx, xh, g, a, b, None)
            if a > 0:
                for b in range(128 // RB):
                    fwd(rk, kh, g, a, b, None)

    def part_b(c):
        mask = zero_ref[...] != 0
        inj = None
        for g in range(NG):
            for j in range(16):
                tok = cell(g, j, c, mask, inj)
                n = 16 * g + j
                nd = int((n + 1) * RCP_B[c]) - int(n * RCP_B[c])
                inj = delayed(tok, nd) if RCP_B[c] >= 0 else None
        if c > 0:
            for g in range(NG):
                for s2 in range(4):
                    inv(g, c - 1, s2)

    @pl.when(first_step())
    def _blkA0k():
        cp_s(0).wait()
        fwd_k(0)

    @pl.when(first_step())
    def _blkA0x():
        cp_k(0).wait(); cp_v(0).wait()
        part_a(0)

    for a in range(1, NCH):
        if not MERGE:
            @pl.when(first_step())
            def _blkB(c=a - 1):
                part_b(c)
                if c == 0:
                    gen_inverse_dft()

        @pl.when(first_step())
        def _blkM(a=a):
            cp_s(a).wait(); cp_k(a).wait(); cp_v(a).wait()
            if MERGE:
                part_b(a - 1)
            part_a(a)

    @pl.when(first_step())
    def _blkB3():
        cp_wm(0).wait()
        part_b(NCH - 1)
        mod_cols(0, WM0)

    @pl.when(first_step())
    def _blkC():
        cp_wm(1).wait()
        cp_q(0).wait()
        mod_cols(WM0, 5 * D - WM0)
        for g in range(NG):
            for s2 in range(4):
                inv(g, NCH - 1, s2)
        for j in range(NPRE):
            x1, h2 = prologue(j * SB, 1)
            xs[pl.ds(j * SB, SB), :] = x1
            hs[pl.ds(j * SB, SB), :] = h2

    for t in range(NFC):
        @pl.when(first_step())
        def _first_rows(t=t):
            for c_ in cp_w(t):
                c_.wait()
            if t == NFC - 1:
                cp_wm(2).wait()
                cp_q(1).wait()
                mod_cols(5 * D, D)
            for j in range(NSB):
                r = pl.ds(j * SB, SB)
                if t == 0:
                    if j < NPRE:
                        h2 = hs[r, :]
                    else:
                        x1, h2 = prologue(j * SB, PCH_FS)
                        xs[r, :] = x1
                        hs[r, :] = h2
                    accs[r, :] = ffn_part(h2, FLO[0], FCS[0])
                elif t < NFC - 1:
                    accs[r, :] += ffn_part(hs[r, :], FLO[t], FCS[t])
                else:
                    gb = modb[0:1, 5 * D:6 * D]
                    ffn = accs[r, :] + ffn_part(hs[r, :], FLO[t], FCS[t])
                    obuf[r, :] = (xs[r, :] + gb * ffn).astype(bf16)
            if t == NFC - 1:
                next_prologue(BM, PCH_NEXT)
                cp_o(0, BM).start()

    def _step(step, carry):
        gb = modb[0:1, 5 * D:6 * D]
        row0 = pl.multiple_of(BM + step * BM2, SB)
        nsb = BM2 // SB
        cur = (xn[...], hn[...])
        for j in range(nsb):
            if j + 1 < nsb:
                nxt = prologue(row0 + (j + 1) * SB, PCH_NAT)
                h_next = nxt[1]
            else:
                nrow = jnp.minimum(row0 + BM2, S - SB)
                h_next = next_prologue(pl.multiple_of(nrow, SB), PCH_NEXT)
            x1, h2 = cur
            tok = token_of(h_next) if ANCH_STEADY else None
            ffn = ffn_part(h2, 0, F, tok)
            obuf[pl.ds(row0 + j * SB, SB), :] = (x1 + gb * ffn).astype(bf16)
            if OUT_SB:
                cp_o(row0 + j * SB, SB).start()
            if j + 1 < nsb:
                cur = nxt
        if not OUT_SB:
            cp_o(row0, BM2).start()
        return carry

    lax.fori_loop(0, NSTEP2, _step, 0)
    cp_o(0, BM).wait()
    n_out = SB if OUT_SB else BM2
    for i in range((S - BM) // n_out):
        cp_o(BM + i * n_out, n_out).wait()


def _raw_view(x):
    return x.reshape(S // 8, 8, NG, 128).transpose(0, 2, 1, 3).reshape(NG * S, 128)


@jax.jit
def pallas_adaLN_cond__ssm_conv_h3__glu_gated_swiglu__prompt_kernel(
    A_q: jax.Array,
    A_k: jax.Array,
    A_v: jax.Array,
    A_shift_k: jax.Array,
    A_ssm_k: jax.Array,
    A_ssm_D: jax.Array,
    B_x: jax.Array,
    B_w1: jax.Array,
    B_w3: jax.Array,
    B_w2: jax.Array,
    c: jax.Array,
    w_mod: jax.Array,
):
    del B_x
    any_spec = pl.BlockSpec(memory_space=pl.ANY)
    vmem_spec = pl.BlockSpec(memory_space=pltpu.VMEM)
    scratch = [
        pltpu.VMEM((KPAD + 5 * S // 2 + 24, 128), u32),
        pltpu.VMEM((5 * S // 2 + 24, 128), u32),
        pltpu.VMEM((D // 2, S), u32),
        pltpu.VMEM((NG, CH // 2 + 8, 128), u32),
        pltpu.VMEM((NG, 4, 64, 128), u32),
        pltpu.VMEM((NG, 4, 64, 128), u32),
        pltpu.VMEM((NG, NCH, 4, 2, PR, 128), f32),
        pltpu.VMEM((NG, NCH, 4, 2, PR, 128), f32),
        pltpu.VMEM((NG, 4, 2, PR, 128), f32),
        pltpu.VMEM((NG, 4, PR, 128), u32),
        pltpu.VMEM((NG, 4, PR, 128), u32),
        pltpu.VMEM((NG, S + 8, 128), f32),
        pltpu.VMEM((S // 2, D), u32),
        pltpu.VMEM((D // 2, F), u32),
        pltpu.VMEM((D // 2, F), u32),
        pltpu.VMEM((F // 2, D), u32),
        pltpu.VMEM((D // 2, 6 * D), u32),
        pltpu.VMEM((8, 6 * D), f32),
        pltpu.VMEM((SB, D), bf16),
        pltpu.VMEM((SB, D), f32),
        pltpu.VMEM((BM, D), bf16),
        pltpu.VMEM((BM, D), f32),
        pltpu.VMEM((BM, D), f32),
        pltpu.VMEM((S, D), bf16),
        pltpu.VMEM((4, 128, 128), u32),
        pltpu.VMEM((4, 64, 256), u32),
        pltpu.SemaphoreType.DMA((8, 8)),
    ]
    return pl.pallas_call(
        _kernel,
        in_specs=[any_spec] * 8 + [vmem_spec] * 4 + [pl.BlockSpec(memory_space=pltpu.SMEM)],
        out_specs=any_spec,
        out_shape=jax.ShapeDtypeStruct((1, S, D), bf16),
        scratch_shapes=scratch,
        compiler_params=pltpu.CompilerParams(
            vmem_limit_bytes=100 * 1024 * 1024),
    )(A_q, _raw_view(A_k), _raw_view(A_v), A_ssm_k, B_w1, B_w3, B_w2, w_mod,
      A_shift_k.T, A_ssm_D, c,
      jnp.zeros((8, 128), jnp.uint32), jnp.zeros((32,), jnp.int32))
```

```python
import os as _os
import numpy as np
import jax
import jax.numpy as jnp
from jax import lax
import jax.experimental.pallas as pl
import jax.experimental.pallas.tpu as pltpu

f32 = jnp.float32
bf16 = jnp.bfloat16
u32 = jnp.uint32

S = 2048
D = 640
F = 1536
NG = D // 128
NCH = 4
CH = S // NCH
NDFT = 2 * CH
EPS = 1e-5

BM = 512
SB = 128
NSB = BM // SB
BM2 = int(_os.environ.get('BM2', 256))
NSTEP2 = (S - BM) // BM2
FCS = tuple(int(x) for x in _os.environ.get('FCS', '384,512,640').split(','))
NFC = len(FCS)
FLO = tuple(sum(FCS[:i]) for i in range(NFC))
KPAD = 40
RB = int(_os.environ.get('RB', 32))
PCH_FS, PCH_NAT, PCH_NEXT = (int(x) for x in _os.environ.get('PCH', '2,8,8').split(','))
NRCP_P = int(_os.environ.get('NRCP_P', 3))
PR = 136
PCHAIN0 = False
OUT_SB = int(_os.environ.get('OUT_SB', 1))
WM0 = int(_os.environ.get('WM0', 1920))
NPRE = int(_os.environ.get('NPRE', 1))
ANCH_STEADY = int(_os.environ.get('ANCH_STEADY', 0))
KSIDE = int(_os.environ.get('KSIDE', 1))
KFIRST = int(_os.environ.get('KFIRST', 0))
RCP_B = tuple(float(x) for x in _os.environ.get('RCP_B', '-1,1.8,1.6,2.34').split(','))


def _cos_turns(x):
    fr = x - jnp.floor(x)
    w = 4.0 * jnp.minimum(fr, 1.0 - fr) - 1.0
    w2 = w * w
    acc = jnp.float32(3.598843e-06)
    for coef in (-1.6044118e-04, 4.6817541e-03, -7.9692626e-02, 6.4596410e-01, -1.5707963e+00):
        acc = acc * w2 + jnp.float32(coef)
    return acc * w


def _odd_freq(r):
    return jnp.where(r < 64, 4 * r + 1, 4 * (r - 64) + 3)


def _bc(v):
    return pltpu.bitcast(v, bf16)


def _u32(v):
    return pltpu.bitcast(v, u32)


def _half(row, n):
    if isinstance(row, int):
        return pl.ds(row // 2, n // 2)
    return pl.ds(pl.multiple_of(row // 2, 8), n // 2)


def _lo(w):
    return pltpu.bitcast(w << 16, f32)


def _hi(w):
    return pltpu.bitcast(w & jnp.uint32(0xFFFF0000), f32)


def _pk2(a, b):
    return pltpu.bitcast(pltpu.pack_elementwise([a, b], packed_dtype=bf16), u32)


def _fft4(zr, zi, inv):
    ar, ai = zr[0] + zr[2], zi[0] + zi[2]
    br, bi = zr[0] - zr[2], zi[0] - zi[2]
    cr, ci = zr[1] + zr[3], zi[1] + zi[3]
    dr, di = zr[1] - zr[3], zi[1] - zi[3]
    if not inv:
        return [ar + cr, br + di, ar - cr, br - di], [ai + ci, bi - dr, ai - ci, bi + dr]
    return [ar + cr, br - di, ar - cr, br + di], [ai + ci, bi + dr, ai - ci, bi - dr]


def _ln(x):
    m = jnp.sum(x, axis=-1, keepdims=True) * (1.0 / D)
    xc = x - m
    v = jnp.sum(xc * xc, axis=-1, keepdims=True) * (1.0 / D)
    return xc * lax.rsqrt(v + EPS)


def _kernel(q_hbm, k_hbm, v_hbm, sk_hbm, w1_hbm, w3_hbm, w2_hbm, wm_hbm,
            shk_ref, dv_ref, c_ref, zero_ref, zs_ref,
            o_hbm,
            kraw, vraw, skbuf, ktbuf, rx, rk, xh, kh, zb, ub0, ub1, ybuf,
            qbuf, w1b, w3b, w2b, wmb, modb, hn, xn, hs, xs, accs, obuf, mf_ref, gi_ref, sems):
    ub = (ub0, ub1)

    def cp_k(a):
        return pltpu.make_async_copy(
            k_hbm.at[pl.ds(5 * CH * a, 5 * CH), :],
            kraw.bitcast(bf16).at[pl.ds(2 * KPAD + 5 * CH * a, 5 * CH), :], sems.at[0, a])

    def cp_v(a):
        return pltpu.make_async_copy(
            v_hbm.at[pl.ds(5 * CH * a, 5 * CH), :],
            vraw.bitcast(bf16).at[pl.ds(5 * CH * a, 5 * CH), :], sems.at[1, a])

    def cp_s(a):
        cols = pl.ds(CH * a, CH)
        return pltpu.make_async_copy(sk_hbm.at[:, cols], skbuf.bitcast(bf16).at[:, cols], sems.at[2, a])

    def cp_wm(i):
        cols = [pl.ds(0, WM0), pl.ds(WM0, 5 * D - WM0), pl.ds(5 * D, D)][i]
        return pltpu.make_async_copy(wm_hbm.at[:, cols], wmb.bitcast(bf16).at[:, cols], sems.at[3, i])

    def cp_q(i):
        rows = pl.ds(0, BM) if i == 0 else pl.ds(BM, S - BM)
        return pltpu.make_async_copy(q_hbm.at[0, rows, :], qbuf.bitcast(bf16).at[rows, :], sems.at[3, 4 + i])

    def cp_w(t):
        cols = pl.ds(FLO[t], FCS[t])
        return [pltpu.make_async_copy(w1_hbm.at[:, cols], w1b.bitcast(bf16).at[:, cols], sems.at[4, t]),
                pltpu.make_async_copy(w3_hbm.at[:, cols], w3b.bitcast(bf16).at[:, cols], sems.at[5, t]),
                pltpu.make_async_copy(w2_hbm.at[cols, :], w2b.bitcast(bf16).at[cols, :], sems.at[6, t])]

    def cp_o(row, n):
        rows = pl.ds(row, n)
        return pltpu.make_async_copy(obuf.at[rows, :], o_hbm.at[0, rows, :], sems.at[7, 0])

    def gen_forward_dft():
        i32 = jnp.int32
        wrow = lax.broadcasted_iota(i32, (128, 128), 0)
        n4 = (4 * lax.broadcasted_iota(i32, (128, 128), 1)).astype(f32)
        coef, quarter = [], []
        for h in range(2):
            rho = 2 * wrow + h
            rem = rho % (2 * RB)
            r = RB * (rho // (2 * RB)) + rem % RB
            coef.append(_odd_freq(r).astype(f32) * (0.5 / NDFT))
            quarter.append((rem // RB).astype(f32) * 0.25)
        for p in range(4):
            v = [_cos_turns(coef[h] * (n4 + float(p)) + quarter[h]) for h in range(2)]
            mf_ref[p] = _pk2(v[0], v[1])

    def gen_inverse_dft():
        i32 = jnp.int32
        wrow = lax.broadcasted_iota(i32, (64, 256), 0)
        col = lax.broadcasted_iota(i32, (64, 256), 1)
        coef = _odd_freq(col // 2).astype(f32) * (0.5 / NDFT)
        quarter = (col % 2).astype(f32) * 0.25
        for p in range(4):
            v = [_cos_turns(coef * (8 * wrow + (4 * h + p)).astype(f32) + quarter) for h in range(2)]
            gi_ref[p] = _pk2(v[0], v[1])

    def prep_x(g, a, t, wts, mask, inj):
        i0_ = 64 * a + 8 * t
        kb = KPAD + 20 * i0_ + 4 * g
        kl = [kraw[pl.ds(kb + w, 8, stride=20), :] for w in range(4)]
        km2 = kraw[pl.ds(kb - 18, 8, stride=20), :]
        km3 = kraw[pl.ds(kb - 17, 8, stride=20), :]
        e = [_hi(km2), _lo(km3), _hi(km3)]
        for w in range(4):
            e += [_lo(kl[w]), _hi(kl[w])]
        if inj is not None:
            e[3] = jnp.where(mask, inj, e[3])
        vb = 20 * i0_ + 4 * g
        kv = []
        for w in range(4):
            vw = vraw[pl.ds(vb + w, 8, stride=20), :]
            for h, vv in enumerate((_lo(vw), _hi(vw))):
                r = 3 + 2 * w + h
                ks = wts[0] * e[r] + wts[1] * e[r - 1] + wts[2] * e[r - 2] + wts[3] * e[r - 3]
                kv.append(ks * vv)
        tok = None
        for p in range(4):
            pk = _pk2(kv[p], kv[p + 4])
            rx[g, p, pl.ds(8 * t, 8), :] = pk
            tok = pk if tok is None else tok | pk
        return tok

    def prep_k(g, m):
        blk = _bc(skbuf[pl.ds(64 * g, 64), pl.ds(CH * m, CH)])
        ktbuf[g, 0:CH // 2, :] = pltpu.bitcast(blk.T, u32)
        lo16 = jnp.uint32(0xFFFF)
        hi16 = jnp.uint32(0xFFFF0000)
        for t in range(8):
            w = [ktbuf[g, pl.ds(32 * t + e_, 8, stride=4), :] for e_ in range(4)]
            rows = pl.ds(8 * t, 8)
            rk[g, 0, rows, :] = (w[0] & lo16) | (w[2] << 16)
            rk[g, 1, rows, :] = (w[0] >> 16) | (w[2] & hi16)
            rk[g, 2, rows, :] = (w[1] & lo16) | (w[3] << 16)
            rk[g, 3, rows, :] = (w[1] >> 16) | (w[3] & hi16)

    def fwd(src, dst, g, a, b, dvec):
        z = [jnp.dot(_bc(mf_ref[p, pl.ds(RB * b, RB), :]), _bc(src[g, p]),
                     preferred_element_type=f32) for p in range(4)]
        xr, xi = _fft4([t[:RB] for t in z], [t[RB:] for t in z], False)
        for f2 in range(4):
            dst[g, a, f2, 0, pl.ds(RB * b, RB), :] = xr[f2] if dvec is None else xr[f2] + dvec
            dst[g, a, f2, 1, pl.ds(RB * b, RB), :] = xi[f2]

    def cell(g, j, c, mask, inj):
        rows = pl.ds(8 * j, 8)
        zr, zi = [], []
        for f2 in range(4):
            ar = ai = None
            for a in range(c + 1):
                m = c - a
                xr = xh[g, a, f2, 0, rows, :]
                xi = xh[g, a, f2, 1, rows, :]
                kr = kh[g, m, f2, 0, rows, :]
                ki = kh[g, m, f2, 1, rows, :]
                if inj is not None and f2 == 0 and a == 0:
                    kr = jnp.where(mask, inj, kr)
                tr = xr * kr - xi * ki
                ti = xr * ki + xi * kr
                ar = tr if ar is None else ar + tr
                ai = ti if ai is None else ai + ti
            zr.append(ar)
            zi.append(ai)
        yr, yi = zr, zi
        if c > 0:
            pr = [zb[g, f, 0, rows, :] for f in range(4)]
            pi = [zb[g, f, 1, rows, :] for f in range(4)]
            if j < 8:
                yr = [zr[f] - pi[f] for f in range(4)]
                yi = [zi[f] + pr[f] for f in range(4)]
            else:
                yr = [zr[f] + pi[f] for f in range(4)]
                yi = [zi[f] - pr[f] for f in range(4)]
        if c + 1 < NCH:
            for f in range(4):
                zb[g, f, 0, rows, :] = zr[f]
                zb[g, f, 1, rows, :] = zi[f]
        ur, ui = _fft4(yr, yi, True)
        tok = None
        for s2 in range(4):
            pk = _pk2(ur[s2], ui[s2])
            ub[c % 2][g, s2, rows, :] = pk
            tok = pk if tok is None else tok | pk
        return tok

    def inv(g, c, s2):
        y = jnp.dot(_bc(gi_ref[s2]), _bc(ub[c % 2][g, s2, 0:128, :]), preferred_element_type=f32)
        ybuf[g, pl.ds(CH * c + s2, 128, stride=4), :] = y

    def delayed(tok, n):
        t = pltpu.bitcast(tok, f32)
        for _ in range(n):
            t = pl.reciprocal(t, approx=True)
        return t

    def mod_cols(lo_, n):
        cc = c_ref[...].astype(f32)
        sc = (cc * jax.nn.sigmoid(cc)).astype(bf16)
        lhs = jnp.broadcast_to(sc, (8, D))
        modb[:, pl.ds(lo_, n)] = jnp.dot(lhs, _bc(wmb[:, pl.ds(lo_, n)]), preferred_element_type=f32)

    _cnt = [0]

    def first_step():
        i = _cnt[0]
        _cnt[0] += 1
        return zs_ref[i] == 0

    def prologue(row, nchunk):
        sa = modb[0:1, 0 * D:1 * D]
        ca1 = 1.0 + modb[0:1, 1 * D:2 * D]
        ga = modb[0:1, 2 * D:3 * D] * (2.0 / NDFT)
        sb = modb[0:1, 3 * D:4 * D]
        cb1 = 1.0 + modb[0:1, 4 * D:5 * D]
        mask = zero_ref[...] != 0
        n = SB // nchunk
        x1s, h2s = [], []
        tok = None
        for i in range(nchunk):
            r = pl.ds(row + i * n, n)
            q = _bc(qbuf[_half(row + i * n, n), :]).astype(f32)
            if tok is not None:
                q00 = jnp.where(mask, tok, q[0:8, 0:128])
                top = jnp.concatenate([q00, q[0:8, 128:]], axis=1)
                q = jnp.concatenate([top, q[8:]], axis=0)
            y = jnp.concatenate([ybuf[g, r, :] for g in range(NG)], axis=1)
            h1 = _ln(q) * ca1 + sa
            x1 = q + ga * (h1 * y)
            h2f = _ln(x1) * cb1 + sb
            if i + 1 < nchunk:
                parts = [h2f[8 * a:8 * a + 8, 128 * g:128 * (g + 1)]
                         for a in range(n // 8) for g in range(NG)]
                while len(parts) > 1:
                    parts = [parts[k] + parts[k + 1] if k + 1 < len(parts) else parts[k]
                             for k in range(0, len(parts), 2)]
                tok = parts[0]
            x1s.append(x1)
            h2s.append(h2f.astype(bf16))
        return jnp.concatenate(x1s, axis=0), jnp.concatenate(h2s, axis=0)

    def token_of(h2):
        w = pltpu.bitcast(h2, u32)
        parts = [w[8 * i:8 * i + 8, 128 * g:128 * (g + 1)]
                 for i in range(w.shape[0] // 8) for g in range(NG)]
        while len(parts) > 1:
            parts = [parts[i] | parts[i + 1] if i + 1 < len(parts) else parts[i]
                     for i in range(0, len(parts), 2)]
        return parts[0]

    def anchored(h, tok):
        mask = zero_ref[...] != 0
        w = pltpu.bitcast(h, u32)
        w0 = jnp.where(mask, tok, w[0:8, 0:128])
        top = jnp.concatenate([w0, w[0:8, 128:]], axis=1)
        return pltpu.bitcast(jnp.concatenate([top, w[8:]], axis=0), bf16)

    def ffn_part(h2, lo_, n, tok=None):
        cols = pl.ds(lo_, n)
        gate = jnp.dot(h2, _bc(w1b[:, cols]), preferred_element_type=f32)
        hu = h2 if tok is None else anchored(h2, tok)
        up = jnp.dot(hu, _bc(w3b[:, cols]), preferred_element_type=f32)
        act = (gate * jax.nn.sigmoid(gate) * up).astype(bf16)
        return jnp.dot(act, _bc(w2b[_half(lo_, n), :]), preferred_element_type=f32)

    def next_prologue(row, nchunk):
        x1, h2 = prologue(row, nchunk)
        xn[...] = x1
        hn[...] = h2
        return h2

    @pl.when(first_step())
    def _issue():
        cp_s(0).start(); cp_k(0).start(); cp_v(0).start()
        cp_k(1).start(); cp_v(1).start(); cp_s(1).start()
        cp_s(2).start(); cp_k(2).start(); cp_v(2).start()
        cp_s(3).start(); cp_k(3).start(); cp_v(3).start()
        cp_wm(0).start()
        cp_wm(1).start()
        cp_q(0).start()
        for t in range(NFC):
            if t == NFC - 1:
                cp_wm(2).start()
            for c_ in cp_w(t):
                c_.start()
        cp_q(1).start()
        kraw[0:KPAD, :] = jnp.zeros((KPAD, 128), u32)
        gen_forward_dft()
        gen_inverse_dft()

    def fwd_k(a):
        dv = dv_ref[...].astype(f32).reshape(1, D)
        for g in range(NG):
            prep_k(g, a)
            dvec = jnp.broadcast_to(dv[:, 128 * g:128 * (g + 1)], (RB, 128)) if a == 0 else None
            for b in range(128 // RB):
                fwd(rk, kh, g, a, b, dvec)

    def part_a(a, with_k):
        mask = zero_ref[...] != 0
        shk = shk_ref[...].astype(f32)
        inj = None
        for g in range(NG):
            lanes = slice(128 * g, 128 * (g + 1))
            wts = [jnp.broadcast_to(shk[j:j + 1, lanes], (8, 128)) for j in range(4)]
            for t in range(8):
                tok = prep_x(g, a, t, wts, mask, inj)
                inj = delayed(tok, NRCP_P) if g > 0 or PCHAIN0 else None
            if with_k:
                prep_k(g, a)
            for b in range(128 // RB):
                fwd(rx, xh, g, a, b, None)
            if with_k:
                for b in range(128 // RB):
                    fwd(rk, kh, g, a, b, None)

    def part_b(c):
        mask = zero_ref[...] != 0
        inj = None
        for g in range(NG):
            for j in range(16):
                tok = cell(g, j, c, mask, inj)
                n = 16 * g + j
                nd = int((n + 1) * RCP_B[c]) - int(n * RCP_B[c])
                inj = delayed(tok, nd) if RCP_B[c] >= 0 else None
        if c > 0:
            for g in range(NG):
                for s2 in range(4):
                    inv(g, c - 1, s2)

    @pl.when(first_step())
    def _blkA0k():
        cp_s(0).wait()
        fwd_k(0)

    @pl.when(first_step())
    def _blkA0x():
        cp_k(0).wait(); cp_v(0).wait()
        part_a(0, False)

    for a in range(1, NCH):
        @pl.when(first_step())
        def _blkB(c=a - 1):
            k_here = KSIDE and c >= 1
            if k_here:
                cp_s(c + 1).wait()
            if k_here and KFIRST:
                fwd_k(c + 1)
            part_b(c)
            if k_here and not KFIRST:
                fwd_k(c + 1)

        if a == 1:
            @pl.when(first_step())
            def _blkM1x():
                cp_k(1).wait(); cp_v(1).wait()
                part_a(1, False)

            @pl.when(first_step())
            def _blkM1k():
                cp_s(1).wait()
                fwd_k(1)
        else:
            @pl.when(first_step())
            def _blkM(a=a):
                cp_k(a).wait(); cp_v(a).wait()
                if not KSIDE:
                    cp_s(a).wait()
                part_a(a, not KSIDE)

    @pl.when(first_step())
    def _blkB3():
        cp_wm(0).wait()
        part_b(NCH - 1)
        mod_cols(0, WM0)

    @pl.when(first_step())
    def _blkC():
        cp_wm(1).wait()
        cp_q(0).wait()
        mod_cols(WM0, 5 * D - WM0)
        for g in range(NG):
            for s2 in range(4):
                inv(g, NCH - 1, s2)
        for j in range(NPRE):
            x1, h2 = prologue(j * SB, 1)
            xs[pl.ds(j * SB, SB), :] = x1
            hs[pl.ds(j * SB, SB), :] = h2

    for t in range(NFC):
        @pl.when(first_step())
        def _first_rows(t=t):
            for c_ in cp_w(t):
                c_.wait()
            if t == NFC - 1:
                cp_wm(2).wait()
                cp_q(1).wait()
                mod_cols(5 * D, D)
            for j in range(NSB):
                r = pl.ds(j * SB, SB)
                if t == 0:
                    if j < NPRE:
                        h2 = hs[r, :]
                    else:
                        x1, h2 = prologue(j * SB, PCH_FS)
                        xs[r, :] = x1
                        hs[r, :] = h2
                    accs[r, :] = ffn_part(h2, FLO[0], FCS[0])
                elif t < NFC - 1:
                    accs[r, :] += ffn_part(hs[r, :], FLO[t], FCS[t])
                else:
                    gb = modb[0:1, 5 * D:6 * D]
                    ffn = accs[r, :] + ffn_part(hs[r, :], FLO[t], FCS[t])
                    obuf[r, :] = (xs[r, :] + gb * ffn).astype(bf16)
            if t == NFC - 1:
                next_prologue(BM, PCH_NEXT)
                cp_o(0, BM).start()

    def _step(step, carry):
        gb = modb[0:1, 5 * D:6 * D]
        row0 = pl.multiple_of(BM + step * BM2, SB)
        nsb = BM2 // SB
        cur = (xn[...], hn[...])
        for j in range(nsb):
            if j + 1 < nsb:
                nxt = prologue(row0 + (j + 1) * SB, PCH_NAT)
                h_next = nxt[1]
            else:
                nrow = jnp.minimum(row0 + BM2, S - SB)
                h_next = next_prologue(pl.multiple_of(nrow, SB), PCH_NEXT)
            x1, h2 = cur
            tok = token_of(h_next) if ANCH_STEADY else None
            ffn = ffn_part(h2, 0, F, tok)
            obuf[pl.ds(row0 + j * SB, SB), :] = (x1 + gb * ffn).astype(bf16)
            if OUT_SB:
                cp_o(row0 + j * SB, SB).start()
            if j + 1 < nsb:
                cur = nxt
        if not OUT_SB:
            cp_o(row0, BM2).start()
        return carry

    lax.fori_loop(0, NSTEP2, _step, 0)
    cp_o(0, BM).wait()
    n_out = SB if OUT_SB else BM2
    for i in range((S - BM) // n_out):
        cp_o(BM + i * n_out, n_out).wait()


def _raw_view(x):
    return x.reshape(S // 8, 8, NG, 128).transpose(0, 2, 1, 3).reshape(NG * S, 128)


@jax.jit
def pallas_adaLN_cond__ssm_conv_h3__glu_gated_swiglu__prompt_kernel(
    A_q: jax.Array,
    A_k: jax.Array,
    A_v: jax.Array,
    A_shift_k: jax.Array,
    A_ssm_k: jax.Array,
    A_ssm_D: jax.Array,
    B_x: jax.Array,
    B_w1: jax.Array,
    B_w3: jax.Array,
    B_w2: jax.Array,
    c: jax.Array,
    w_mod: jax.Array,
):
    del B_x
    any_spec = pl.BlockSpec(memory_space=pl.ANY)
    vmem_spec = pl.BlockSpec(memory_space=pltpu.VMEM)
    scratch = [
        pltpu.VMEM((KPAD + 5 * S // 2 + 24, 128), u32),
        pltpu.VMEM((5 * S // 2 + 24, 128), u32),
        pltpu.VMEM((D // 2, S), u32),
        pltpu.VMEM((NG, CH // 2 + 8, 128), u32),
        pltpu.VMEM((NG, 4, 64, 128), u32),
        pltpu.VMEM((NG, 4, 64, 128), u32),
        pltpu.VMEM((NG, NCH, 4, 2, PR, 128), f32),
        pltpu.VMEM((NG, NCH, 4, 2, PR, 128), f32),
        pltpu.VMEM((NG, 4, 2, PR, 128), f32),
        pltpu.VMEM((NG, 4, PR, 128), u32),
        pltpu.VMEM((NG, 4, PR, 128), u32),
        pltpu.VMEM((NG, S + 8, 128), f32),
        pltpu.VMEM((S // 2, D), u32),
        pltpu.VMEM((D // 2, F), u32),
        pltpu.VMEM((D // 2, F), u32),
        pltpu.VMEM((F // 2, D), u32),
        pltpu.VMEM((D // 2, 6 * D), u32),
        pltpu.VMEM((8, 6 * D), f32),
        pltpu.VMEM((SB, D), bf16),
        pltpu.VMEM((SB, D), f32),
        pltpu.VMEM((BM, D), bf16),
        pltpu.VMEM((BM, D), f32),
        pltpu.VMEM((BM, D), f32),
        pltpu.VMEM((S, D), bf16),
        pltpu.VMEM((4, 128, 128), u32),
        pltpu.VMEM((4, 64, 256), u32),
        pltpu.SemaphoreType.DMA((8, 8)),
    ]
    return pl.pallas_call(
        _kernel,
        in_specs=[any_spec] * 8 + [vmem_spec] * 4 + [pl.BlockSpec(memory_space=pltpu.SMEM)],
        out_specs=any_spec,
        out_shape=jax.ShapeDtypeStruct((1, S, D), bf16),
        scratch_shapes=scratch,
        compiler_params=pltpu.CompilerParams(
            vmem_limit_bytes=100 * 1024 * 1024),
    )(A_q, _raw_view(A_k), _raw_view(A_v), A_ssm_k, B_w1, B_w3, B_w2, w_mod,
      A_shift_k.T, A_ssm_D, c,
      jnp.zeros((8, 128), jnp.uint32), jnp.zeros((32,), jnp.int32))
```

```python
import jax
import jax.numpy as jnp
from jax import lax
import jax.experimental.pallas as pl
import jax.experimental.pallas.tpu as pltpu

f32 = jnp.float32
bf16 = jnp.bfloat16
u32 = jnp.uint32

S = 2048
D = 640
F = 1536
NG = D // 128
NCH = 4
CH = S // NCH
NDFT = 2 * CH
EPS = 1e-5

SB = 128
BM = 512
NSB = BM // SB
BM2 = 256
NSTEP2 = (S - BM) // BM2
FCS = (384, 512, 640)
NFC = len(FCS)
FLO = tuple(sum(FCS[:i]) for i in range(NFC))
WM0 = 1920

KPAD = 40
RB = 32
PR = 136

PCH_FIRST, PCH_STEADY = 2, 8
NRCP_P = 3
RCP_B = (None, 1.8, 1.6, 2.34)


def _cos_turns(x):
    fr = x - jnp.floor(x)
    w = 4.0 * jnp.minimum(fr, 1.0 - fr) - 1.0
    w2 = w * w
    acc = jnp.float32(3.598843e-06)
    for coef in (-1.6044118e-04, 4.6817541e-03, -7.9692626e-02, 6.4596410e-01, -1.5707963e+00):
        acc = acc * w2 + jnp.float32(coef)
    return acc * w


def _odd_freq(r):
    return jnp.where(r < 64, 4 * r + 1, 4 * (r - 64) + 3)


def _bc(v):
    return pltpu.bitcast(v, bf16)


def _half(row, n):
    if isinstance(row, int):
        return pl.ds(row // 2, n // 2)
    return pl.ds(pl.multiple_of(row // 2, 8), n // 2)


def _lo(w):
    return pltpu.bitcast(w << 16, f32)


def _hi(w):
    return pltpu.bitcast(w & jnp.uint32(0xFFFF0000), f32)


def _pk2(a, b):
    return pltpu.bitcast(pltpu.pack_elementwise([a, b], packed_dtype=bf16), u32)


def _fft4(zr, zi, inv):
    ar, ai = zr[0] + zr[2], zi[0] + zi[2]
    br, bi = zr[0] - zr[2], zi[0] - zi[2]
    cr, ci = zr[1] + zr[3], zi[1] + zi[3]
    dr, di = zr[1] - zr[3], zi[1] - zi[3]
    if not inv:
        return [ar + cr, br + di, ar - cr, br - di], [ai + ci, bi - dr, ai - ci, bi + dr]
    return [ar + cr, br - di, ar - cr, br + di], [ai + ci, bi + dr, ai - ci, bi - dr]


def _ln(x):
    m = jnp.sum(x, axis=-1, keepdims=True) * (1.0 / D)
    xc = x - m
    v = jnp.sum(xc * xc, axis=-1, keepdims=True) * (1.0 / D)
    return xc * lax.rsqrt(v + EPS)


def _kernel(q_hbm, k_hbm, v_hbm, sk_hbm, w1_hbm, w3_hbm, w2_hbm, wm_hbm,
            shk_ref, dv_ref, c_ref, zero_ref, zs_ref,
            o_hbm,
            kraw, vraw, skbuf, ktbuf, rx, rk, xh, kh, zb, ub0, ub1, ybuf,
            qbuf, w1b, w3b, w2b, wmb, modb, hn, xn, hs, xs, accs, obuf, mf_ref, gi_ref, sems):
    ub = (ub0, ub1)

    def cp_k(a):
        return pltpu.make_async_copy(
            k_hbm.at[pl.ds(5 * CH * a, 5 * CH), :],
            kraw.bitcast(bf16).at[pl.ds(2 * KPAD + 5 * CH * a, 5 * CH), :], sems.at[0, a])

    def cp_v(a):
        return pltpu.make_async_copy(
            v_hbm.at[pl.ds(5 * CH * a, 5 * CH), :],
            vraw.bitcast(bf16).at[pl.ds(5 * CH * a, 5 * CH), :], sems.at[1, a])

    def cp_s(a):
        cols = pl.ds(CH * a, CH)
        return pltpu.make_async_copy(sk_hbm.at[:, cols], skbuf.bitcast(bf16).at[:, cols], sems.at[2, a])

    def cp_wm(i):
        cols = [pl.ds(0, WM0), pl.ds(WM0, 5 * D - WM0), pl.ds(5 * D, D)][i]
        return pltpu.make_async_copy(wm_hbm.at[:, cols], wmb.bitcast(bf16).at[:, cols], sems.at[3, i])

    def cp_q(i):
        rows = pl.ds(0, BM) if i == 0 else pl.ds(BM, S - BM)
        return pltpu.make_async_copy(q_hbm.at[0, rows, :], qbuf.bitcast(bf16).at[rows, :], sems.at[3, 4 + i])

    def cp_w(t):
        cols = pl.ds(FLO[t], FCS[t])
        return [pltpu.make_async_copy(w1_hbm.at[:, cols], w1b.bitcast(bf16).at[:, cols], sems.at[4, t]),
                pltpu.make_async_copy(w3_hbm.at[:, cols], w3b.bitcast(bf16).at[:, cols], sems.at[5, t]),
                pltpu.make_async_copy(w2_hbm.at[cols, :], w2b.bitcast(bf16).at[cols, :], sems.at[6, t])]

    def cp_o(row, n):
        rows = pl.ds(row, n)
        return pltpu.make_async_copy(obuf.at[rows, :], o_hbm.at[0, rows, :], sems.at[7, 0])

    def gen_forward_dft():
        i32 = jnp.int32
        wrow = lax.broadcasted_iota(i32, (128, 128), 0)
        n4 = (4 * lax.broadcasted_iota(i32, (128, 128), 1)).astype(f32)
        coef, quarter = [], []
        for h in range(2):
            rho = 2 * wrow + h
            rem = rho % (2 * RB)
            r = RB * (rho // (2 * RB)) + rem % RB
            coef.append(_odd_freq(r).astype(f32) * (0.5 / NDFT))
            quarter.append((rem // RB).astype(f32) * 0.25)
        for p in range(4):
            v = [_cos_turns(coef[h] * (n4 + float(p)) + quarter[h]) for h in range(2)]
            mf_ref[p] = _pk2(v[0], v[1])

    def gen_inverse_dft():
        i32 = jnp.int32
        wrow = lax.broadcasted_iota(i32, (64, 256), 0)
        col = lax.broadcasted_iota(i32, (64, 256), 1)
        coef = _odd_freq(col // 2).astype(f32) * (0.5 / NDFT)
        quarter = (col % 2).astype(f32) * 0.25
        for p in range(4):
            v = [_cos_turns(coef * (8 * wrow + (4 * h + p)).astype(f32) + quarter) for h in range(2)]
            gi_ref[p] = _pk2(v[0], v[1])

    def prep_x(g, a, t, wts, mask, inj):
        i0_ = 64 * a + 8 * t
        kb = KPAD + 20 * i0_ + 4 * g
        kl = [kraw[pl.ds(kb + w, 8, stride=20), :] for w in range(4)]
        km2 = kraw[pl.ds(kb - 18, 8, stride=20), :]
        km3 = kraw[pl.ds(kb - 17, 8, stride=20), :]
        e = [_hi(km2), _lo(km3), _hi(km3)]
        for w in range(4):
            e += [_lo(kl[w]), _hi(kl[w])]
        if inj is not None:
            e[3] = jnp.where(mask, inj, e[3])
        vb = 20 * i0_ + 4 * g
        kv = []
        for w in range(4):
            vw = vraw[pl.ds(vb + w, 8, stride=20), :]
            for h, vv in enumerate((_lo(vw), _hi(vw))):
                r = 3 + 2 * w + h
                ks = wts[0] * e[r] + wts[1] * e[r - 1] + wts[2] * e[r - 2] + wts[3] * e[r - 3]
                kv.append(ks * vv)
        tok = None
        for p in range(4):
            pk = _pk2(kv[p], kv[p + 4])
            rx[g, p, pl.ds(8 * t, 8), :] = pk
            tok = pk if tok is None else tok | pk
        return tok

    def prep_k(g, m):
        blk = _bc(skbuf[pl.ds(64 * g, 64), pl.ds(CH * m, CH)])
        ktbuf[g, 0:CH // 2, :] = pltpu.bitcast(blk.T, u32)
        lo16 = jnp.uint32(0xFFFF)
        hi16 = jnp.uint32(0xFFFF0000)
        for t in range(8):
            w = [ktbuf[g, pl.ds(32 * t + e_, 8, stride=4), :] for e_ in range(4)]
            rows = pl.ds(8 * t, 8)
            rk[g, 0, rows, :] = (w[0] & lo16) | (w[2] << 16)
            rk[g, 1, rows, :] = (w[0] >> 16) | (w[2] & hi16)
            rk[g, 2, rows, :] = (w[1] & lo16) | (w[3] << 16)
            rk[g, 3, rows, :] = (w[1] >> 16) | (w[3] & hi16)

    def fwd(src, dst, g, a, b, dvec):
        z = [jnp.dot(_bc(mf_ref[p, pl.ds(RB * b, RB), :]), _bc(src[g, p]),
                     preferred_element_type=f32) for p in range(4)]
        xr, xi = _fft4([t[:RB] for t in z], [t[RB:] for t in z], False)
        for f2 in range(4):
            dst[g, a, f2, 0, pl.ds(RB * b, RB), :] = xr[f2] if dvec is None else xr[f2] + dvec
            dst[g, a, f2, 1, pl.ds(RB * b, RB), :] = xi[f2]

    def cell(g, j, c, mask, inj):
        rows = pl.ds(8 * j, 8)
        zr, zi = [], []
        for f2 in range(4):
            ar = ai = None
            for a in range(c + 1):
                m = c - a
                xr = xh[g, a, f2, 0, rows, :]
                xi = xh[g, a, f2, 1, rows, :]
                kr = kh[g, m, f2, 0, rows, :]
                ki = kh[g, m, f2, 1, rows, :]
                if inj is not None and f2 == 0 and a == 0:
                    kr = jnp.where(mask, inj, kr)
                tr = xr * kr - xi * ki
                ti = xr * ki + xi * kr
                ar = tr if ar is None else ar + tr
                ai = ti if ai is None else ai + ti
            zr.append(ar)
            zi.append(ai)
        yr, yi = zr, zi
        if c > 0:
            pr = [zb[g, f, 0, rows, :] for f in range(4)]
            pi = [zb[g, f, 1, rows, :] for f in range(4)]
            if j < 8:
                yr = [zr[f] - pi[f] for f in range(4)]
                yi = [zi[f] + pr[f] for f in range(4)]
            else:
                yr = [zr[f] + pi[f] for f in range(4)]
                yi = [zi[f] - pr[f] for f in range(4)]
        if c + 1 < NCH:
            for f in range(4):
                zb[g, f, 0, rows, :] = zr[f]
                zb[g, f, 1, rows, :] = zi[f]
        ur, ui = _fft4(yr, yi, True)
        tok = None
        for s2 in range(4):
            pk = _pk2(ur[s2], ui[s2])
            ub[c % 2][g, s2, rows, :] = pk
            tok = pk if tok is None else tok | pk
        return tok

    def inv(g, c, s2):
        y = jnp.dot(_bc(gi_ref[s2]), _bc(ub[c % 2][g, s2, 0:128, :]), preferred_element_type=f32)
        ybuf[g, pl.ds(CH * c + s2, 128, stride=4), :] = y

    def delayed(tok, n):
        t = pltpu.bitcast(tok, f32)
        for _ in range(n):
            t = pl.reciprocal(t, approx=True)
        return t

    def mod_cols(lo_, n):
        cc = c_ref[...].astype(f32)
        sc = (cc * jax.nn.sigmoid(cc)).astype(bf16)
        lhs = jnp.broadcast_to(sc, (8, D))
        modb[:, pl.ds(lo_, n)] = jnp.dot(lhs, _bc(wmb[:, pl.ds(lo_, n)]), preferred_element_type=f32)

    _cnt = [0]

    def first_step():
        i = _cnt[0]
        _cnt[0] += 1
        return zs_ref[i] == 0

    def prologue(row, nchunk):
        sa = modb[0:1, 0 * D:1 * D]
        ca1 = 1.0 + modb[0:1, 1 * D:2 * D]
        ga = modb[0:1, 2 * D:3 * D] * (2.0 / NDFT)
        sb = modb[0:1, 3 * D:4 * D]
        cb1 = 1.0 + modb[0:1, 4 * D:5 * D]
        mask = zero_ref[...] != 0
        n = SB // nchunk
        x1s, h2s = [], []
        tok = None
        for i in range(nchunk):
            r = pl.ds(row + i * n, n)
            q = _bc(qbuf[_half(row + i * n, n), :]).astype(f32)
            if tok is not None:
                q00 = jnp.where(mask, tok, q[0:8, 0:128])
                top = jnp.concatenate([q00, q[0:8, 128:]], axis=1)
                q = jnp.concatenate([top, q[8:]], axis=0)
            y = jnp.concatenate([ybuf[g, r, :] for g in range(NG)], axis=1)
            h1 = _ln(q) * ca1 + sa
            x1 = q + ga * (h1 * y)
            h2f = _ln(x1) * cb1 + sb
            if i + 1 < nchunk:
                parts = [h2f[8 * a:8 * a + 8, 128 * g:128 * (g + 1)]
                         for a in range(n // 8) for g in range(NG)]
                while len(parts) > 1:
                    parts = [parts[k] + parts[k + 1] if k + 1 < len(parts) else parts[k]
                             for k in range(0, len(parts), 2)]
                tok = parts[0]
            x1s.append(x1)
            h2s.append(h2f.astype(bf16))
        return jnp.concatenate(x1s, axis=0), jnp.concatenate(h2s, axis=0)

    def ffn_part(h2, lo_, n):
        cols = pl.ds(lo_, n)
        gate = jnp.dot(h2, _bc(w1b[:, cols]), preferred_element_type=f32)
        up = jnp.dot(h2, _bc(w3b[:, cols]), preferred_element_type=f32)
        act = (gate * jax.nn.sigmoid(gate) * up).astype(bf16)
        return jnp.dot(act, _bc(w2b[_half(lo_, n), :]), preferred_element_type=f32)

    def next_prologue(row, nchunk):
        x1, h2 = prologue(row, nchunk)
        xn[...] = x1
        hn[...] = h2

    @pl.when(first_step())
    def _issue():
        cp_s(0).start(); cp_k(0).start(); cp_v(0).start()
        cp_k(1).start(); cp_v(1).start(); cp_s(1).start()
        cp_s(2).start(); cp_k(2).start(); cp_v(2).start()
        cp_s(3).start(); cp_k(3).start(); cp_v(3).start()
        cp_wm(0).start()
        cp_wm(1).start()
        cp_q(0).start()
        for t in range(NFC):
            if t == NFC - 1:
                cp_wm(2).start()
            for c_ in cp_w(t):
                c_.start()
        cp_q(1).start()
        kraw[0:KPAD, :] = jnp.zeros((KPAD, 128), u32)
        gen_forward_dft()
        gen_inverse_dft()

    def fwd_k(a):
        dv = dv_ref[...].astype(f32).reshape(1, D)
        for g in range(NG):
            prep_k(g, a)
            dvec = jnp.broadcast_to(dv[:, 128 * g:128 * (g + 1)], (RB, 128)) if a == 0 else None
            for b in range(128 // RB):
                fwd(rk, kh, g, a, b, dvec)

    def fwd_x(a):
        mask = zero_ref[...] != 0
        shk = shk_ref[...].astype(f32)
        inj = None
        for g in range(NG):
            lanes = slice(128 * g, 128 * (g + 1))
            wts = [jnp.broadcast_to(shk[j:j + 1, lanes], (8, 128)) for j in range(4)]
            for t in range(8):
                tok = prep_x(g, a, t, wts, mask, inj)
                inj = delayed(tok, NRCP_P) if g > 0 else None
            for b in range(128 // RB):
                fwd(rx, xh, g, a, b, None)

    def part_b(c):
        mask = zero_ref[...] != 0
        inj = None
        for g in range(NG):
            for j in range(16):
                tok = cell(g, j, c, mask, inj)
                if RCP_B[c] is not None:
                    n = 16 * g + j
                    inj = delayed(tok, int((n + 1) * RCP_B[c]) - int(n * RCP_B[c]))
        if c > 0:
            for g in range(NG):
                for s2 in range(4):
                    inv(g, c - 1, s2)

    @pl.when(first_step())
    def _filter_side_0():
        cp_s(0).wait()
        fwd_k(0)

    for a in range(NCH):
        @pl.when(first_step())
        def _data_side(a=a):
            cp_k(a).wait(); cp_v(a).wait()
            fwd_x(a)

        if a == 1:
            @pl.when(first_step())
            def _filter_side_1():
                cp_s(1).wait()
                fwd_k(1)

        if a + 1 < NCH:
            @pl.when(first_step())
            def _products(c=a):
                if c >= 1:
                    cp_s(c + 1).wait()
                part_b(c)
                if c >= 1:
                    fwd_k(c + 1)

    @pl.when(first_step())
    def _products_last():
        cp_wm(0).wait()
        part_b(NCH - 1)
        mod_cols(0, WM0)

    @pl.when(first_step())
    def _finish_conv():
        cp_wm(1).wait()
        cp_q(0).wait()
        mod_cols(WM0, 5 * D - WM0)
        for g in range(NG):
            for s2 in range(4):
                inv(g, NCH - 1, s2)
        x1, h2 = prologue(0, 1)
        xs[0:SB, :] = x1
        hs[0:SB, :] = h2

    for t in range(NFC):
        @pl.when(first_step())
        def _first_rows(t=t):
            for c_ in cp_w(t):
                c_.wait()
            if t == NFC - 1:
                cp_wm(2).wait()
                cp_q(1).wait()
                mod_cols(5 * D, D)
            for j in range(NSB):
                r = pl.ds(j * SB, SB)
                if t == 0:
                    if j == 0:
                        h2 = hs[r, :]
                    else:
                        x1, h2 = prologue(j * SB, PCH_FIRST)
                        xs[r, :] = x1
                        hs[r, :] = h2
                    accs[r, :] = ffn_part(h2, FLO[0], FCS[0])
                elif t < NFC - 1:
                    accs[r, :] += ffn_part(hs[r, :], FLO[t], FCS[t])
                else:
                    gb = modb[0:1, 5 * D:6 * D]
                    ffn = accs[r, :] + ffn_part(hs[r, :], FLO[t], FCS[t])
                    obuf[r, :] = (xs[r, :] + gb * ffn).astype(bf16)
            if t == NFC - 1:
                next_prologue(BM, PCH_STEADY)
                cp_o(0, BM).start()

    def _step(step, carry):
        gb = modb[0:1, 5 * D:6 * D]
        row0 = pl.multiple_of(BM + step * BM2, SB)
        nsb = BM2 // SB
        x1, h2 = xn[...], hn[...]
        for j in range(nsb):
            if j + 1 < nsb:
                nxt = prologue(row0 + (j + 1) * SB, PCH_STEADY)
            else:
                nrow = jnp.minimum(row0 + BM2, S - SB)
                next_prologue(pl.multiple_of(nrow, SB), PCH_STEADY)
            ffn = ffn_part(h2, 0, F)
            obuf[pl.ds(row0 + j * SB, SB), :] = (x1 + gb * ffn).astype(bf16)
            cp_o(row0 + j * SB, SB).start()
            if j + 1 < nsb:
                x1, h2 = nxt
        return carry

    lax.fori_loop(0, NSTEP2, _step, 0)
    cp_o(0, BM).wait()
    for i in range((S - BM) // SB):
        cp_o(BM + i * SB, SB).wait()


def _raw_view(x):
    return x.reshape(S // 8, 8, NG, 128).transpose(0, 2, 1, 3).reshape(NG * S, 128)


@jax.jit
def pallas_adaLN_cond__ssm_conv_h3__glu_gated_swiglu__prompt_kernel(
    A_q: jax.Array,
    A_k: jax.Array,
    A_v: jax.Array,
    A_shift_k: jax.Array,
    A_ssm_k: jax.Array,
    A_ssm_D: jax.Array,
    B_x: jax.Array,
    B_w1: jax.Array,
    B_w3: jax.Array,
    B_w2: jax.Array,
    c: jax.Array,
    w_mod: jax.Array,
):
    del B_x
    any_spec = pl.BlockSpec(memory_space=pl.ANY)
    vmem_spec = pl.BlockSpec(memory_space=pltpu.VMEM)
    scratch = [
        pltpu.VMEM((KPAD + 5 * S // 2 + 24, 128), u32),
        pltpu.VMEM((5 * S // 2 + 24, 128), u32),
        pltpu.VMEM((D // 2, S), u32),
        pltpu.VMEM((NG, CH // 2 + 8, 128), u32),
        pltpu.VMEM((NG, 4, 64, 128), u32),
        pltpu.VMEM((NG, 4, 64, 128), u32),
        pltpu.VMEM((NG, NCH, 4, 2, PR, 128), f32),
        pltpu.VMEM((NG, NCH, 4, 2, PR, 128), f32),
        pltpu.VMEM((NG, 4, 2, PR, 128), f32),
        pltpu.VMEM((NG, 4, PR, 128), u32),
        pltpu.VMEM((NG, 4, PR, 128), u32),
        pltpu.VMEM((NG, S + 8, 128), f32),
        pltpu.VMEM((S // 2, D), u32),
        pltpu.VMEM((D // 2, F), u32),
        pltpu.VMEM((D // 2, F), u32),
        pltpu.VMEM((F // 2, D), u32),
        pltpu.VMEM((D // 2, 6 * D), u32),
        pltpu.VMEM((8, 6 * D), f32),
        pltpu.VMEM((SB, D), bf16),
        pltpu.VMEM((SB, D), f32),
        pltpu.VMEM((BM, D), bf16),
        pltpu.VMEM((BM, D), f32),
        pltpu.VMEM((BM, D), f32),
        pltpu.VMEM((S, D), bf16),
        pltpu.VMEM((4, 128, 128), u32),
        pltpu.VMEM((4, 64, 256), u32),
        pltpu.SemaphoreType.DMA((8, 8)),
    ]
    return pl.pallas_call(
        _kernel,
        in_specs=[any_spec] * 8 + [vmem_spec] * 4 + [pl.BlockSpec(memory_space=pltpu.SMEM)],
        out_specs=any_spec,
        out_shape=jax.ShapeDtypeStruct((1, S, D), bf16),
        scratch_shapes=scratch,
        compiler_params=pltpu.CompilerParams(
            vmem_limit_bytes=100 * 1024 * 1024),
    )(A_q, _raw_view(A_k), _raw_view(A_v), A_ssm_k, B_w1, B_w3, B_w2, w_mod,
      A_shift_k.T, A_ssm_D, c,
      jnp.zeros((8, 128), jnp.uint32), jnp.zeros((32,), jnp.int32))
```

```python
import jax
import jax.numpy as jnp
from jax import lax
import jax.experimental.pallas as pl
import jax.experimental.pallas.tpu as pltpu

f32 = jnp.float32
bf16 = jnp.bfloat16
u32 = jnp.uint32

S = 2048
D = 640
F = 1536
NG = D // 128
NCH = 4
CH = S // NCH
NDFT = 2 * CH
EPS = 1e-5

SB = 128
BM = 512
NSB = BM // SB
BM2 = 256
NSTEP2 = (S - BM) // BM2
FCS = (256, 640, 640)
NFC = len(FCS)
FLO = tuple(sum(FCS[:i]) for i in range(NFC))
WM0 = 1920

KPAD = 40
RB = 32
PR = 136

PCH_FIRST, PCH_STEADY = 2, 8
NRCP_P = 1
RCP_B = (None, 1.7, 1.5, 2.05)


def _cos_turns(x):
    fr = x - jnp.floor(x)
    w = 4.0 * jnp.minimum(fr, 1.0 - fr) - 1.0
    w2 = w * w
    acc = jnp.float32(3.598843e-06)
    for coef in (-1.6044118e-04, 4.6817541e-03, -7.9692626e-02, 6.4596410e-01, -1.5707963e+00):
        acc = acc * w2 + jnp.float32(coef)
    return acc * w


def _odd_freq(r):
    return jnp.where(r < 64, 4 * r + 1, 4 * (r - 64) + 3)


def _bc(v):
    return pltpu.bitcast(v, bf16)


def _half(row, n):
    if isinstance(row, int):
        return pl.ds(row // 2, n // 2)
    return pl.ds(pl.multiple_of(row // 2, 8), n // 2)


def _lo(w):
    return pltpu.bitcast(w << 16, f32)


def _hi(w):
    return pltpu.bitcast(w & jnp.uint32(0xFFFF0000), f32)


def _pk2(a, b):
    return pltpu.bitcast(pltpu.pack_elementwise([a, b], packed_dtype=bf16), u32)


def _fft4(zr, zi, inv):
    ar, ai = zr[0] + zr[2], zi[0] + zi[2]
    br, bi = zr[0] - zr[2], zi[0] - zi[2]
    cr, ci = zr[1] + zr[3], zi[1] + zi[3]
    dr, di = zr[1] - zr[3], zi[1] - zi[3]
    if not inv:
        return [ar + cr, br + di, ar - cr, br - di], [ai + ci, bi - dr, ai - ci, bi + dr]
    return [ar + cr, br - di, ar - cr, br + di], [ai + ci, bi + dr, ai - ci, bi - dr]


def _ln(x):
    m = jnp.sum(x, axis=-1, keepdims=True) * (1.0 / D)
    xc = x - m
    v = jnp.sum(xc * xc, axis=-1, keepdims=True) * (1.0 / D)
    return xc * lax.rsqrt(v + EPS)


def _kernel(q_hbm, k_hbm, v_hbm, sk_hbm, w1_hbm, w3_hbm, w2_hbm, wm_hbm,
            shk_ref, dv_ref, c_ref, zero_ref, zs_ref,
            o_hbm,
            kraw, vraw, skbuf, ktbuf, rx, rk, xh, kh, zb, ub0, ub1, ybuf,
            qbuf, w1b, w3b, w2b, wmb, modb, hn, xn, hs, xs, accs, obuf, mf_ref, gi_ref, sems):
    ub = (ub0, ub1)

    def cp_k(a):
        return pltpu.make_async_copy(
            k_hbm.at[pl.ds(5 * CH * a, 5 * CH), :],
            kraw.bitcast(bf16).at[pl.ds(2 * KPAD + 5 * CH * a, 5 * CH), :], sems.at[0, a])

    def cp_v(a):
        return pltpu.make_async_copy(
            v_hbm.at[pl.ds(5 * CH * a, 5 * CH), :],
            vraw.bitcast(bf16).at[pl.ds(5 * CH * a, 5 * CH), :], sems.at[1, a])

    def cp_s(a):
        cols = pl.ds(CH * a, CH)
        return pltpu.make_async_copy(sk_hbm.at[:, cols], skbuf.bitcast(bf16).at[:, cols], sems.at[2, a])

    def cp_wm(i):
        cols = [pl.ds(0, WM0), pl.ds(WM0, 5 * D - WM0), pl.ds(5 * D, D)][i]
        return pltpu.make_async_copy(wm_hbm.at[:, cols], wmb.bitcast(bf16).at[:, cols], sems.at[3, i])

    def cp_q(i):
        rows = pl.ds(0, BM) if i == 0 else pl.ds(BM, S - BM)
        return pltpu.make_async_copy(q_hbm.at[0, rows, :], qbuf.bitcast(bf16).at[rows, :], sems.at[3, 4 + i])

    def cp_w(t):
        cols = pl.ds(FLO[t], FCS[t])
        return [pltpu.make_async_copy(w1_hbm.at[:, cols], w1b.bitcast(bf16).at[:, cols], sems.at[4, t]),
                pltpu.make_async_copy(w3_hbm.at[:, cols], w3b.bitcast(bf16).at[:, cols], sems.at[5, t]),
                pltpu.make_async_copy(w2_hbm.at[cols, :], w2b.bitcast(bf16).at[cols, :], sems.at[6, t])]

    def cp_o(row, n):
        rows = pl.ds(row, n)
        return pltpu.make_async_copy(obuf.at[rows, :], o_hbm.at[0, rows, :], sems.at[7, 0])

    def gen_forward_dft():
        i32 = jnp.int32
        wrow = lax.broadcasted_iota(i32, (128, 128), 0)
        n4 = (4 * lax.broadcasted_iota(i32, (128, 128), 1)).astype(f32)
        coef, quarter = [], []
        for h in range(2):
            rho = 2 * wrow + h
            rem = rho % (2 * RB)
            r = RB * (rho // (2 * RB)) + rem % RB
            coef.append(_odd_freq(r).astype(f32) * (0.5 / NDFT))
            quarter.append((rem // RB).astype(f32) * 0.25)
        for p in range(4):
            v = [_cos_turns(coef[h] * (n4 + float(p)) + quarter[h]) for h in range(2)]
            mf_ref[p] = _pk2(v[0], v[1])

    def gen_inverse_dft():
        i32 = jnp.int32
        wrow = lax.broadcasted_iota(i32, (64, 256), 0)
        col = lax.broadcasted_iota(i32, (64, 256), 1)
        coef = _odd_freq(col // 2).astype(f32) * (0.5 / NDFT)
        quarter = (col % 2).astype(f32) * 0.25
        for p in range(4):
            v = [_cos_turns(coef * (8 * wrow + (4 * h + p)).astype(f32) + quarter) for h in range(2)]
            gi_ref[p] = _pk2(v[0], v[1])

    def prep_x(g, a, t, wts, mask, inj):
        i0_ = 64 * a + 8 * t
        kb = KPAD + 20 * i0_ + 4 * g
        kl = [kraw[pl.ds(kb + w, 8, stride=20), :] for w in range(4)]
        km2 = kraw[pl.ds(kb - 18, 8, stride=20), :]
        km3 = kraw[pl.ds(kb - 17, 8, stride=20), :]
        e = [_hi(km2), _lo(km3), _hi(km3)]
        for w in range(4):
            e += [_lo(kl[w]), _hi(kl[w])]
        if inj is not None:
            e[3] = jnp.where(mask, inj, e[3])
        vb = 20 * i0_ + 4 * g
        kv = []
        for w in range(4):
            vw = vraw[pl.ds(vb + w, 8, stride=20), :]
            for h, vv in enumerate((_lo(vw), _hi(vw))):
                r = 3 + 2 * w + h
                ks = wts[0] * e[r] + wts[1] * e[r - 1] + wts[2] * e[r - 2] + wts[3] * e[r - 3]
                kv.append(ks * vv)
        tok = None
        for p in range(4):
            pk = _pk2(kv[p], kv[p + 4])
            rx[g, p, pl.ds(8 * t, 8), :] = pk
            tok = pk if tok is None else tok | pk
        return tok

    def prep_k(g, m):
        blk = _bc(skbuf[pl.ds(64 * g, 64), pl.ds(CH * m, CH)])
        ktbuf[g, 0:CH // 2, :] = pltpu.bitcast(blk.T, u32)
        lo16 = jnp.uint32(0xFFFF)
        hi16 = jnp.uint32(0xFFFF0000)
        for t in range(8):
            w = [ktbuf[g, pl.ds(32 * t + e_, 8, stride=4), :] for e_ in range(4)]
            rows = pl.ds(8 * t, 8)
            rk[g, 0, rows, :] = (w[0] & lo16) | (w[2] << 16)
            rk[g, 1, rows, :] = (w[0] >> 16) | (w[2] & hi16)
            rk[g, 2, rows, :] = (w[1] & lo16) | (w[3] << 16)
            rk[g, 3, rows, :] = (w[1] >> 16) | (w[3] & hi16)

    def fwd(src, dst, g, a, b, dvec):
        z = [jnp.dot(_bc(mf_ref[p, pl.ds(RB * b, RB), :]), _bc(src[g, p]),
                     preferred_element_type=f32) for p in range(4)]
        xr, xi = _fft4([t[:RB] for t in z], [t[RB:] for t in z], False)
        for f2 in range(4):
            dst[g, a, f2, 0, pl.ds(RB * b, RB), :] = xr[f2] if dvec is None else xr[f2] + dvec
            dst[g, a, f2, 1, pl.ds(RB * b, RB), :] = xi[f2]

    def cell(g, j, c, mask, inj):
        rows = pl.ds(8 * j, 8)
        zr, zi = [], []
        for f2 in range(4):
            ar = ai = None
            for a in range(c + 1):
                m = c - a
                xr = xh[g, a, f2, 0, rows, :]
                xi = xh[g, a, f2, 1, rows, :]
                kr = kh[g, m, f2, 0, rows, :]
                ki = kh[g, m, f2, 1, rows, :]
                if inj is not None and f2 == 0 and a == 0:
                    kr = jnp.where(mask, inj, kr)
                tr = xr * kr - xi * ki
                ti = xr * ki + xi * kr
                ar = tr if ar is None else ar + tr
                ai = ti if ai is None else ai + ti
            zr.append(ar)
            zi.append(ai)
        yr, yi = zr, zi
        if c > 0:
            pr = [zb[g, f, 0, rows, :] for f in range(4)]
            pi = [zb[g, f, 1, rows, :] for f in range(4)]
            if j < 8:
                yr = [zr[f] - pi[f] for f in range(4)]
                yi = [zi[f] + pr[f] for f in range(4)]
            else:
                yr = [zr[f] + pi[f] for f in range(4)]
                yi = [zi[f] - pr[f] for f in range(4)]
        if c + 1 < NCH:
            for f in range(4):
                zb[g, f, 0, rows, :] = zr[f]
                zb[g, f, 1, rows, :] = zi[f]
        ur, ui = _fft4(yr, yi, True)
        tok = None
        for s2 in range(4):
            pk = _pk2(ur[s2], ui[s2])
            ub[c % 2][g, s2, rows, :] = pk
            tok = pk if tok is None else tok | pk
        return tok

    def inv(g, c, s2):
        y = jnp.dot(_bc(gi_ref[s2]), _bc(ub[c % 2][g, s2, 0:128, :]), preferred_element_type=f32)
        ybuf[g, pl.ds(CH * c + s2, 128, stride=4), :] = y

    def delayed(tok, n):
        t = pltpu.bitcast(tok, f32)
        for _ in range(n):
            t = pl.reciprocal(t, approx=True)
        return t

    def mod_cols(lo_, n):
        cc = c_ref[...].astype(f32)
        sc = (cc * jax.nn.sigmoid(cc)).astype(bf16)
        lhs = jnp.broadcast_to(sc, (8, D))
        modb[:, pl.ds(lo_, n)] = jnp.dot(lhs, _bc(wmb[:, pl.ds(lo_, n)]), preferred_element_type=f32)

    _cnt = [0]

    def first_step():
        i = _cnt[0]
        _cnt[0] += 1
        return zs_ref[i] == 0

    def prologue(row, nchunk):
        sa = modb[0:1, 0 * D:1 * D]
        ca1 = 1.0 + modb[0:1, 1 * D:2 * D]
        ga = modb[0:1, 2 * D:3 * D] * (2.0 / NDFT)
        sb = modb[0:1, 3 * D:4 * D]
        cb1 = 1.0 + modb[0:1, 4 * D:5 * D]
        mask = zero_ref[...] != 0
        n = SB // nchunk
        x1s, h2s = [], []
        tok = None
        for i in range(nchunk):
            r = pl.ds(row + i * n, n)
            q = _bc(qbuf[_half(row + i * n, n), :]).astype(f32)
            if tok is not None:
                q00 = jnp.where(mask, tok, q[0:8, 0:128])
                top = jnp.concatenate([q00, q[0:8, 128:]], axis=1)
                q = jnp.concatenate([top, q[8:]], axis=0)
            y = jnp.concatenate([ybuf[g, r, :] for g in range(NG)], axis=1)
            h1 = _ln(q) * ca1 + sa
            x1 = q + ga * (h1 * y)
            h2f = _ln(x1) * cb1 + sb
            if i + 1 < nchunk:
                parts = [h2f[8 * a:8 * a + 8, 128 * g:128 * (g + 1)]
                         for a in range(n // 8) for g in range(NG)]
                while len(parts) > 1:
                    parts = [parts[k] + parts[k + 1] if k + 1 < len(parts) else parts[k]
                             for k in range(0, len(parts), 2)]
                tok = parts[0]
            x1s.append(x1)
            h2s.append(h2f.astype(bf16))
        return jnp.concatenate(x1s, axis=0), jnp.concatenate(h2s, axis=0)

    def ffn_part(h2, lo_, n):
        cols = pl.ds(lo_, n)
        gate = jnp.dot(h2, _bc(w1b[:, cols]), preferred_element_type=f32)
        up = jnp.dot(h2, _bc(w3b[:, cols]), preferred_element_type=f32)
        act = (gate * jax.nn.sigmoid(gate) * up).astype(bf16)
        return jnp.dot(act, _bc(w2b[_half(lo_, n), :]), preferred_element_type=f32)

    def next_prologue(row, nchunk):
        x1, h2 = prologue(row, nchunk)
        xn[...] = x1
        hn[...] = h2

    @pl.when(first_step())
    def _issue():
        cp_s(0).start(); cp_s(1).start()
        cp_k(0).start(); cp_v(0).start()
        cp_k(1).start(); cp_v(1).start()
        for a in range(2, NCH):
            cp_s(a).start(); cp_k(a).start(); cp_v(a).start()
        cp_wm(0).start()
        cp_wm(1).start()
        cp_q(0).start()
        for t in range(NFC):
            if t == NFC - 1:
                cp_wm(2).start()
            for c_ in cp_w(t):
                c_.start()
        cp_q(1).start()
        kraw[0:KPAD, :] = jnp.zeros((KPAD, 128), u32)
        gen_forward_dft()
        gen_inverse_dft()

    def fwd_k(a):
        dv = dv_ref[...].astype(f32).reshape(1, D)
        for g in range(NG):
            prep_k(g, a)
            dvec = jnp.broadcast_to(dv[:, 128 * g:128 * (g + 1)], (RB, 128)) if a == 0 else None
            for b in range(128 // RB):
                fwd(rk, kh, g, a, b, dvec)

    def fwd_x(a):
        mask = zero_ref[...] != 0
        shk = shk_ref[...].astype(f32)
        inj = None
        for g in range(NG):
            lanes = slice(128 * g, 128 * (g + 1))
            wts = [jnp.broadcast_to(shk[j:j + 1, lanes], (8, 128)) for j in range(4)]
            for t in range(8):
                tok = prep_x(g, a, t, wts, mask, inj)
                inj = delayed(tok, NRCP_P) if g > 0 else None
            for b in range(128 // RB):
                fwd(rx, xh, g, a, b, None)

    def part_b(c):
        mask = zero_ref[...] != 0
        inj = None
        for g in range(NG):
            for j in range(16):
                tok = cell(g, j, c, mask, inj)
                if RCP_B[c] is not None:
                    n = 16 * g + j
                    inj = delayed(tok, int((n + 1) * RCP_B[c]) - int(n * RCP_B[c]))
        if c > 0:
            for g in range(NG):
                for s2 in range(4):
                    inv(g, c - 1, s2)

    for a in range(2):
        @pl.when(first_step())
        def _filter_side(a=a):
            cp_s(a).wait()
            fwd_k(a)

    for a in range(NCH):
        @pl.when(first_step())
        def _data_side(a=a):
            cp_k(a).wait(); cp_v(a).wait()
            fwd_x(a)

        if a + 1 < NCH:
            @pl.when(first_step())
            def _products(c=a):
                if c >= 1:
                    cp_s(c + 1).wait()
                part_b(c)
                if c >= 1:
                    fwd_k(c + 1)

    @pl.when(first_step())
    def _products_last():
        cp_wm(0).wait()
        part_b(NCH - 1)
        mod_cols(0, WM0)

    @pl.when(first_step())
    def _finish_conv():
        cp_wm(1).wait()
        cp_q(0).wait()
        mod_cols(WM0, 5 * D - WM0)
        for g in range(NG):
            for s2 in range(4):
                inv(g, NCH - 1, s2)
        x1, h2 = prologue(0, 1)
        xs[0:SB, :] = x1
        hs[0:SB, :] = h2

    for t in range(NFC):
        @pl.when(first_step())
        def _first_rows(t=t):
            for c_ in cp_w(t):
                c_.wait()
            if t == NFC - 1:
                cp_wm(2).wait()
                cp_q(1).wait()
                mod_cols(5 * D, D)
            for j in range(NSB):
                r = pl.ds(j * SB, SB)
                if t == 0:
                    if j == 0:
                        h2 = hs[r, :]
                    else:
                        x1, h2 = prologue(j * SB, PCH_FIRST)
                        xs[r, :] = x1
                        hs[r, :] = h2
                    accs[r, :] = ffn_part(h2, FLO[0], FCS[0])
                elif t < NFC - 1:
                    accs[r, :] += ffn_part(hs[r, :], FLO[t], FCS[t])
                else:
                    gb = modb[0:1, 5 * D:6 * D]
                    ffn = accs[r, :] + ffn_part(hs[r, :], FLO[t], FCS[t])
                    obuf[r, :] = (xs[r, :] + gb * ffn).astype(bf16)
            if t == NFC - 1:
                next_prologue(BM, PCH_STEADY)
                cp_o(0, BM).start()

    def _step(step, carry):
        gb = modb[0:1, 5 * D:6 * D]
        row0 = pl.multiple_of(BM + step * BM2, SB)
        nsb = BM2 // SB
        x1, h2 = xn[...], hn[...]
        for j in range(nsb):
            if j + 1 < nsb:
                nxt = prologue(row0 + (j + 1) * SB, PCH_STEADY)
            else:
                nrow = jnp.minimum(row0 + BM2, S - SB)
                next_prologue(pl.multiple_of(nrow, SB), PCH_STEADY)
            ffn = ffn_part(h2, 0, F)
            obuf[pl.ds(row0 + j * SB, SB), :] = (x1 + gb * ffn).astype(bf16)
            cp_o(row0 + j * SB, SB).start()
            if j + 1 < nsb:
                x1, h2 = nxt
        return carry

    lax.fori_loop(0, NSTEP2, _step, 0)
    cp_o(0, BM).wait()
    for i in range((S - BM) // SB):
        cp_o(BM + i * SB, SB).wait()


def _raw_view(x):
    return x.reshape(S // 8, 8, NG, 128).transpose(0, 2, 1, 3).reshape(NG * S, 128)


@jax.jit
def pallas_adaLN_cond__ssm_conv_h3__glu_gated_swiglu__prompt_kernel(
    A_q: jax.Array,
    A_k: jax.Array,
    A_v: jax.Array,
    A_shift_k: jax.Array,
    A_ssm_k: jax.Array,
    A_ssm_D: jax.Array,
    B_x: jax.Array,
    B_w1: jax.Array,
    B_w3: jax.Array,
    B_w2: jax.Array,
    c: jax.Array,
    w_mod: jax.Array,
):
    del B_x
    any_spec = pl.BlockSpec(memory_space=pl.ANY)
    vmem_spec = pl.BlockSpec(memory_space=pltpu.VMEM)
    scratch = [
        pltpu.VMEM((KPAD + 5 * S // 2 + 24, 128), u32),
        pltpu.VMEM((5 * S // 2 + 24, 128), u32),
        pltpu.VMEM((D // 2, S), u32),
        pltpu.VMEM((NG, CH // 2 + 8, 128), u32),
        pltpu.VMEM((NG, 4, 64, 128), u32),
        pltpu.VMEM((NG, 4, 64, 128), u32),
        pltpu.VMEM((NG, NCH, 4, 2, PR, 128), f32),
        pltpu.VMEM((NG, NCH, 4, 2, PR, 128), f32),
        pltpu.VMEM((NG, 4, 2, PR, 128), f32),
        pltpu.VMEM((NG, 4, PR, 128), u32),
        pltpu.VMEM((NG, 4, PR, 128), u32),
        pltpu.VMEM((NG, S + 8, 128), f32),
        pltpu.VMEM((S // 2, D), u32),
        pltpu.VMEM((D // 2, F), u32),
        pltpu.VMEM((D // 2, F), u32),
        pltpu.VMEM((F // 2, D), u32),
        pltpu.VMEM((D // 2, 6 * D), u32),
        pltpu.VMEM((8, 6 * D), f32),
        pltpu.VMEM((SB, D), bf16),
        pltpu.VMEM((SB, D), f32),
        pltpu.VMEM((BM, D), bf16),
        pltpu.VMEM((BM, D), f32),
        pltpu.VMEM((BM, D), f32),
        pltpu.VMEM((S, D), bf16),
        pltpu.VMEM((4, 128, 128), u32),
        pltpu.VMEM((4, 64, 256), u32),
        pltpu.SemaphoreType.DMA((8, 8)),
    ]
    return pl.pallas_call(
        _kernel,
        in_specs=[any_spec] * 8 + [vmem_spec] * 4 + [pl.BlockSpec(memory_space=pltpu.SMEM)],
        out_specs=any_spec,
        out_shape=jax.ShapeDtypeStruct((1, S, D), bf16),
        scratch_shapes=scratch,
        compiler_params=pltpu.CompilerParams(
            vmem_limit_bytes=100 * 1024 * 1024),
    )(A_q, _raw_view(A_k), _raw_view(A_v), A_ssm_k, B_w1, B_w3, B_w2, w_mod,
      A_shift_k.T, A_ssm_D, c,
      jnp.zeros((8, 128), jnp.uint32), jnp.zeros((32,), jnp.int32))
```

```python
import jax
import jax.numpy as jnp
from jax import lax
import jax.experimental.pallas as pl
import jax.experimental.pallas.tpu as pltpu

f32 = jnp.float32
bf16 = jnp.bfloat16
u32 = jnp.uint32

S = 2048
D = 640
F = 1536
NG = D // 128
NCH = 4
CH = S // NCH
NDFT = 2 * CH
EPS = 1e-5

SB = 128
BM = 512
NSB = BM // SB
BM2 = 256
NSTEP2 = (S - BM) // BM2
FCS = (256, 640, 640)
NFC = len(FCS)
FLO = tuple(sum(FCS[:i]) for i in range(NFC))
WM0 = 1920

KPAD = 40
RB = 32
PR = 136

PCH_FIRST, PCH_STEADY = 2, 8
NRCP_P = 1
RCP_B = (None, 1.7, 1.5, 2.05)


def _cos_turns(x):
    fr = x - jnp.floor(x)
    w = 4.0 * jnp.minimum(fr, 1.0 - fr) - 1.0
    w2 = w * w
    acc = jnp.float32(3.598843e-06)
    for coef in (-1.6044118e-04, 4.6817541e-03, -7.9692626e-02, 6.4596410e-01, -1.5707963e+00):
        acc = acc * w2 + jnp.float32(coef)
    return acc * w


def _odd_freq(r):
    return jnp.where(r < 64, 4 * r + 1, 4 * (r - 64) + 3)


def _bc(v):
    return pltpu.bitcast(v, bf16)


def _half(row, n):
    if isinstance(row, int):
        return pl.ds(row // 2, n // 2)
    return pl.ds(pl.multiple_of(row // 2, 8), n // 2)


def _lo(w):
    return pltpu.bitcast(w << 16, f32)


def _hi(w):
    return pltpu.bitcast(w & jnp.uint32(0xFFFF0000), f32)


def _pk2(a, b):
    return pltpu.bitcast(pltpu.pack_elementwise([a, b], packed_dtype=bf16), u32)


def _fft4(zr, zi, inv):
    ar, ai = zr[0] + zr[2], zi[0] + zi[2]
    br, bi = zr[0] - zr[2], zi[0] - zi[2]
    cr, ci = zr[1] + zr[3], zi[1] + zi[3]
    dr, di = zr[1] - zr[3], zi[1] - zi[3]
    if not inv:
        return [ar + cr, br + di, ar - cr, br - di], [ai + ci, bi - dr, ai - ci, bi + dr]
    return [ar + cr, br - di, ar - cr, br + di], [ai + ci, bi + dr, ai - ci, bi - dr]


def _ln(x):
    m = jnp.sum(x, axis=-1, keepdims=True) * (1.0 / D)
    xc = x - m
    v = jnp.sum(xc * xc, axis=-1, keepdims=True) * (1.0 / D)
    return xc * lax.rsqrt(v + EPS)


def _kernel(q_hbm, k_hbm, v_hbm, sk_hbm, w1_hbm, w3_hbm, w2_hbm, wm_hbm,
            shk_hbm, dv_hbm, c_hbm, zero_hbm, zs_hbm,
            o_hbm,
            kraw, vraw, skbuf, ktbuf, rx, rk, xh, kh, zb, ub0, ub1, ybuf,
            qbuf, w1b, w3b, w2b, wmb, modb, hn, xn, hs, xs, accs, obuf, mf_ref, gi_ref,
            shk_ref, dv_ref, c_ref, zero_ref, zs_ref, sems):
    ub = (ub0, ub1)

    def cp_k(a):
        return pltpu.make_async_copy(
            k_hbm.at[pl.ds(5 * CH * a, 5 * CH), :],
            kraw.bitcast(bf16).at[pl.ds(2 * KPAD + 5 * CH * a, 5 * CH), :], sems.at[0, a])

    def cp_v(a):
        return pltpu.make_async_copy(
            v_hbm.at[pl.ds(5 * CH * a, 5 * CH), :],
            vraw.bitcast(bf16).at[pl.ds(5 * CH * a, 5 * CH), :], sems.at[1, a])

    def cp_s(a):
        cols = pl.ds(CH * a, CH)
        return pltpu.make_async_copy(sk_hbm.at[:, cols], skbuf.bitcast(bf16).at[:, cols], sems.at[2, a])

    def cp_wm(i):
        cols = [pl.ds(0, WM0), pl.ds(WM0, 5 * D - WM0), pl.ds(5 * D, D)][i]
        return pltpu.make_async_copy(wm_hbm.at[:, cols], wmb.bitcast(bf16).at[:, cols], sems.at[3, i])

    def cp_q(i):
        rows = pl.ds(0, BM) if i == 0 else pl.ds(BM, S - BM)
        return pltpu.make_async_copy(q_hbm.at[0, rows, :], qbuf.bitcast(bf16).at[rows, :], sems.at[3, 4 + i])

    def cp_w(t):
        cols = pl.ds(FLO[t], FCS[t])
        return [pltpu.make_async_copy(w1_hbm.at[:, cols], w1b.bitcast(bf16).at[:, cols], sems.at[4, t]),
                pltpu.make_async_copy(w3_hbm.at[:, cols], w3b.bitcast(bf16).at[:, cols], sems.at[5, t]),
                pltpu.make_async_copy(w2_hbm.at[cols, :], w2b.bitcast(bf16).at[cols, :], sems.at[6, t])]

    small = [pltpu.make_async_copy(src, dst, sems.at[7, 1 + i]) for i, (src, dst) in enumerate(
        [(zs_hbm, zs_ref), (zero_hbm, zero_ref), (dv_hbm, dv_ref), (shk_hbm, shk_ref), (c_hbm, c_ref)])]

    def cp_o(row, n):
        rows = pl.ds(row, n)
        return pltpu.make_async_copy(obuf.at[rows, :], o_hbm.at[0, rows, :], sems.at[7, 0])

    def gen_forward_dft():
        i32 = jnp.int32
        wrow = lax.broadcasted_iota(i32, (128, 128), 0)
        n4 = (4 * lax.broadcasted_iota(i32, (128, 128), 1)).astype(f32)
        coef, quarter = [], []
        for h in range(2):
            rho = 2 * wrow + h
            rem = rho % (2 * RB)
            r = RB * (rho // (2 * RB)) + rem % RB
            coef.append(_odd_freq(r).astype(f32) * (0.5 / NDFT))
            quarter.append((rem // RB).astype(f32) * 0.25)
        for p in range(4):
            v = [_cos_turns(coef[h] * (n4 + float(p)) + quarter[h]) for h in range(2)]
            mf_ref[p] = _pk2(v[0], v[1])

    def gen_inverse_dft():
        i32 = jnp.int32
        wrow = lax.broadcasted_iota(i32, (64, 256), 0)
        col = lax.broadcasted_iota(i32, (64, 256), 1)
        coef = _odd_freq(col // 2).astype(f32) * (0.5 / NDFT)
        quarter = (col % 2).astype(f32) * 0.25
        for p in range(4):
            v = [_cos_turns(coef * (8 * wrow + (4 * h + p)).astype(f32) + quarter) for h in range(2)]
            gi_ref[p] = _pk2(v[0], v[1])

    def prep_x(g, a, t, wts, mask, inj):
        i0_ = 64 * a + 8 * t
        kb = KPAD + 20 * i0_ + 4 * g
        kl = [kraw[pl.ds(kb + w, 8, stride=20), :] for w in range(4)]
        km2 = kraw[pl.ds(kb - 18, 8, stride=20), :]
        km3 = kraw[pl.ds(kb - 17, 8, stride=20), :]
        e = [_hi(km2), _lo(km3), _hi(km3)]
        for w in range(4):
            e += [_lo(kl[w]), _hi(kl[w])]
        if inj is not None:
            e[3] = jnp.where(mask, inj, e[3])
        vb = 20 * i0_ + 4 * g
        kv = []
        for w in range(4):
            vw = vraw[pl.ds(vb + w, 8, stride=20), :]
            for h, vv in enumerate((_lo(vw), _hi(vw))):
                r = 3 + 2 * w + h
                ks = wts[0] * e[r] + wts[1] * e[r - 1] + wts[2] * e[r - 2] + wts[3] * e[r - 3]
                kv.append(ks * vv)
        tok = None
        for p in range(4):
            pk = _pk2(kv[p], kv[p + 4])
            rx[g, p, pl.ds(8 * t, 8), :] = pk
            tok = pk if tok is None else tok | pk
        return tok

    def prep_k(g, m):
        blk = _bc(skbuf[pl.ds(64 * g, 64), pl.ds(CH * m, CH)])
        ktbuf[g, 0:CH // 2, :] = pltpu.bitcast(blk.T, u32)
        lo16 = jnp.uint32(0xFFFF)
        hi16 = jnp.uint32(0xFFFF0000)
        for t in range(8):
            w = [ktbuf[g, pl.ds(32 * t + e_, 8, stride=4), :] for e_ in range(4)]
            rows = pl.ds(8 * t, 8)
            rk[g, 0, rows, :] = (w[0] & lo16) | (w[2] << 16)
            rk[g, 1, rows, :] = (w[0] >> 16) | (w[2] & hi16)
            rk[g, 2, rows, :] = (w[1] & lo16) | (w[3] << 16)
            rk[g, 3, rows, :] = (w[1] >> 16) | (w[3] & hi16)

    def fwd(src, dst, g, a, b, dvec):
        z = [jnp.dot(_bc(mf_ref[p, pl.ds(RB * b, RB), :]), _bc(src[g, p]),
                     preferred_element_type=f32) for p in range(4)]
        xr, xi = _fft4([t[:RB] for t in z], [t[RB:] for t in z], False)
        for f2 in range(4):
            dst[g, a, f2, 0, pl.ds(RB * b, RB), :] = xr[f2] if dvec is None else xr[f2] + dvec
            dst[g, a, f2, 1, pl.ds(RB * b, RB), :] = xi[f2]

    def cell(g, j, c, mask, inj):
        rows = pl.ds(8 * j, 8)
        zr, zi = [], []
        for f2 in range(4):
            ar = ai = None
            for a in range(c + 1):
                m = c - a
                xr = xh[g, a, f2, 0, rows, :]
                xi = xh[g, a, f2, 1, rows, :]
                kr = kh[g, m, f2, 0, rows, :]
                ki = kh[g, m, f2, 1, rows, :]
                if inj is not None and f2 == 0 and a == 0:
                    kr = jnp.where(mask, inj, kr)
                tr = xr * kr - xi * ki
                ti = xr * ki + xi * kr
                ar = tr if ar is None else ar + tr
                ai = ti if ai is None else ai + ti
            zr.append(ar)
            zi.append(ai)
        yr, yi = zr, zi
        if c > 0:
            pr = [zb[g, f, 0, rows, :] for f in range(4)]
            pi = [zb[g, f, 1, rows, :] for f in range(4)]
            if j < 8:
                yr = [zr[f] - pi[f] for f in range(4)]
                yi = [zi[f] + pr[f] for f in range(4)]
            else:
                yr = [zr[f] + pi[f] for f in range(4)]
                yi = [zi[f] - pr[f] for f in range(4)]
        if c + 1 < NCH:
            for f in range(4):
                zb[g, f, 0, rows, :] = zr[f]
                zb[g, f, 1, rows, :] = zi[f]
        ur, ui = _fft4(yr, yi, True)
        tok = None
        for s2 in range(4):
            pk = _pk2(ur[s2], ui[s2])
            ub[c % 2][g, s2, rows, :] = pk
            tok = pk if tok is None else tok | pk
        return tok

    def inv(g, c, s2):
        y = jnp.dot(_bc(gi_ref[s2]), _bc(ub[c % 2][g, s2, 0:128, :]), preferred_element_type=f32)
        ybuf[g, pl.ds(CH * c + s2, 128, stride=4), :] = y

    def delayed(tok, n):
        t = pltpu.bitcast(tok, f32)
        for _ in range(n):
            t = pl.reciprocal(t, approx=True)
        return t

    def mod_cols(lo_, n):
        cc = c_ref[...].astype(f32)
        sc = (cc * jax.nn.sigmoid(cc)).astype(bf16)
        lhs = jnp.broadcast_to(sc, (8, D))
        modb[:, pl.ds(lo_, n)] = jnp.dot(lhs, _bc(wmb[:, pl.ds(lo_, n)]), preferred_element_type=f32)

    _cnt = [0]

    def first_step():
        i = _cnt[0]
        _cnt[0] += 1
        return zs_ref[i] == 0

    def prologue(row, nchunk):
        sa = modb[0:1, 0 * D:1 * D]
        ca1 = 1.0 + modb[0:1, 1 * D:2 * D]
        ga = modb[0:1, 2 * D:3 * D] * (2.0 / NDFT)
        sb = modb[0:1, 3 * D:4 * D]
        cb1 = 1.0 + modb[0:1, 4 * D:5 * D]
        mask = zero_ref[...] != 0
        n = SB // nchunk
        x1s, h2s = [], []
        tok = None
        for i in range(nchunk):
            r = pl.ds(row + i * n, n)
            q = _bc(qbuf[_half(row + i * n, n), :]).astype(f32)
            if tok is not None:
                q00 = jnp.where(mask, tok, q[0:8, 0:128])
                top = jnp.concatenate([q00, q[0:8, 128:]], axis=1)
                q = jnp.concatenate([top, q[8:]], axis=0)
            y = jnp.concatenate([ybuf[g, r, :] for g in range(NG)], axis=1)
            h1 = _ln(q) * ca1 + sa
            x1 = q + ga * (h1 * y)
            h2f = _ln(x1) * cb1 + sb
            if i + 1 < nchunk:
                parts = [h2f[8 * a:8 * a + 8, 128 * g:128 * (g + 1)]
                         for a in range(n // 8) for g in range(NG)]
                while len(parts) > 1:
                    parts = [parts[k] + parts[k + 1] if k + 1 < len(parts) else parts[k]
                             for k in range(0, len(parts), 2)]
                tok = parts[0]
            x1s.append(x1)
            h2s.append(h2f.astype(bf16))
        return jnp.concatenate(x1s, axis=0), jnp.concatenate(h2s, axis=0)

    def ffn_part(h2, lo_, n):
        cols = pl.ds(lo_, n)
        gate = jnp.dot(h2, _bc(w1b[:, cols]), preferred_element_type=f32)
        up = jnp.dot(h2, _bc(w3b[:, cols]), preferred_element_type=f32)
        act = (gate * jax.nn.sigmoid(gate) * up).astype(bf16)
        return jnp.dot(act, _bc(w2b[_half(lo_, n), :]), preferred_element_type=f32)

    def next_prologue(row, nchunk):
        x1, h2 = prologue(row, nchunk)
        xn[...] = x1
        hn[...] = h2

    cp_s(0).start()
    for c_ in small:
        c_.start()
    cp_s(1).start()
    cp_k(0).start(); cp_v(0).start()
    cp_k(1).start(); cp_v(1).start()
    for a in range(2, NCH):
        cp_s(a).start(); cp_k(a).start(); cp_v(a).start()
    cp_wm(0).start()
    cp_wm(1).start()
    cp_q(0).start()
    for t in range(NFC):
        if t == NFC - 1:
            cp_wm(2).start()
        for c_ in cp_w(t):
            c_.start()
    cp_q(1).start()
    kraw[0:KPAD, :] = jnp.zeros((KPAD, 128), u32)
    gen_forward_dft()
    gen_inverse_dft()
    for c_ in small:
        c_.wait()

    def fwd_k(a):
        dv = dv_ref[...].astype(f32).reshape(1, D)
        for g in range(NG):
            prep_k(g, a)
            dvec = jnp.broadcast_to(dv[:, 128 * g:128 * (g + 1)], (RB, 128)) if a == 0 else None
            for b in range(128 // RB):
                fwd(rk, kh, g, a, b, dvec)

    def fwd_x(a):
        mask = zero_ref[...] != 0
        shk = shk_ref[...].astype(f32)
        inj = None
        for g in range(NG):
            lanes = slice(128 * g, 128 * (g + 1))
            wts = [jnp.broadcast_to(shk[j:j + 1, lanes], (8, 128)) for j in range(4)]
            for t in range(8):
                tok = prep_x(g, a, t, wts, mask, inj)
                inj = delayed(tok, NRCP_P) if g > 0 else None
            for b in range(128 // RB):
                fwd(rx, xh, g, a, b, None)

    def part_b(c):
        mask = zero_ref[...] != 0
        inj = None
        for g in range(NG):
            for j in range(16):
                tok = cell(g, j, c, mask, inj)
                if RCP_B[c] is not None:
                    n = 16 * g + j
                    inj = delayed(tok, int((n + 1) * RCP_B[c]) - int(n * RCP_B[c]))
        if c > 0:
            for g in range(NG):
                for s2 in range(4):
                    inv(g, c - 1, s2)

    for a in range(2):
        @pl.when(first_step())
        def _filter_side(a=a):
            cp_s(a).wait()
            fwd_k(a)

    for a in range(NCH):
        @pl.when(first_step())
        def _data_side(a=a):
            cp_k(a).wait(); cp_v(a).wait()
            fwd_x(a)

        if a + 1 < NCH:
            @pl.when(first_step())
            def _products(c=a):
                if c >= 1:
                    cp_s(c + 1).wait()
                part_b(c)
                if c >= 1:
                    fwd_k(c + 1)

    @pl.when(first_step())
    def _products_last():
        cp_wm(0).wait()
        part_b(NCH - 1)
        mod_cols(0, WM0)

    @pl.when(first_step())
    def _finish_conv():
        cp_wm(1).wait()
        cp_q(0).wait()
        mod_cols(WM0, 5 * D - WM0)
        for g in range(NG):
            for s2 in range(4):
                inv(g, NCH - 1, s2)
        x1, h2 = prologue(0, 1)
        xs[0:SB, :] = x1
        hs[0:SB, :] = h2

    for t in range(NFC):
        @pl.when(first_step())
        def _first_rows(t=t):
            for c_ in cp_w(t):
                c_.wait()
            if t == NFC - 1:
                cp_wm(2).wait()
                cp_q(1).wait()
                mod_cols(5 * D, D)
            for j in range(NSB):
                r = pl.ds(j * SB, SB)
                if t == 0:
                    if j == 0:
                        h2 = hs[r, :]
                    else:
                        x1, h2 = prologue(j * SB, PCH_FIRST)
                        xs[r, :] = x1
                        hs[r, :] = h2
                    accs[r, :] = ffn_part(h2, FLO[0], FCS[0])
                elif t < NFC - 1:
                    accs[r, :] += ffn_part(hs[r, :], FLO[t], FCS[t])
                else:
                    gb = modb[0:1, 5 * D:6 * D]
                    ffn = accs[r, :] + ffn_part(hs[r, :], FLO[t], FCS[t])
                    obuf[r, :] = (xs[r, :] + gb * ffn).astype(bf16)
            if t == NFC - 1:
                next_prologue(BM, PCH_STEADY)
                cp_o(0, BM).start()

    def _step(step, carry):
        gb = modb[0:1, 5 * D:6 * D]
        row0 = pl.multiple_of(BM + step * BM2, SB)
        nsb = BM2 // SB
        x1, h2 = xn[...], hn[...]
        for j in range(nsb):
            if j + 1 < nsb:
                nxt = prologue(row0 + (j + 1) * SB, PCH_STEADY)
            else:
                nrow = jnp.minimum(row0 + BM2, S - SB)
                next_prologue(pl.multiple_of(nrow, SB), PCH_STEADY)
            ffn = ffn_part(h2, 0, F)
            obuf[pl.ds(row0 + j * SB, SB), :] = (x1 + gb * ffn).astype(bf16)
            cp_o(row0 + j * SB, SB).start()
            if j + 1 < nsb:
                x1, h2 = nxt
        return carry

    lax.fori_loop(0, NSTEP2, _step, 0)
    cp_o(0, BM).wait()
    for i in range((S - BM) // SB):
        cp_o(BM + i * SB, SB).wait()


def _raw_view(x):
    return x.reshape(S // 8, 8, NG, 128).transpose(0, 2, 1, 3).reshape(NG * S, 128)


@jax.jit
def pallas_adaLN_cond__ssm_conv_h3__glu_gated_swiglu__prompt_kernel(
    A_q: jax.Array,
    A_k: jax.Array,
    A_v: jax.Array,
    A_shift_k: jax.Array,
    A_ssm_k: jax.Array,
    A_ssm_D: jax.Array,
    B_x: jax.Array,
    B_w1: jax.Array,
    B_w3: jax.Array,
    B_w2: jax.Array,
    c: jax.Array,
    w_mod: jax.Array,
):
    del B_x
    any_spec = pl.BlockSpec(memory_space=pl.ANY)
    scratch = [
        pltpu.VMEM((KPAD + 5 * S // 2 + 24, 128), u32),
        pltpu.VMEM((5 * S // 2 + 24, 128), u32),
        pltpu.VMEM((D // 2, S), u32),
        pltpu.VMEM((NG, CH // 2 + 8, 128), u32),
        pltpu.VMEM((NG, 4, 64, 128), u32),
        pltpu.VMEM((NG, 4, 64, 128), u32),
        pltpu.VMEM((NG, NCH, 4, 2, PR, 128), f32),
        pltpu.VMEM((NG, NCH, 4, 2, PR, 128), f32),
        pltpu.VMEM((NG, 4, 2, PR, 128), f32),
        pltpu.VMEM((NG, 4, PR, 128), u32),
        pltpu.VMEM((NG, 4, PR, 128), u32),
        pltpu.VMEM((NG, S + 8, 128), f32),
        pltpu.VMEM((S // 2, D), u32),
        pltpu.VMEM((D // 2, F), u32),
        pltpu.VMEM((D // 2, F), u32),
        pltpu.VMEM((F // 2, D), u32),
        pltpu.VMEM((D // 2, 6 * D), u32),
        pltpu.VMEM((8, 6 * D), f32),
        pltpu.VMEM((SB, D), bf16),
        pltpu.VMEM((SB, D), f32),
        pltpu.VMEM((BM, D), bf16),
        pltpu.VMEM((BM, D), f32),
        pltpu.VMEM((BM, D), f32),
        pltpu.VMEM((S, D), bf16),
        pltpu.VMEM((4, 128, 128), u32),
        pltpu.VMEM((4, 64, 256), u32),
        pltpu.VMEM((4, D), bf16),
        pltpu.VMEM((D,), bf16),
        pltpu.VMEM((1, D), bf16),
        pltpu.VMEM((8, 128), u32),
        pltpu.SMEM((32,), jnp.int32),
        pltpu.SemaphoreType.DMA((8, 8)),
    ]
    return pl.pallas_call(
        _kernel,
        in_specs=[any_spec] * 13,
        out_specs=any_spec,
        out_shape=jax.ShapeDtypeStruct((1, S, D), bf16),
        scratch_shapes=scratch,
        compiler_params=pltpu.CompilerParams(
            vmem_limit_bytes=100 * 1024 * 1024,
            disable_semaphore_checks=True,
            disable_bounds_checks=True),
    )(A_q, _raw_view(A_k), _raw_view(A_v), A_ssm_k, B_w1, B_w3, B_w2, w_mod,
      A_shift_k.T, A_ssm_D, c,
      jnp.zeros((8, 128), jnp.uint32), jnp.zeros((32,), jnp.int32))
```

```python
import jax
import jax.numpy as jnp
from jax import lax
import jax.experimental.pallas as pl
import jax.experimental.pallas.tpu as pltpu

f32 = jnp.float32
bf16 = jnp.bfloat16
u32 = jnp.uint32

S = 2048
D = 640
F = 1536
NG = D // 128
NCH = 4
CH = S // NCH
NDFT = 2 * CH
EPS = 1e-5

SB = 128
BM = 512
NSB = BM // SB
BM2 = 256
NSTEP2 = (S - BM) // BM2
FCS = (256, 640, 640)
NFC = len(FCS)
FLO = tuple(sum(FCS[:i]) for i in range(NFC))
WM0 = 1920

KPAD = 40
RB = 32
PR = 136

PCH_FIRST, PCH_STEADY = 2, 8
NRCP_P = 1
RCP_B = (None, 1.7, 1.5, 2.05)


def _cos_turns(x):
    fr = x - jnp.floor(x)
    w = 4.0 * jnp.minimum(fr, 1.0 - fr) - 1.0
    w2 = w * w
    acc = jnp.float32(3.598843e-06)
    for coef in (-1.6044118e-04, 4.6817541e-03, -7.9692626e-02, 6.4596410e-01, -1.5707963e+00):
        acc = acc * w2 + jnp.float32(coef)
    return acc * w


def _odd_freq(r):
    return jnp.where(r < 64, 4 * r + 1, 4 * (r - 64) + 3)


def _bc(v):
    return pltpu.bitcast(v, bf16)


def _half(row, n):
    if isinstance(row, int):
        return pl.ds(row // 2, n // 2)
    return pl.ds(pl.multiple_of(row // 2, 8), n // 2)


def _lo(w):
    return pltpu.bitcast(w << 16, f32)


def _hi(w):
    return pltpu.bitcast(w & jnp.uint32(0xFFFF0000), f32)


def _pk2(a, b):
    return pltpu.bitcast(pltpu.pack_elementwise([a, b], packed_dtype=bf16), u32)


def _fft4(zr, zi, inv):
    ar, ai = zr[0] + zr[2], zi[0] + zi[2]
    br, bi = zr[0] - zr[2], zi[0] - zi[2]
    cr, ci = zr[1] + zr[3], zi[1] + zi[3]
    dr, di = zr[1] - zr[3], zi[1] - zi[3]
    if not inv:
        return [ar + cr, br + di, ar - cr, br - di], [ai + ci, bi - dr, ai - ci, bi + dr]
    return [ar + cr, br - di, ar - cr, br + di], [ai + ci, bi + dr, ai - ci, bi - dr]


def _ln(x):
    m = jnp.sum(x, axis=-1, keepdims=True) * (1.0 / D)
    xc = x - m
    v = jnp.sum(xc * xc, axis=-1, keepdims=True) * (1.0 / D)
    return xc * lax.rsqrt(v + EPS)


def _kernel(q_hbm, k_hbm, v_hbm, sk_hbm, w1_hbm, w3_hbm, w2_hbm, wm_hbm,
            shk_hbm, dv_hbm, c_hbm, zs_hbm,
            o_hbm,
            kraw, vraw, skbuf, ktbuf, rx, rk, xh, kh, zb, ub0, ub1, ybuf,
            qbuf, w1b, w3b, w2b, wmb, modb, hn, xn, hs, xs, accs, obuf, mf_ref, gi_ref,
            shk_ref, dv_ref, c_ref, zs_ref, sems):
    ub = (ub0, ub1)

    def cp_k(a):
        return pltpu.make_async_copy(
            k_hbm.at[pl.ds(5 * CH * a, 5 * CH), :],
            kraw.bitcast(bf16).at[pl.ds(2 * KPAD + 5 * CH * a, 5 * CH), :], sems.at[0, a])

    def cp_v(a):
        return pltpu.make_async_copy(
            v_hbm.at[pl.ds(5 * CH * a, 5 * CH), :],
            vraw.bitcast(bf16).at[pl.ds(5 * CH * a, 5 * CH), :], sems.at[1, a])

    def cp_s(a):
        cols = pl.ds(CH * a, CH)
        return pltpu.make_async_copy(sk_hbm.at[:, cols], skbuf.bitcast(bf16).at[:, cols], sems.at[2, a])

    def cp_wm(i):
        cols = [pl.ds(0, WM0), pl.ds(WM0, 5 * D - WM0), pl.ds(5 * D, D)][i]
        return pltpu.make_async_copy(wm_hbm.at[:, cols], wmb.bitcast(bf16).at[:, cols], sems.at[3, i])

    def cp_q(i):
        rows = pl.ds(0, BM) if i == 0 else pl.ds(BM, S - BM)
        return pltpu.make_async_copy(q_hbm.at[0, rows, :], qbuf.bitcast(bf16).at[rows, :], sems.at[3, 4 + i])

    def cp_w(t):
        cols = pl.ds(FLO[t], FCS[t])
        return [pltpu.make_async_copy(w1_hbm.at[:, cols], w1b.bitcast(bf16).at[:, cols], sems.at[4, t]),
                pltpu.make_async_copy(w3_hbm.at[:, cols], w3b.bitcast(bf16).at[:, cols], sems.at[5, t]),
                pltpu.make_async_copy(w2_hbm.at[cols, :], w2b.bitcast(bf16).at[cols, :], sems.at[6, t])]

    cp_zs, cp_dv, cp_shk, cp_c = [
        pltpu.make_async_copy(src, dst, sems.at[7, 1 + i]) for i, (src, dst) in enumerate(
            [(zs_hbm, zs_ref), (dv_hbm, dv_ref), (shk_hbm, shk_ref), (c_hbm, c_ref)])]

    def false_mask():
        return jnp.full((8, 128), zs_ref[31], jnp.int32) != 0

    def cp_o(row, n):
        rows = pl.ds(row, n)
        return pltpu.make_async_copy(obuf.at[rows, :], o_hbm.at[0, rows, :], sems.at[7, 0])

    def gen_forward_dft():
        i32 = jnp.int32
        wrow = lax.broadcasted_iota(i32, (128, 128), 0)
        n4 = (4 * lax.broadcasted_iota(i32, (128, 128), 1)).astype(f32)
        coef, quarter = [], []
        for h in range(2):
            rho = 2 * wrow + h
            rem = rho % (2 * RB)
            r = RB * (rho // (2 * RB)) + rem % RB
            coef.append(_odd_freq(r).astype(f32) * (0.5 / NDFT))
            quarter.append((rem // RB).astype(f32) * 0.25)
        for p in range(4):
            v = [_cos_turns(coef[h] * (n4 + float(p)) + quarter[h]) for h in range(2)]
            mf_ref[p] = _pk2(v[0], v[1])

    def gen_inverse_dft():
        i32 = jnp.int32
        wrow = lax.broadcasted_iota(i32, (64, 256), 0)
        col = lax.broadcasted_iota(i32, (64, 256), 1)
        coef = _odd_freq(col // 2).astype(f32) * (0.5 / NDFT)
        quarter = (col % 2).astype(f32) * 0.25
        for p in range(4):
            v = [_cos_turns(coef * (8 * wrow + (4 * h + p)).astype(f32) + quarter) for h in range(2)]
            gi_ref[p] = _pk2(v[0], v[1])

    def prep_x(g, a, t, wts, mask, inj):
        i0_ = 64 * a + 8 * t
        kb = KPAD + 20 * i0_ + 4 * g
        kl = [kraw[pl.ds(kb + w, 8, stride=20), :] for w in range(4)]
        km2 = kraw[pl.ds(kb - 18, 8, stride=20), :]
        km3 = kraw[pl.ds(kb - 17, 8, stride=20), :]
        e = [_hi(km2), _lo(km3), _hi(km3)]
        for w in range(4):
            e += [_lo(kl[w]), _hi(kl[w])]
        if inj is not None:
            e[3] = jnp.where(mask, inj, e[3])
        vb = 20 * i0_ + 4 * g
        kv = []
        for w in range(4):
            vw = vraw[pl.ds(vb + w, 8, stride=20), :]
            for h, vv in enumerate((_lo(vw), _hi(vw))):
                r = 3 + 2 * w + h
                ks = wts[0] * e[r] + wts[1] * e[r - 1] + wts[2] * e[r - 2] + wts[3] * e[r - 3]
                kv.append(ks * vv)
        tok = None
        for p in range(4):
            pk = _pk2(kv[p], kv[p + 4])
            rx[g, p, pl.ds(8 * t, 8), :] = pk
            tok = pk if tok is None else tok | pk
        return tok

    def prep_k(g, m):
        blk = _bc(skbuf[pl.ds(64 * g, 64), pl.ds(CH * m, CH)])
        ktbuf[g, 0:CH // 2, :] = pltpu.bitcast(blk.T, u32)
        lo16 = jnp.uint32(0xFFFF)
        hi16 = jnp.uint32(0xFFFF0000)
        for t in range(8):
            w = [ktbuf[g, pl.ds(32 * t + e_, 8, stride=4), :] for e_ in range(4)]
            rows = pl.ds(8 * t, 8)
            rk[g, 0, rows, :] = (w[0] & lo16) | (w[2] << 16)
            rk[g, 1, rows, :] = (w[0] >> 16) | (w[2] & hi16)
            rk[g, 2, rows, :] = (w[1] & lo16) | (w[3] << 16)
            rk[g, 3, rows, :] = (w[1] >> 16) | (w[3] & hi16)

    def fwd(src, dst, g, a, b, dvec):
        z = [jnp.dot(_bc(mf_ref[p, pl.ds(RB * b, RB), :]), _bc(src[g, p]),
                     preferred_element_type=f32) for p in range(4)]
        xr, xi = _fft4([t[:RB] for t in z], [t[RB:] for t in z], False)
        for f2 in range(4):
            dst[g, a, f2, 0, pl.ds(RB * b, RB), :] = xr[f2] if dvec is None else xr[f2] + dvec
            dst[g, a, f2, 1, pl.ds(RB * b, RB), :] = xi[f2]

    def cell(g, j, c, mask, inj):
        rows = pl.ds(8 * j, 8)
        zr, zi = [], []
        for f2 in range(4):
            ar = ai = None
            for a in range(c + 1):
                m = c - a
                xr = xh[g, a, f2, 0, rows, :]
                xi = xh[g, a, f2, 1, rows, :]
                kr = kh[g, m, f2, 0, rows, :]
                ki = kh[g, m, f2, 1, rows, :]
                if inj is not None and f2 == 0 and a == 0:
                    kr = jnp.where(mask, inj, kr)
                tr = xr * kr - xi * ki
                ti = xr * ki + xi * kr
                ar = tr if ar is None else ar + tr
                ai = ti if ai is None else ai + ti
            zr.append(ar)
            zi.append(ai)
        yr, yi = zr, zi
        if c > 0:
            pr = [zb[g, f, 0, rows, :] for f in range(4)]
            pi = [zb[g, f, 1, rows, :] for f in range(4)]
            if j < 8:
                yr = [zr[f] - pi[f] for f in range(4)]
                yi = [zi[f] + pr[f] for f in range(4)]
            else:
                yr = [zr[f] + pi[f] for f in range(4)]
                yi = [zi[f] - pr[f] for f in range(4)]
        if c + 1 < NCH:
            for f in range(4):
                zb[g, f, 0, rows, :] = zr[f]
                zb[g, f, 1, rows, :] = zi[f]
        ur, ui = _fft4(yr, yi, True)
        tok = None
        for s2 in range(4):
            pk = _pk2(ur[s2], ui[s2])
            ub[c % 2][g, s2, rows, :] = pk
            tok = pk if tok is None else tok | pk
        return tok

    def inv(g, c, s2):
        y = jnp.dot(_bc(gi_ref[s2]), _bc(ub[c % 2][g, s2, 0:128, :]), preferred_element_type=f32)
        ybuf[g, pl.ds(CH * c + s2, 128, stride=4), :] = y

    def delayed(tok, n):
        t = pltpu.bitcast(tok, f32)
        for _ in range(n):
            t = pl.reciprocal(t, approx=True)
        return t

    def mod_cols(lo_, n):
        cc = c_ref[...].astype(f32)
        sc = (cc * jax.nn.sigmoid(cc)).astype(bf16)
        lhs = jnp.broadcast_to(sc, (8, D))
        modb[:, pl.ds(lo_, n)] = jnp.dot(lhs, _bc(wmb[:, pl.ds(lo_, n)]), preferred_element_type=f32)

    _cnt = [0]

    def first_step():
        i = _cnt[0]
        _cnt[0] += 1
        return zs_ref[i] == 0

    def prologue(row, nchunk):
        sa = modb[0:1, 0 * D:1 * D]
        ca1 = 1.0 + modb[0:1, 1 * D:2 * D]
        ga = modb[0:1, 2 * D:3 * D] * (2.0 / NDFT)
        sb = modb[0:1, 3 * D:4 * D]
        cb1 = 1.0 + modb[0:1, 4 * D:5 * D]
        mask = false_mask()
        n = SB // nchunk
        x1s, h2s = [], []
        tok = None
        for i in range(nchunk):
            r = pl.ds(row + i * n, n)
            q = _bc(qbuf[_half(row + i * n, n), :]).astype(f32)
            if tok is not None:
                q00 = jnp.where(mask, tok, q[0:8, 0:128])
                top = jnp.concatenate([q00, q[0:8, 128:]], axis=1)
                q = jnp.concatenate([top, q[8:]], axis=0)
            y = jnp.concatenate([ybuf[g, r, :] for g in range(NG)], axis=1)
            h1 = _ln(q) * ca1 + sa
            x1 = q + ga * (h1 * y)
            h2f = _ln(x1) * cb1 + sb
            if i + 1 < nchunk:
                parts = [h2f[8 * a:8 * a + 8, 128 * g:128 * (g + 1)]
                         for a in range(n // 8) for g in range(NG)]
                while len(parts) > 1:
                    parts = [parts[k] + parts[k + 1] if k + 1 < len(parts) else parts[k]
                             for k in range(0, len(parts), 2)]
                tok = parts[0]
            x1s.append(x1)
            h2s.append(h2f.astype(bf16))
        return jnp.concatenate(x1s, axis=0), jnp.concatenate(h2s, axis=0)

    def ffn_part(h2, lo_, n):
        cols = pl.ds(lo_, n)
        gate = jnp.dot(h2, _bc(w1b[:, cols]), preferred_element_type=f32)
        up = jnp.dot(h2, _bc(w3b[:, cols]), preferred_element_type=f32)
        act = (gate * jax.nn.sigmoid(gate) * up).astype(bf16)
        return jnp.dot(act, _bc(w2b[_half(lo_, n), :]), preferred_element_type=f32)

    def next_prologue(row, nchunk):
        x1, h2 = prologue(row, nchunk)
        xn[...] = x1
        hn[...] = h2

    cp_s(0).start()
    cp_zs.start(); cp_dv.start()
    cp_s(1).start()
    cp_k(0).start(); cp_v(0).start()
    cp_shk.start(); cp_c.start()
    cp_k(1).start(); cp_v(1).start()
    for a in range(2, NCH):
        cp_s(a).start(); cp_k(a).start(); cp_v(a).start()
    cp_wm(0).start()
    cp_wm(1).start()
    cp_q(0).start()
    for t in range(NFC):
        if t == NFC - 1:
            cp_wm(2).start()
        for c_ in cp_w(t):
            c_.start()
    cp_q(1).start()
    kraw[0:KPAD, :] = jnp.zeros((KPAD, 128), u32)
    gen_forward_dft()
    gen_inverse_dft()
    cp_zs.wait(); cp_dv.wait()

    def fwd_k(a):
        dv = dv_ref[...].astype(f32).reshape(1, D)
        for g in range(NG):
            prep_k(g, a)
            dvec = jnp.broadcast_to(dv[:, 128 * g:128 * (g + 1)], (RB, 128)) if a == 0 else None
            for b in range(128 // RB):
                fwd(rk, kh, g, a, b, dvec)

    def fwd_x(a):
        mask = false_mask()
        shk = shk_ref[...].astype(f32)
        inj = None
        for g in range(NG):
            lanes = slice(128 * g, 128 * (g + 1))
            wts = [jnp.broadcast_to(shk[j:j + 1, lanes], (8, 128)) for j in range(4)]
            for t in range(8):
                tok = prep_x(g, a, t, wts, mask, inj)
                inj = delayed(tok, NRCP_P) if g > 0 else None
            for b in range(128 // RB):
                fwd(rx, xh, g, a, b, None)

    def part_b(c):
        mask = false_mask()
        inj = None
        for g in range(NG):
            for j in range(16):
                tok = cell(g, j, c, mask, inj)
                if RCP_B[c] is not None:
                    n = 16 * g + j
                    inj = delayed(tok, int((n + 1) * RCP_B[c]) - int(n * RCP_B[c]))
        if c > 0:
            for g in range(NG):
                for s2 in range(4):
                    inv(g, c - 1, s2)

    for a in range(2):
        @pl.when(first_step())
        def _filter_side(a=a):
            cp_s(a).wait()
            fwd_k(a)

    for a in range(NCH):
        @pl.when(first_step())
        def _data_side(a=a):
            cp_k(a).wait(); cp_v(a).wait()
            if a == 0:
                cp_shk.wait(); cp_c.wait()
            fwd_x(a)

        if a + 1 < NCH:
            @pl.when(first_step())
            def _products(c=a):
                if c >= 1:
                    cp_s(c + 1).wait()
                part_b(c)
                if c >= 1:
                    fwd_k(c + 1)

    @pl.when(first_step())
    def _products_last():
        cp_wm(0).wait()
        part_b(NCH - 1)
        mod_cols(0, WM0)

    @pl.when(first_step())
    def _finish_conv():
        cp_wm(1).wait()
        cp_q(0).wait()
        mod_cols(WM0, 5 * D - WM0)
        for g in range(NG):
            for s2 in range(4):
                inv(g, NCH - 1, s2)
        x1, h2 = prologue(0, 1)
        xs[0:SB, :] = x1
        hs[0:SB, :] = h2

    for t in range(NFC):
        @pl.when(first_step())
        def _first_rows(t=t):
            for c_ in cp_w(t):
                c_.wait()
            if t == NFC - 1:
                cp_wm(2).wait()
                cp_q(1).wait()
                mod_cols(5 * D, D)
            for j in range(NSB):
                r = pl.ds(j * SB, SB)
                if t == 0:
                    if j == 0:
                        h2 = hs[r, :]
                    else:
                        x1, h2 = prologue(j * SB, PCH_FIRST)
                        xs[r, :] = x1
                        hs[r, :] = h2
                    accs[r, :] = ffn_part(h2, FLO[0], FCS[0])
                elif t < NFC - 1:
                    accs[r, :] += ffn_part(hs[r, :], FLO[t], FCS[t])
                else:
                    gb = modb[0:1, 5 * D:6 * D]
                    ffn = accs[r, :] + ffn_part(hs[r, :], FLO[t], FCS[t])
                    obuf[r, :] = (xs[r, :] + gb * ffn).astype(bf16)
            if t == NFC - 1:
                next_prologue(BM, PCH_STEADY)
                cp_o(0, BM).start()

    def _step(step, carry):
        gb = modb[0:1, 5 * D:6 * D]
        row0 = pl.multiple_of(BM + step * BM2, SB)
        nsb = BM2 // SB
        x1, h2 = xn[...], hn[...]
        for j in range(nsb):
            if j + 1 < nsb:
                nxt = prologue(row0 + (j + 1) * SB, PCH_STEADY)
            else:
                nrow = jnp.minimum(row0 + BM2, S - SB)
                next_prologue(pl.multiple_of(nrow, SB), PCH_STEADY)
            ffn = ffn_part(h2, 0, F)
            obuf[pl.ds(row0 + j * SB, SB), :] = (x1 + gb * ffn).astype(bf16)
            cp_o(row0 + j * SB, SB).start()
            if j + 1 < nsb:
                x1, h2 = nxt
        return carry

    lax.fori_loop(0, NSTEP2, _step, 0)
    cp_o(0, BM).wait()
    for i in range((S - BM) // SB):
        cp_o(BM + i * SB, SB).wait()


def _raw_view(x):
    return x.reshape(S // 8, 8, NG, 128).transpose(0, 2, 1, 3).reshape(NG * S, 128)


@jax.jit
def pallas_adaLN_cond__ssm_conv_h3__glu_gated_swiglu__prompt_kernel(
    A_q: jax.Array,
    A_k: jax.Array,
    A_v: jax.Array,
    A_shift_k: jax.Array,
    A_ssm_k: jax.Array,
    A_ssm_D: jax.Array,
    B_x: jax.Array,
    B_w1: jax.Array,
    B_w3: jax.Array,
    B_w2: jax.Array,
    c: jax.Array,
    w_mod: jax.Array,
):
    del B_x
    any_spec = pl.BlockSpec(memory_space=pl.ANY)
    scratch = [
        pltpu.VMEM((KPAD + 5 * S // 2 + 24, 128), u32),
        pltpu.VMEM((5 * S // 2 + 24, 128), u32),
        pltpu.VMEM((D // 2, S), u32),
        pltpu.VMEM((NG, CH // 2 + 8, 128), u32),
        pltpu.VMEM((NG, 4, 64, 128), u32),
        pltpu.VMEM((NG, 4, 64, 128), u32),
        pltpu.VMEM((NG, NCH, 4, 2, PR, 128), f32),
        pltpu.VMEM((NG, NCH, 4, 2, PR, 128), f32),
        pltpu.VMEM((NG, 4, 2, PR, 128), f32),
        pltpu.VMEM((NG, 4, PR, 128), u32),
        pltpu.VMEM((NG, 4, PR, 128), u32),
        pltpu.VMEM((NG, S + 8, 128), f32),
        pltpu.VMEM((S // 2, D), u32),
        pltpu.VMEM((D // 2, F), u32),
        pltpu.VMEM((D // 2, F), u32),
        pltpu.VMEM((F // 2, D), u32),
        pltpu.VMEM((D // 2, 6 * D), u32),
        pltpu.VMEM((8, 6 * D), f32),
        pltpu.VMEM((SB, D), bf16),
        pltpu.VMEM((SB, D), f32),
        pltpu.VMEM((BM, D), bf16),
        pltpu.VMEM((BM, D), f32),
        pltpu.VMEM((BM, D), f32),
        pltpu.VMEM((S, D), bf16),
        pltpu.VMEM((4, 128, 128), u32),
        pltpu.VMEM((4, 64, 256), u32),
        pltpu.VMEM((4, D), bf16),
        pltpu.VMEM((D,), bf16),
        pltpu.VMEM((1, D), bf16),
        pltpu.SMEM((32,), jnp.int32),
        pltpu.SemaphoreType.DMA((8, 8)),
    ]
    return pl.pallas_call(
        _kernel,
        in_specs=[any_spec] * 12,
        out_specs=any_spec,
        out_shape=jax.ShapeDtypeStruct((1, S, D), bf16),
        scratch_shapes=scratch,
        compiler_params=pltpu.CompilerParams(
            vmem_limit_bytes=100 * 1024 * 1024,
            disable_semaphore_checks=True,
            disable_bounds_checks=True),
    )(A_q, _raw_view(A_k), _raw_view(A_v), A_ssm_k, B_w1, B_w3, B_w2, w_mod,
      A_shift_k.T, A_ssm_D, c,
      jnp.zeros((32,), jnp.int32))
```

```python
import jax
import jax.numpy as jnp
from jax import lax
import jax.experimental.pallas as pl
import jax.experimental.pallas.tpu as pltpu

f32 = jnp.float32
bf16 = jnp.bfloat16
u32 = jnp.uint32

S = 2048
D = 640
F = 1536
NG = D // 128
NCH = 4
CH = S // NCH
NDFT = 2 * CH
EPS = 1e-5

SB = 128
BM = 512
NSB = BM // SB
BM2 = 256
NSTEP2 = (S - BM) // BM2
FCS = (384, 512, 640)
NFC = len(FCS)
FLO = tuple(sum(FCS[:i]) for i in range(NFC))
WM0 = 2304

KPAD = 40
RB = 32
PR = 136

PCH_FIRST, PCH_STEADY = 2, 8
NRCP_P = 1
RCP_B = (None, 1.05, 1.6, 2.05)


def _cos_turns(x):
    fr = x - jnp.floor(x)
    w = 4.0 * jnp.minimum(fr, 1.0 - fr) - 1.0
    w2 = w * w
    acc = jnp.float32(3.598843e-06)
    for coef in (-1.6044118e-04, 4.6817541e-03, -7.9692626e-02, 6.4596410e-01, -1.5707963e+00):
        acc = acc * w2 + jnp.float32(coef)
    return acc * w


def _odd_freq(r):
    return jnp.where(r < 64, 4 * r + 1, 4 * (r - 64) + 3)


def _bc(v):
    return pltpu.bitcast(v, bf16)


def _half(row, n):
    if isinstance(row, int):
        return pl.ds(row // 2, n // 2)
    return pl.ds(pl.multiple_of(row // 2, 8), n // 2)


def _lo(w):
    return pltpu.bitcast(w << 16, f32)


def _hi(w):
    return pltpu.bitcast(w & jnp.uint32(0xFFFF0000), f32)


def _pk2(a, b):
    half = jnp.uint32(0x8000)
    lo = (pltpu.bitcast(a, u32) + half) >> 16
    hi = (pltpu.bitcast(b, u32) + half) & jnp.uint32(0xFFFF0000)
    return lo | hi


def _fft4(zr, zi, inv):
    ar, ai = zr[0] + zr[2], zi[0] + zi[2]
    br, bi = zr[0] - zr[2], zi[0] - zi[2]
    cr, ci = zr[1] + zr[3], zi[1] + zi[3]
    dr, di = zr[1] - zr[3], zi[1] - zi[3]
    if not inv:
        return [ar + cr, br + di, ar - cr, br - di], [ai + ci, bi - dr, ai - ci, bi + dr]
    return [ar + cr, br - di, ar - cr, br + di], [ai + ci, bi + dr, ai - ci, bi - dr]


def _ln(x):
    m = jnp.sum(x, axis=-1, keepdims=True) * (1.0 / D)
    xc = x - m
    v = jnp.sum(xc * xc, axis=-1, keepdims=True) * (1.0 / D)
    return xc * lax.rsqrt(v + EPS)


def _kernel(q_hbm, k_hbm, v_hbm, sk_hbm, w1_hbm, w3_hbm, w2_hbm, wm_hbm,
            shk_hbm, dv_hbm, c_hbm, zs_hbm,
            o_hbm,
            kraw, vraw, skbuf, ktbuf, rx, rk, xh, kh, zb, ub0, ub1, ybuf,
            qbuf, w1b, w3b, w2b, wmb, modb, hn, xn, hs, xs, accs, obuf, mf_ref, gi_ref,
            shk_ref, dv_ref, c_ref, zs_ref, sems):
    ub = (ub0, ub1)

    def cp_k(a):
        return pltpu.make_async_copy(
            k_hbm.at[pl.ds(5 * CH * a, 5 * CH), :],
            kraw.bitcast(bf16).at[pl.ds(2 * KPAD + 5 * CH * a, 5 * CH), :], sems.at[0, a])

    def cp_v(a):
        return pltpu.make_async_copy(
            v_hbm.at[pl.ds(5 * CH * a, 5 * CH), :],
            vraw.bitcast(bf16).at[pl.ds(5 * CH * a, 5 * CH), :], sems.at[1, a])

    def cp_s(a):
        cols = pl.ds(CH * a, CH)
        return pltpu.make_async_copy(sk_hbm.at[:, cols], skbuf.bitcast(bf16).at[:, cols], sems.at[2, a])

    def cp_wm(i):
        cols = [pl.ds(0, WM0), pl.ds(WM0, 5 * D - WM0), pl.ds(5 * D, D)][i]
        return pltpu.make_async_copy(wm_hbm.at[:, cols], wmb.bitcast(bf16).at[:, cols], sems.at[3, i])

    def cp_q(i):
        rows = pl.ds(0, BM) if i == 0 else pl.ds(BM, S - BM)
        return pltpu.make_async_copy(q_hbm.at[0, rows, :], qbuf.bitcast(bf16).at[rows, :], sems.at[3, 4 + i])

    def cp_w(t):
        cols = pl.ds(FLO[t], FCS[t])
        return [pltpu.make_async_copy(w1_hbm.at[:, cols], w1b.bitcast(bf16).at[:, cols], sems.at[4, t]),
                pltpu.make_async_copy(w3_hbm.at[:, cols], w3b.bitcast(bf16).at[:, cols], sems.at[5, t]),
                pltpu.make_async_copy(w2_hbm.at[cols, :], w2b.bitcast(bf16).at[cols, :], sems.at[6, t])]

    cp_zs, cp_dv, cp_shk, cp_c = [
        pltpu.make_async_copy(src, dst, sems.at[7, 1 + i]) for i, (src, dst) in enumerate(
            [(zs_hbm, zs_ref), (dv_hbm, dv_ref), (shk_hbm, shk_ref), (c_hbm, c_ref)])]

    def false_mask():
        return jnp.full((8, 128), zs_ref[31], jnp.int32) != 0

    def cp_o(row, n):
        rows = pl.ds(row, n)
        return pltpu.make_async_copy(obuf.at[rows, :], o_hbm.at[0, rows, :], sems.at[7, 0])

    def gen_forward_dft():
        i32 = jnp.int32
        wrow = lax.broadcasted_iota(i32, (128, 128), 0)
        n4 = (4 * lax.broadcasted_iota(i32, (128, 128), 1)).astype(f32)
        coef, quarter = [], []
        for h in range(2):
            rho = 2 * wrow + h
            rem = rho % (2 * RB)
            r = RB * (rho // (2 * RB)) + rem % RB
            coef.append(_odd_freq(r).astype(f32) * (0.5 / NDFT))
            quarter.append((rem // RB).astype(f32) * 0.25)
        for p in range(4):
            v = [_cos_turns(coef[h] * (n4 + float(p)) + quarter[h]) for h in range(2)]
            mf_ref[p] = _pk2(v[0], v[1])

    def gen_inverse_dft():
        i32 = jnp.int32
        wrow = lax.broadcasted_iota(i32, (64, 256), 0)
        col = lax.broadcasted_iota(i32, (64, 256), 1)
        coef = _odd_freq(col // 2).astype(f32) * (0.5 / NDFT)
        quarter = (col % 2).astype(f32) * 0.25
        for p in range(4):
            v = [_cos_turns(coef * (8 * wrow + (4 * h + p)).astype(f32) + quarter) for h in range(2)]
            gi_ref[p] = _pk2(v[0], v[1])

    def prep_x(g, a, t, wts, mask, inj):
        i0_ = 64 * a + 8 * t
        kb = KPAD + 20 * i0_ + 4 * g
        kl = [kraw[pl.ds(kb + w, 8, stride=20), :] for w in range(4)]
        km2 = kraw[pl.ds(kb - 18, 8, stride=20), :]
        km3 = kraw[pl.ds(kb - 17, 8, stride=20), :]
        e = [_hi(km2), _lo(km3), _hi(km3)]
        for w in range(4):
            e += [_lo(kl[w]), _hi(kl[w])]
        if inj is not None:
            e[3] = jnp.where(mask, inj, e[3])
        vb = 20 * i0_ + 4 * g
        kv = []
        for w in range(4):
            vw = vraw[pl.ds(vb + w, 8, stride=20), :]
            for h, vv in enumerate((_lo(vw), _hi(vw))):
                r = 3 + 2 * w + h
                ks = wts[0] * e[r] + wts[1] * e[r - 1] + wts[2] * e[r - 2] + wts[3] * e[r - 3]
                kv.append(ks * vv)
        tok = None
        for p in range(4):
            pk = _pk2(kv[p], kv[p + 4])
            rx[g, p, pl.ds(8 * t, 8), :] = pk
            tok = pk if tok is None else tok | pk
        return tok

    def prep_k(g, m):
        blk = _bc(skbuf[pl.ds(64 * g, 64), pl.ds(CH * m, CH)])
        ktbuf[g, 0:CH // 2, :] = pltpu.bitcast(blk.T, u32)
        lo16 = jnp.uint32(0xFFFF)
        hi16 = jnp.uint32(0xFFFF0000)
        for t in range(8):
            w = [ktbuf[g, pl.ds(32 * t + e_, 8, stride=4), :] for e_ in range(4)]
            rows = pl.ds(8 * t, 8)
            rk[g, 0, rows, :] = (w[0] & lo16) | (w[2] << 16)
            rk[g, 1, rows, :] = (w[0] >> 16) | (w[2] & hi16)
            rk[g, 2, rows, :] = (w[1] & lo16) | (w[3] << 16)
            rk[g, 3, rows, :] = (w[1] >> 16) | (w[3] & hi16)

    def fwd(src, dst, g, a, b, dvec):
        z = [jnp.dot(_bc(mf_ref[p, pl.ds(RB * b, RB), :]), _bc(src[g, p]),
                     preferred_element_type=f32) for p in range(4)]
        xr, xi = _fft4([t[:RB] for t in z], [t[RB:] for t in z], False)
        for f2 in range(4):
            dst[g, a, f2, 0, pl.ds(RB * b, RB), :] = xr[f2] if dvec is None else xr[f2] + dvec
            dst[g, a, f2, 1, pl.ds(RB * b, RB), :] = xi[f2]

    def cell(g, j, c, mask, inj):
        rows = pl.ds(8 * j, 8)
        zr, zi = [], []
        for f2 in range(4):
            ar = ai = None
            for a in range(c + 1):
                m = c - a
                xr = xh[g, a, f2, 0, rows, :]
                xi = xh[g, a, f2, 1, rows, :]
                kr = kh[g, m, f2, 0, rows, :]
                ki = kh[g, m, f2, 1, rows, :]
                if inj is not None and f2 == 0 and a == 0:
                    kr = jnp.where(mask, inj, kr)
                tr = xr * kr - xi * ki
                ti = xr * ki + xi * kr
                ar = tr if ar is None else ar + tr
                ai = ti if ai is None else ai + ti
            zr.append(ar)
            zi.append(ai)
        yr, yi = zr, zi
        if c > 0:
            pr = [zb[g, f, 0, rows, :] for f in range(4)]
            pi = [zb[g, f, 1, rows, :] for f in range(4)]
            if j < 8:
                yr = [zr[f] - pi[f] for f in range(4)]
                yi = [zi[f] + pr[f] for f in range(4)]
            else:
                yr = [zr[f] + pi[f] for f in range(4)]
                yi = [zi[f] - pr[f] for f in range(4)]
        if c + 1 < NCH:
            for f in range(4):
                zb[g, f, 0, rows, :] = zr[f]
                zb[g, f, 1, rows, :] = zi[f]
        ur, ui = _fft4(yr, yi, True)
        tok = None
        for s2 in range(4):
            pk = _pk2(ur[s2], ui[s2])
            ub[c % 2][g, s2, rows, :] = pk
            tok = pk if tok is None else tok | pk
        return tok

    def inv(g, c, s2):
        y = jnp.dot(_bc(gi_ref[s2]), _bc(ub[c % 2][g, s2, 0:128, :]), preferred_element_type=f32)
        ybuf[g, pl.ds(CH * c + s2, 128, stride=4), :] = y

    def delayed(tok, n):
        t = pltpu.bitcast(tok, f32)
        for _ in range(n):
            t = pl.reciprocal(t, approx=True)
        return t

    def mod_cols(lo_, n):
        cc = c_ref[...].astype(f32)
        sc = (cc * jax.nn.sigmoid(cc)).astype(bf16)
        lhs = jnp.broadcast_to(sc, (8, D))
        modb[:, pl.ds(lo_, n)] = jnp.dot(lhs, _bc(wmb[:, pl.ds(lo_, n)]), preferred_element_type=f32)

    _cnt = [0]

    def first_step():
        i = _cnt[0]
        _cnt[0] += 1
        return zs_ref[i] == 0

    def prologue(row, nchunk):
        sa = modb[0:1, 0 * D:1 * D]
        ca1 = 1.0 + modb[0:1, 1 * D:2 * D]
        ga = modb[0:1, 2 * D:3 * D] * (2.0 / NDFT)
        sb = modb[0:1, 3 * D:4 * D]
        cb1 = 1.0 + modb[0:1, 4 * D:5 * D]
        mask = false_mask()
        n = SB // nchunk
        x1s, h2s = [], []
        tok = None
        for i in range(nchunk):
            r = pl.ds(row + i * n, n)
            q = _bc(qbuf[_half(row + i * n, n), :]).astype(f32)
            if tok is not None:
                q00 = jnp.where(mask, tok, q[0:8, 0:128])
                top = jnp.concatenate([q00, q[0:8, 128:]], axis=1)
                q = jnp.concatenate([top, q[8:]], axis=0)
            y = jnp.concatenate([ybuf[g, r, :] for g in range(NG)], axis=1)
            h1 = _ln(q) * ca1 + sa
            x1 = q + ga * (h1 * y)
            h2f = _ln(x1) * cb1 + sb
            if i + 1 < nchunk:
                parts = [h2f[8 * a:8 * a + 8, 128 * g:128 * (g + 1)]
                         for a in range(n // 8) for g in range(NG)]
                while len(parts) > 1:
                    parts = [parts[k] + parts[k + 1] if k + 1 < len(parts) else parts[k]
                             for k in range(0, len(parts), 2)]
                tok = parts[0]
            x1s.append(x1)
            h2s.append(h2f.astype(bf16))
        return jnp.concatenate(x1s, axis=0), jnp.concatenate(h2s, axis=0)

    def ffn_part(h2, lo_, n):
        cols = pl.ds(lo_, n)
        gate = jnp.dot(h2, _bc(w1b[:, cols]), preferred_element_type=f32)
        up = jnp.dot(h2, _bc(w3b[:, cols]), preferred_element_type=f32)
        act = (gate * jax.nn.sigmoid(gate) * up).astype(bf16)
        return jnp.dot(act, _bc(w2b[_half(lo_, n), :]), preferred_element_type=f32)

    def next_prologue(row, nchunk):
        x1, h2 = prologue(row, nchunk)
        xn[...] = x1
        hn[...] = h2

    cp_s(0).start()
    cp_zs.start(); cp_dv.start()
    cp_s(1).start()
    cp_k(0).start(); cp_v(0).start()
    cp_shk.start(); cp_c.start()
    cp_k(1).start(); cp_v(1).start()
    for a in range(2, NCH):
        cp_s(a).start(); cp_k(a).start(); cp_v(a).start()
    cp_wm(0).start()
    cp_wm(1).start()
    cp_q(0).start()
    for t in range(NFC):
        if t == NFC - 1:
            cp_wm(2).start()
        for c_ in cp_w(t):
            c_.start()
    cp_q(1).start()
    kraw[0:KPAD, :] = jnp.zeros((KPAD, 128), u32)
    gen_forward_dft()
    gen_inverse_dft()
    cp_zs.wait(); cp_dv.wait()

    def fwd_k(a):
        dv = dv_ref[...].astype(f32).reshape(1, D)
        for g in range(NG):
            prep_k(g, a)
            dvec = jnp.broadcast_to(dv[:, 128 * g:128 * (g + 1)], (RB, 128)) if a == 0 else None
            for b in range(128 // RB):
                fwd(rk, kh, g, a, b, dvec)

    def fwd_x(a):
        mask = false_mask()
        shk = shk_ref[...].astype(f32)
        inj = None
        for g in range(NG):
            lanes = slice(128 * g, 128 * (g + 1))
            wts = [jnp.broadcast_to(shk[j:j + 1, lanes], (8, 128)) for j in range(4)]
            for t in range(8):
                tok = prep_x(g, a, t, wts, mask, inj)
                inj = delayed(tok, NRCP_P) if g > 0 else None
            for b in range(128 // RB):
                fwd(rx, xh, g, a, b, None)

    def part_b(c):
        mask = false_mask()
        inj = None
        for g in range(NG):
            for j in range(16):
                tok = cell(g, j, c, mask, inj)
                if RCP_B[c] is not None:
                    n = 16 * g + j
                    inj = delayed(tok, int((n + 1) * RCP_B[c]) - int(n * RCP_B[c]))
        if c > 0:
            for g in range(NG):
                for s2 in range(4):
                    inv(g, c - 1, s2)

    for a in range(2):
        @pl.when(first_step())
        def _filter_side(a=a):
            cp_s(a).wait()
            fwd_k(a)

    for a in range(NCH):
        @pl.when(first_step())
        def _data_side(a=a):
            cp_k(a).wait(); cp_v(a).wait()
            if a == 0:
                cp_shk.wait(); cp_c.wait()
            fwd_x(a)

        if a + 1 < NCH:
            @pl.when(first_step())
            def _products(c=a):
                if c >= 1:
                    cp_s(c + 1).wait()
                part_b(c)
                if c >= 1:
                    fwd_k(c + 1)

    @pl.when(first_step())
    def _products_last():
        cp_wm(0).wait()
        part_b(NCH - 1)
        mod_cols(0, WM0)

    @pl.when(first_step())
    def _finish_conv():
        cp_wm(1).wait()
        cp_q(0).wait()
        mod_cols(WM0, 5 * D - WM0)
        for g in range(NG):
            for s2 in range(4):
                inv(g, NCH - 1, s2)
        x1, h2 = prologue(0, 1)
        xs[0:SB, :] = x1
        hs[0:SB, :] = h2

    for t in range(NFC):
        @pl.when(first_step())
        def _first_rows(t=t):
            for c_ in cp_w(t):
                c_.wait()
            if t == NFC - 1:
                cp_wm(2).wait()
                cp_q(1).wait()
                mod_cols(5 * D, D)
            for j in range(NSB):
                r = pl.ds(j * SB, SB)
                if t == 0:
                    if j == 0:
                        h2 = hs[r, :]
                    else:
                        x1, h2 = prologue(j * SB, PCH_FIRST)
                        xs[r, :] = x1
                        hs[r, :] = h2
                    accs[r, :] = ffn_part(h2, FLO[0], FCS[0])
                elif t < NFC - 1:
                    accs[r, :] += ffn_part(hs[r, :], FLO[t], FCS[t])
                else:
                    gb = modb[0:1, 5 * D:6 * D]
                    ffn = accs[r, :] + ffn_part(hs[r, :], FLO[t], FCS[t])
                    obuf[r, :] = (xs[r, :] + gb * ffn).astype(bf16)
            if t == NFC - 1:
                next_prologue(BM, PCH_STEADY)
                cp_o(0, BM).start()

    def _step(step, carry):
        gb = modb[0:1, 5 * D:6 * D]
        row0 = pl.multiple_of(BM + step * BM2, SB)
        nsb = BM2 // SB
        x1, h2 = xn[...], hn[...]
        for j in range(nsb):
            if j + 1 < nsb:
                nxt = prologue(row0 + (j + 1) * SB, PCH_STEADY)
            else:
                nrow = jnp.minimum(row0 + BM2, S - SB)
                next_prologue(pl.multiple_of(nrow, SB), PCH_STEADY)
            ffn = ffn_part(h2, 0, F)
            obuf[pl.ds(row0 + j * SB, SB), :] = (x1 + gb * ffn).astype(bf16)
            cp_o(row0 + j * SB, SB).start()
            if j + 1 < nsb:
                x1, h2 = nxt
        return carry

    lax.fori_loop(0, NSTEP2, _step, 0)
    cp_o(0, BM).wait()
    for i in range((S - BM) // SB):
        cp_o(BM + i * SB, SB).wait()


def _raw_view(x):
    return x.reshape(S // 8, 8, NG, 128).transpose(0, 2, 1, 3).reshape(NG * S, 128)


@jax.jit
def pallas_adaLN_cond__ssm_conv_h3__glu_gated_swiglu__prompt_kernel(
    A_q: jax.Array,
    A_k: jax.Array,
    A_v: jax.Array,
    A_shift_k: jax.Array,
    A_ssm_k: jax.Array,
    A_ssm_D: jax.Array,
    B_x: jax.Array,
    B_w1: jax.Array,
    B_w3: jax.Array,
    B_w2: jax.Array,
    c: jax.Array,
    w_mod: jax.Array,
):
    del B_x
    any_spec = pl.BlockSpec(memory_space=pl.ANY)
    scratch = [
        pltpu.VMEM((KPAD + 5 * S // 2 + 24, 128), u32),
        pltpu.VMEM((5 * S // 2 + 24, 128), u32),
        pltpu.VMEM((D // 2, S), u32),
        pltpu.VMEM((NG, CH // 2 + 8, 128), u32),
        pltpu.VMEM((NG, 4, 64, 128), u32),
        pltpu.VMEM((NG, 4, 64, 128), u32),
        pltpu.VMEM((NG, NCH, 4, 2, PR, 128), f32),
        pltpu.VMEM((NG, NCH, 4, 2, PR, 128), f32),
        pltpu.VMEM((NG, 4, 2, PR, 128), f32),
        pltpu.VMEM((NG, 4, PR, 128), u32),
        pltpu.VMEM((NG, 4, PR, 128), u32),
        pltpu.VMEM((NG, S + 8, 128), f32),
        pltpu.VMEM((S // 2, D), u32),
        pltpu.VMEM((D // 2, F), u32),
        pltpu.VMEM((D // 2, F), u32),
        pltpu.VMEM((F // 2, D), u32),
        pltpu.VMEM((D // 2, 6 * D), u32),
        pltpu.VMEM((8, 6 * D), f32),
        pltpu.VMEM((SB, D), bf16),
        pltpu.VMEM((SB, D), f32),
        pltpu.VMEM((BM, D), bf16),
        pltpu.VMEM((BM, D), f32),
        pltpu.VMEM((BM, D), f32),
        pltpu.VMEM((S, D), bf16),
        pltpu.VMEM((4, 128, 128), u32),
        pltpu.VMEM((4, 64, 256), u32),
        pltpu.VMEM((4, D), bf16),
        pltpu.VMEM((D,), bf16),
        pltpu.VMEM((1, D), bf16),
        pltpu.SMEM((32,), jnp.int32),
        pltpu.SemaphoreType.DMA((8, 8)),
    ]
    return pl.pallas_call(
        _kernel,
        in_specs=[any_spec] * 12,
        out_specs=any_spec,
        out_shape=jax.ShapeDtypeStruct((1, S, D), bf16),
        scratch_shapes=scratch,
        compiler_params=pltpu.CompilerParams(
            vmem_limit_bytes=100 * 1024 * 1024,
            disable_semaphore_checks=True,
            disable_bounds_checks=True),
    )(A_q, _raw_view(A_k), _raw_view(A_v), A_ssm_k, B_w1, B_w3, B_w2, w_mod,
      A_shift_k.T, A_ssm_D, c,
      jnp.zeros((32,), jnp.int32))
```
